```python
import jax
import jax.numpy as jnp

def _softmax(x, axis=-1):
    return jax.nn.softmax(x, axis=axis)
def _gelu(x):
    return jax.nn.gelu(x, approximate=True)
def _silu(x):
    return jax.nn.silu(x)
def _sigmoid(x):
    return jax.nn.sigmoid(x)
def _layernorm(x, axis=-1, eps=1e-5):
    m = jnp.mean(x, axis=axis, keepdims=True)
    v = jnp.var(x, axis=axis, keepdims=True)
    return (x - m) / jnp.sqrt(v + eps)
def _scatter_add(tgt, idx, src, axis=0):
    return tgt.at[idx].add(src)
def _segment_sum(src, seg, n):
    return jax.ops.segment_sum(src, seg, n)
class _Rng:
    def __init__(self, key):
        self._k = key
    def _next(self):
        self._k, sub = jax.random.split(self._k)
        return sub
    def normal(self, shape):
        return jax.random.normal(self._next(), shape, dtype=jnp.bfloat16)
    def randint(self, lo, hi, shape):
        return jax.random.randint(self._next(), shape, lo, hi, dtype=jnp.int32)
    def uniform(self, shape, lo=0.0, hi=1.0):
        return jax.random.uniform(self._next(), shape, jnp.bfloat16, lo, hi)
    def permutation(self, n):
        return jax.random.permutation(self._next(), n)


kernel_name = 'concat_heads__sliding_block_cached__compressed_kv_cla__decode'

def setup_inputs():
    _rng = _Rng(jax.random.key(int.from_bytes(__import__("os").urandom(4), "little")))
    _w = (lambda a: (lambda t: t.astype(jnp.bfloat16) if jnp.issubdtype(t.dtype, jnp.floating) else t)(jnp.asarray(a)))
    def _A_setup():
        B, Sq, D = 4, 1, 512
        Hq, Hkv, Sk, Dh = 32, 32, 4096, 128
        assert Hq % Hkv == 0, (Hq, Hkv)
        return {
            "x": _w((lambda *s: _rng.normal(s) * 0.05)(B, Sq, D)),
            "k_cache": _w((lambda *s: _rng.normal(s) * 0.05)(B, Hkv, Sk, Dh)),
            "v_cache": _w((lambda *s: _rng.normal(s) * 0.05)(B, Hkv, Sk, Dh)),
            "wq": _w((lambda *s: _rng.normal(s) * 0.05)(D, Hq * Dh) * (D ** -0.5)),
            "wo": _w((lambda *s: _rng.normal(s) * 0.05)(Hq * Dh, D) * ((Hq * Dh) ** -0.5)),
        }
    _A_in = _A_setup()

    def _B_setup():
        B, H, Sq, Sk, D, M = 4, 32, 1, 4096, 128, 512
        Dc = 4 * D
        return {
            "x": _w((lambda *s: _rng.normal(s) * 0.05)(B, Sq, M)),
            "c_kv": _w((lambda *s: _rng.normal(s) * 0.05)(B, Sk, Dc)),
            "w_q": _w((lambda *s: _rng.normal(s) * 0.05)(M, H, D) * (M ** -0.5)),
            "w_uk": _w((lambda *s: _rng.normal(s) * 0.05)(Dc, H, D) * (Dc ** -0.5)),
            "w_uv": _w((lambda *s: _rng.normal(s) * 0.05)(Dc, H, D) * (Dc ** -0.5)),
            "w_o": _w((lambda *s: _rng.normal(s) * 0.05)(H, D, M) * ((H * D) ** -0.5)),
        }
    _B_in = _B_setup()

    return {
        "A_x": _A_in["x"],
        "A_k_cache": _A_in["k_cache"],
        "A_v_cache": _A_in["v_cache"],
        "A_wq": _A_in["wq"],
        "A_wo": _A_in["wo"],
        "B_x": _B_in["x"],
        "B_c_kv": _B_in["c_kv"],
        "B_w_q": _B_in["w_q"],
        "B_w_uk": _B_in["w_uk"],
        "B_w_uv": _B_in["w_uv"],
        "B_w_o": _B_in["w_o"],
    }

def reference(A_x, A_k_cache, A_v_cache, A_wq, A_wo, B_x, B_c_kv, B_w_q, B_w_uk, B_w_uv, B_w_o):
    def _A_ref(x, k_cache, v_cache, wq, wo):
        B, Sq, D = x.shape
        Hq, Dh = 32, 128
        Hkv, Sk = k_cache.shape[1], k_cache.shape[2]
        W = min(4096, max(256, Sk // 4))
        rep = Hq // Hkv
        q = (lambda x, *d: x.transpose(*d))((x @ wq).reshape(B, Sq, Hq, Dh), 0, 2, 1, 3)
        k = jnp.repeat(k_cache[:, :, Sk - W:, :], rep, axis=1)
        v = jnp.repeat(v_cache[:, :, Sk - W:, :], rep, axis=1)
        scores = jnp.einsum("bhqd,bhkd->bhqk", q, k) * (Dh ** -0.5)
        p = _softmax(scores, axis=-1)
        o = jnp.einsum("bhqk,bhkd->bhqd", p, v)
        return (lambda x, *d: x.transpose(*d))(o, 0, 2, 1, 3).reshape(B, Sq, Hq * Dh) @ wo

    def _B_ref(x, c_kv, w_q, w_uk, w_uv, w_o):
        B, Sq, M = x.shape[0], x.shape[1], x.shape[2]
        Sk = c_kv.shape[1]
        H, D = w_q.shape[1], w_q.shape[2]
        q = jnp.einsum("bqm,mhd->bhqd", x, w_q)
        k = jnp.einsum("bkc,chd->bhkd", c_kv, w_uk)
        v = jnp.einsum("bkc,chd->bhkd", c_kv, w_uv)
        scores = jnp.einsum("bhqd,bhkd->bhqk", q, k) * (D ** -0.5)
        off = Sk - Sq
        qi = jnp.arange(Sq)[:, None]
        kj = jnp.arange(Sk)[None, :]
        cmask = kj <= (qi + off)
        scores = jnp.where(cmask[None, None], scores, -1e9)
        p = _softmax(scores, axis=-1)
        ctx = jnp.einsum("bhqk,bhkd->bhqd", p, v)
        return jnp.einsum("bhqd,hdm->bqm", ctx, w_o)

    a = _A_ref(A_x, A_k_cache, A_v_cache, A_wq, A_wo)
    b = _B_ref(B_x, B_c_kv, B_w_q, B_w_uk, B_w_uv, B_w_o)
    return jnp.concatenate([a, b], axis=-1)
```

```python
import jax
import jax.numpy as jnp
from jax import lax
import jax.experimental.pallas as pl
import jax.experimental.pallas.tpu as pltpu

F32 = jnp.float32
BF16 = jnp.bfloat16
_NT = (((1,), (1,)), ((), ()))
_NN = (((1,), (0,)), ((), ()))

LO, HI = 1, 0
NS = 16
PRE_IT = NS // 4
C_ITERS = 64
A_ITERS = 256


def _dot(a, b):
    return lax.dot_general(a, b, _NN, preferred_element_type=F32)


def _dot_nt(a, b):
    return lax.dot_general(a, b, _NT, preferred_element_type=F32)


def _kernel(xa_hbm, k_hbm, v_hbm, wq_hbm, wo_hbm, xb_hbm, c_hbm, wbq_hbm, wuk_hbm,
            wuv_hbm, wbo_hbm, out_ref,
            kvbuf, cbuf, wq_buf, wo_buf, wbq_buf, wuk_buf, wuv_buf, wbo_buf,
            xa_buf, xb_buf, e0_ref, xa32_ref, xb32_ref,
            qa_ref, sa_ref, pa_ref, linv_ref, oacc_ref, oa_ref,
            qb_ref, qabs_ref, sb_ref, mb_ref, lb_ref, cacc_ref, cc_ref, ctx_ref,
            acca_ref, accb_ref,
            lsem, hsem, xsem, *, win_off, scale):

    def low_c(it, t):
        pair = it // 32
        row = pl.multiple_of((it % 32) * 32 + t * 8, 8)
        seg = pair * 8
        return pltpu.make_async_copy(
            c_hbm.at[pl.ds(seg, 8), pl.ds(row, 8), :],
            cbuf.at[pl.ds(seg, 8), pl.ds(row, 8), :],
            lsem.at[(it % PRE_IT) * 4 + t])

    def low_kv(src, i, t):
        g = i // 16
        r = i % 16
        head = (g % 4) * 32 + (g // 4) * 8
        row = pl.multiple_of((r % 8) * 128 + t * 32, 32)
        return pltpu.make_async_copy(
            src.at[pl.ds(head, 8), pl.ds(win_off + row, 32), :],
            kvbuf.at[r // 8, :, pl.ds(row, 32), :],
            lsem.at[(i % PRE_IT) * 4 + t])

    def start_low_kv(i, t):
        @pl.when(i % 16 < 8)
        def _():
            low_kv(k_hbm, i, t).start(priority=LO)

        @pl.when(i % 16 >= 8)
        def _():
            low_kv(v_hbm, i, t).start(priority=LO)

    def high_wq(n):
        row = pl.multiple_of((n // 2) * 8, 8)
        col = pl.multiple_of((n % 2) * 2048, 2048)
        return pltpu.make_async_copy(
            wq_hbm.at[pl.ds(row, 8), pl.ds(col, 2048)],
            wq_buf.at[pl.ds(row, 8), pl.ds(col, 2048)], hsem.at[0])

    def high_3d(src, dst, n, rows, sem):
        return pltpu.make_async_copy(
            src.at[pl.ds(n * rows, rows)], dst.at[pl.ds(n * rows, rows)], hsem.at[sem])

    def high_2d(src, dst, n, sem):
        row = pl.multiple_of(n * 16, 16)
        return pltpu.make_async_copy(
            src.at[pl.ds(row, 16), :], dst.at[pl.ds(row, 16), :], hsem.at[sem])

    def start_high_a(i, t):
        n = (i % 64) * 4 + t

        @pl.when(i < 64)
        def _():
            high_3d(wuk_hbm, wuk_buf, n, 2, 2).start(priority=HI)

        @pl.when(jnp.logical_and(i >= 64, i < 128))
        def _():
            high_3d(wuv_hbm, wuv_buf, n, 2, 3).start(priority=HI)

        @pl.when(jnp.logical_and(i >= 128, i < 192))
        def _():
            high_2d(wbo_hbm, wbo_buf, n, 4).start(priority=HI)

        @pl.when(jnp.logical_and(i >= 192, i < 256))
        def _():
            high_2d(wo_hbm, wo_buf, n, 5 + (i % 64) // 16).start(priority=HI)

    def wait_all(buf, sem):
        pltpu.make_async_copy(buf, buf, hsem.at[sem]).wait()

    for t in range(4):
        low_c(0, t).start(priority=LO)
    cp_xa = pltpu.make_async_copy(xa_hbm, xa_buf, xsem.at[0])
    cp_xb = pltpu.make_async_copy(xb_hbm, xb_buf, xsem.at[1])
    cp_xa.start(priority=HI)
    cp_xb.start(priority=HI)
    pltpu.make_async_copy(wq_hbm.at[pl.ds(0, NS * 4), :], wq_buf.at[pl.ds(0, NS * 4), :],
                          hsem.at[0]).start(priority=HI)
    for it in range(1, PRE_IT):
        for t in range(4):
            low_c(it, t).start(priority=LO)

    row8 = lax.broadcasted_iota(jnp.int32, (8, 128), 0)
    row32 = lax.broadcasted_iota(jnp.int32, (32, 128), 0) & 7
    lane32 = lax.broadcasted_iota(jnp.int32, (32, 128), 1) & 7

    def e0_body(i, c):
        r0 = pl.multiple_of(i * 16, 16)
        rr = lax.broadcasted_iota(jnp.int32, (16, 1024), 0) + r0
        cc = lax.broadcasted_iota(jnp.int32, (16, 1024), 1) >> 3
        e0_ref[pl.ds(r0, 16), :] = jnp.where(rr == cc, 1.0, 0.0).astype(BF16)
        return c
    lax.fori_loop(0, 8, e0_body, 0)

    qb_ref[...] = jnp.zeros(qb_ref.shape, F32)
    ctx_ref[...] = jnp.zeros(ctx_ref.shape, F32)
    acca_ref[...] = jnp.zeros(acca_ref.shape, F32)
    accb_ref[...] = jnp.zeros(accb_ref.shape, F32)

    cp_xa.wait()
    cp_xb.wait()
    xa = xa_buf[...].astype(F32)
    xb = xb_buf[...].astype(F32)
    for b in range(4):
        xa32_ref[8 * b:8 * b + 8, :] = jnp.broadcast_to(xa[b:b + 1, :], (8, 512))
        for u in range(4):
            xb32_ref[u, 8 * b:8 * b + 8, :] = jnp.broadcast_to(
                xb[b:b + 1, 128 * u:128 * u + 128], (8, 128))

    def qa_item(n):
        hg = n // 4
        x32 = xa32_ref[...].astype(BF16)
        col = pl.multiple_of(n * 256, 256)
        w = wq_buf[:, pl.ds(col, 256)]
        r = _dot(x32, w)
        j0 = (n % 4) * 2
        old = jnp.where(n % 4 == 0, 0.0, qa_ref[hg])
        new = jnp.where(row32 == j0, r[:, :128], old)
        new = jnp.where(row32 == j0 + 1, r[:, 128:], new)
        qa_ref[hg] = new

    def expand_proj(c32, w_buf, hg, u, acc_ref):
        ce = _dot(c32.astype(BF16), e0_ref[...])
        ce = jnp.concatenate(
            [jnp.where(row32 == lane32, ce[:, 128 * k:128 * k + 128], 0.0).astype(BF16)
             for k in range(8)], axis=1)
        w = w_buf[pl.ds(u * 128, 128), hg].reshape(1024, 128)
        acc_ref[hg] = acc_ref[hg] + _dot(ce, w)

    def qabs_item(hg, u):
        q = qb_ref[hg].astype(BF16)
        w = wuk_buf[pl.ds(u * 128, 128), hg].reshape(1024, 128)
        r = _dot_nt(q, w)
        r = jnp.concatenate(
            [jnp.where(row32 == lane32, r[:, 128 * k:128 * k + 128], 0.0).astype(BF16)
             for k in range(8)], axis=1)
        qa = _dot_nt(r, e0_ref[...])
        for b in range(4):
            qabs_ref[u, b, hg] = qa[8 * b:8 * b + 8, :]

    def score_item(b, n):
        qa = jnp.concatenate(
            [qabs_ref[u, b].reshape(32, 128).astype(BF16) for u in range(4)], axis=1)
        row = pl.multiple_of((n % 4) * 256, 256)
        c = cbuf[b * 4 + n // 4, pl.ds(row, 256), :]
        s = _dot_nt(qa, c)
        sb_ref[n] = s
        m = jnp.maximum(s[:, :128], s[:, 128:])
        m = jnp.maximum(m, jnp.where(n == 0, -jnp.inf, mb_ref[...]))

        @pl.when(n < 15)
        def _():
            mb_ref[...] = m

        @pl.when(n == 15)
        def _():
            mb_ref[...] = jnp.broadcast_to(jnp.max(m, axis=1, keepdims=True), (32, 128))
            lb_ref[...] = jnp.zeros(lb_ref.shape, F32)
            cacc_ref[...] = jnp.zeros(cacc_ref.shape, F32)

    def pv_item(b, n):
        s = sb_ref[n]
        m = mb_ref[...]
        p0 = jnp.exp((s[:, :128] - m) * scale)
        p1 = jnp.exp((s[:, 128:] - m) * scale)
        lsum = lb_ref[...] + (p0 + p1)
        lb_ref[...] = lsum
        p = jnp.concatenate([p0.astype(BF16), p1.astype(BF16)], axis=1)
        row = pl.multiple_of((n % 4) * 256, 256)
        c = cbuf[b * 4 + n // 4, pl.ds(row, 256), :]
        acc = cacc_ref[...] + _dot(p, c)
        cacc_ref[...] = acc

        @pl.when(n == 15)
        def _():
            inv = 1.0 / jnp.sum(lsum, axis=1, keepdims=True)
            res = acc * inv
            for u in range(4):
                cc_ref[u, b] = res[:, 128 * u:128 * u + 128].reshape(4, 8, 128)

    def out_item(o32, w_buf, hg, u, acc_ref):
        lhs = jnp.concatenate(
            [jnp.where(row32 == 2 * u, o32, 0.0).astype(BF16),
             jnp.where(row32 == 2 * u + 1, o32, 0.0).astype(BF16)], axis=1)
        row = pl.multiple_of(hg * 1024 + u * 256, 256)
        acc_ref[...] = acc_ref[...] + _dot(lhs, w_buf[pl.ds(row, 256), :])

    def finish(acc):
        return jnp.sum(acc.reshape(4, 8, 512), axis=1).astype(out_ref.dtype)

    def c_body(it, carry):
        nx = it + PRE_IT
        for t in range(4):
            low_c(it, t).wait()

            @pl.when(nx < 32)
            def _():
                high_wq(nx * 4 + t).start(priority=HI)

            @pl.when(jnp.logical_and(nx >= 32, nx < C_ITERS))
            def _():
                high_3d(wbq_hbm, wbq_buf, (nx % 32) * 4 + t, 4, 1).start(priority=HI)

            @pl.when(nx < C_ITERS)
            def _():
                low_c(nx, t).start(priority=LO)

            @pl.when(nx >= C_ITERS)
            def _():
                high_3d(wuk_hbm, wuk_buf, (nx % C_ITERS) * 4 + t, 2, 2).start(priority=HI)
                low_kv(k_hbm, nx % C_ITERS, t).start(priority=LO)

        @pl.when(it == 32)
        def _():
            wait_all(wq_buf, 0)

        @pl.when(jnp.logical_and(it >= 32, it < 48))
        def _():
            qa_item(it % 16)
        return carry

    lax.fori_loop(0, C_ITERS, c_body, 0)

    def a_body(i, carry):
        g = i // 16
        r = i % 16
        hg = g // 4
        b = g % 4
        nx = i + PRE_IT

        def tick(t):
            low_kv(k_hbm, i, t).wait()
            start_high_a(nx, t)

            @pl.when(nx < A_ITERS)
            def _():
                start_low_kv(nx, t)

        tick(0)
        tick(1)

        @pl.when(g == 0)
        def _():
            @pl.when(r == 0)
            def _():
                wait_all(wbq_buf, 1)
            expand_proj(xb32_ref[r % 4], wbq_buf, r // 4, r % 4, qb_ref)

        @pl.when(g == 4)
        def _():
            @pl.when(r == 0)
            def _():
                wait_all(wuk_buf, 2)
            qabs_item(r // 4, r % 4)

        @pl.when(jnp.logical_and(g >= 5, g < 13))
        def _():
            @pl.when(g % 2 == 1)
            def _():
                score_item((g - 5) // 2, r)

            @pl.when(g % 2 == 0)
            def _():
                pv_item((g - 5) // 2, r)

        @pl.when(g == 13)
        def _():
            @pl.when(r == 0)
            def _():
                wait_all(wuv_buf, 3)
            c32 = jnp.concatenate([cc_ref[r % 4, bb, r // 4] for bb in range(4)], axis=0)
            expand_proj(c32, wuv_buf, r // 4, r % 4, ctx_ref)

        @pl.when(g == 14)
        def _():
            @pl.when(r == 0)
            def _():
                wait_all(wbo_buf, 4)
            out_item(ctx_ref[r // 4], wbo_buf, r // 4, r % 4, accb_ref)

        @pl.when(g == 15)
        def _():
            @pl.when(r == 0)
            def _():
                for q in range(3):
                    wait_all(wo_buf.at[pl.ds(q * 1024, 1024), :], 5 + q)

            @pl.when(r < 12)
            def _():
                out_item(oa_ref[r // 4], wo_buf, r // 4, r % 4, acca_ref)

            @pl.when(r == 12)
            def _():
                out_ref[:, 512:] = finish(accb_ref[...])

        tick(2)
        tick(3)

        @pl.when(r < 8)
        def _():
            q = qa_ref[hg, pl.ds(pl.multiple_of(b * 8, 8), 8), :].astype(BF16)
            row = pl.multiple_of(r * 128, 128)
            s = jnp.zeros((8, 128), F32)
            for j in range(8):
                sj = _dot_nt(q, kvbuf[0, j, pl.ds(row, 128), :])
                s = jnp.where(row8 == j, sj, s)
            sa_ref[r] = s

        @pl.when(r == 7)
        def _():
            s = sa_ref[...]
            m = jnp.max(jnp.max(s, axis=0), axis=1, keepdims=True)
            p = jnp.exp((s - m[None]) * scale)
            pa_ref[...] = p
            l = jnp.sum(jnp.sum(p, axis=0), axis=1, keepdims=True)
            linv_ref[...] = jnp.broadcast_to(1.0 / l, (8, 128))
            oacc_ref[...] = jnp.zeros((8, 128), F32)

        @pl.when(r >= 8)
        def _():
            rr = r % 8
            p = pa_ref[rr].astype(BF16)
            row = pl.multiple_of(rr * 128, 128)
            o = jnp.zeros((8, 128), F32)
            for j in range(8):
                oj = _dot(p, kvbuf[1, j, pl.ds(row, 128), :])
                o = jnp.where(row8 == j, oj, o)
            o = oacc_ref[...] + o
            oacc_ref[...] = o
            oa_ref[hg, pl.ds(pl.multiple_of(b * 8, 8), 8), :] = o * linv_ref[...]
        return carry

    lax.fori_loop(0, A_ITERS, a_body, 0)

    wait_all(wo_buf.at[pl.ds(3072, 1024), :], 8)
    o32 = oa_ref[3]
    lhs = jnp.concatenate(
        [jnp.where(row32 == j, o32, 0.0).astype(BF16) for j in range(8)], axis=1)
    acc = acca_ref[...] + _dot(lhs, wo_buf[3072:4096, :])
    out_ref[:, :512] = finish(acc)


@jax.jit
def pallas_concat_heads__sliding_block_cached__compressed_kv_cla__decode_kernel(
    A_x: jax.Array,
    A_k_cache: jax.Array,
    A_v_cache: jax.Array,
    A_wq: jax.Array,
    A_wo: jax.Array,
    B_x: jax.Array,
    B_c_kv: jax.Array,
    B_w_q: jax.Array,
    B_w_uk: jax.Array,
    B_w_uv: jax.Array,
    B_w_o: jax.Array,
):
    B, Sq, D = A_x.shape
    _, H, Sk, Dh = A_k_cache.shape
    W = min(4096, max(256, Sk // 4))
    assert (B, Sq, D, H, Sk, Dh, W) == (4, 1, 512, 32, 4096, 128, 1024)
    assert B_c_kv.shape == (4, 4096, 512) and B_w_q.shape == (512, 32, 128)

    def body(*refs):
        _kernel(*refs, win_off=Sk - W, scale=float(Dh) ** -0.5)

    vm = pltpu.VMEM
    scratch = [
        vm((2, 8, 1024, 128), BF16),
        vm((16, 1024, 512), BF16),
        vm((512, 4096), BF16),
        vm((4096, 512), BF16),
        vm((512, 4, 8, 128), BF16),
        vm((512, 4, 8, 128), BF16),
        vm((512, 4, 8, 128), BF16),
        vm((4096, 512), BF16),
        vm((4, 512), BF16),
        vm((4, 512), BF16),
        vm((128, 1024), BF16),
        vm((32, 512), F32),
        vm((4, 32, 128), F32),
        vm((4, 32, 128), F32),
        vm((8, 8, 128), F32),
        vm((8, 8, 128), F32),
        vm((8, 128), F32),
        vm((8, 128), F32),
        vm((4, 32, 128), F32),
        vm((4, 32, 128), F32),
        vm((4, 4, 4, 8, 128), F32),
        vm((16, 32, 256), F32),
        vm((32, 128), F32),
        vm((32, 128), F32),
        vm((32, 512), F32),
        vm((4, 4, 4, 8, 128), F32),
        vm((4, 32, 128), F32),
        vm((32, 512), F32),
        vm((32, 512), F32),
        pltpu.SemaphoreType.DMA((NS,)),
        pltpu.SemaphoreType.DMA((9,)),
        pltpu.SemaphoreType.DMA((2,)),
    ]
    out = pl.pallas_call(
        body,
        out_shape=jax.ShapeDtypeStruct((B, 2 * D), A_x.dtype),
        in_specs=[pl.BlockSpec(memory_space=pl.ANY)] * 11,
        scratch_shapes=scratch,
        compiler_params=pltpu.CompilerParams(
            vmem_limit_bytes=64 * 1024 * 1024,
            disable_bounds_checks=True,
            disable_semaphore_checks=True,
        ),
    )(
        A_x.reshape(B, D),
        A_k_cache.reshape(B * H, Sk, Dh),
        A_v_cache.reshape(B * H, Sk, Dh),
        A_wq,
        A_wo,
        B_x.reshape(B, D),
        B_c_kv.reshape(16, 1024, 512),
        B_w_q.reshape(512, 4, 8, 128),
        B_w_uk.reshape(512, 4, 8, 128),
        B_w_uv.reshape(512, 4, 8, 128),
        B_w_o.reshape(4096, 512),
    )
    return out.reshape(B, Sq, 2 * D)
```

```python
import jax
import jax.numpy as jnp
from jax import lax
import jax.experimental.pallas as pl
import jax.experimental.pallas.tpu as pltpu

F32 = jnp.float32
BF16 = jnp.bfloat16
_NT = (((1,), (1,)), ((), ()))
_NN = (((1,), (0,)), ((), ()))

LO, HI = 1, 0
NS = 16
N_MAIN = 120

S_WQ, S_WBQ, S_WUK, S_WUV, S_WBO, S_WO = 0, 1, 2, 3, 4, 5


def _dot(a, b):
    return lax.dot_general(a, b, _NN, preferred_element_type=F32)


def _dot_nt(a, b):
    return lax.dot_general(a, b, _NT, preferred_element_type=F32)


def _mo(x, m):
    return x if isinstance(x, int) else pl.multiple_of(x, m)


def _kernel(xa_hbm, k_hbm, v_hbm, wq_hbm, wo_hbm, xb_hbm, c_hbm, wbq_hbm, wuk_hbm,
            wuv_hbm, wbo_hbm, out_ref,
            kbuf, vbuf, cbuf, wq_buf, wo_buf, wbq_buf, wuk_buf, wuv_buf, wbo_buf,
            xa_buf, xb_buf, e0_ref, xa32_ref, xexp_ref,
            qa_ref, sa_ref, pa_ref, psum_ref, oacc_ref, oa_ref,
            qb_ref, qabs_ref, sb_ref, mb_ref, lb_ref, cacc_ref, cc_ref, ctx_ref,
            acca_ref, accb_ref,
            lsem, hsem, xsem, *, win_off, scale):

    def low_c(pair, it, t, sem):
        row = _mo(it * 32 + t * 8, 8)
        return pltpu.make_async_copy(
            c_hbm.at[pl.ds(pair * 8, 8), pl.ds(row, 8), :],
            cbuf.at[pl.ds(pair * 8, 8), pl.ds(row, 8), :],
            lsem.at[sem])

    def head_of(g):
        return (g & 3) * 32 + (g >> 2) * 8

    def low_kv(src, dst, head, r, t, sem):
        row = _mo(r * 128 + t * 32, 32)
        return pltpu.make_async_copy(
            src.at[pl.ds(head, 8), pl.ds(_mo(win_off + row, 32), 32), :],
            dst.at[:, pl.ds(row, 32), :],
            lsem.at[sem])

    def high_wq(it, t):
        row = _mo(it * 16 + (t >> 1) * 8, 8)
        col = (t & 1) * 2048
        return pltpu.make_async_copy(
            wq_hbm.at[pl.ds(row, 8), pl.ds(col, 2048)],
            wq_buf.at[pl.ds(row, 8), pl.ds(col, 2048)], hsem.at[S_WQ])

    def high_3d(src, dst, row, rows, sem):
        return pltpu.make_async_copy(
            src.at[pl.ds(row, rows)], dst.at[pl.ds(row, rows)], hsem.at[sem])

    def high_2d(src, dst, row, rows, sem):
        row = _mo(row, 8)
        return pltpu.make_async_copy(
            src.at[pl.ds(row, rows), :], dst.at[pl.ds(row, rows), :], hsem.at[sem])

    def wait_all(buf, sem):
        pltpu.make_async_copy(buf, buf, hsem.at[sem]).wait()

    for t in range(4):
        low_kv(k_hbm, kbuf, 0, 0, t, t).start(priority=LO)
    cp_xa = pltpu.make_async_copy(xa_hbm, xa_buf, xsem.at[0])
    cp_xb = pltpu.make_async_copy(xb_hbm, xb_buf, xsem.at[1])
    cp_xa.start(priority=HI)
    cp_xb.start(priority=HI)
    high_2d(wo_hbm, wo_buf, 0, 128, S_WO).start(priority=HI)
    for r in range(1, 4):
        for t in range(4):
            low_kv(k_hbm, kbuf, 0, r, t, r * 4 + t).start(priority=LO)

    row8 = lax.broadcasted_iota(jnp.int32, (8, 128), 0)
    row32 = lax.broadcasted_iota(jnp.int32, (32, 128), 0) & 7
    lane32 = lax.broadcasted_iota(jnp.int32, (32, 128), 1) & 7

    def e0_body(i, c):
        r0 = pl.multiple_of(i * 16, 16)
        rr = lax.broadcasted_iota(jnp.int32, (16, 1024), 0) + r0
        cc = lax.broadcasted_iota(jnp.int32, (16, 1024), 1) >> 3
        e0_ref[pl.ds(r0, 16), :] = jnp.where(rr == cc, 1.0, 0.0).astype(BF16)
        return c
    lax.fori_loop(0, 8, e0_body, 0)

    qa_ref[...] = jnp.zeros(qa_ref.shape, F32)
    qb_ref[...] = jnp.zeros(qb_ref.shape, F32)
    ctx_ref[...] = jnp.zeros(ctx_ref.shape, F32)
    acca_ref[...] = jnp.zeros(acca_ref.shape, F32)
    accb_ref[...] = jnp.zeros(accb_ref.shape, F32)
    mb_ref[...] = jnp.zeros(mb_ref.shape, F32)

    def expand(c32):
        ce = _dot(c32.astype(BF16), e0_ref[...])
        return jnp.concatenate(
            [jnp.where(row32 == lane32, ce[:, 128 * k:128 * k + 128], 0.0).astype(BF16)
             for k in range(8)], axis=1)

    def x_prep():
        cp_xa.wait()
        cp_xb.wait()
        xa = xa_buf[...].astype(F32)
        xb = xb_buf[...].astype(F32)
        xa32_ref[...] = jnp.concatenate(
            [jnp.broadcast_to(xa[b:b + 1, :], (8, 512)) for b in range(4)], axis=0).astype(BF16)
        xb32 = jnp.concatenate(
            [jnp.broadcast_to(xb[b:b + 1, :], (8, 512)) for b in range(4)], axis=0)
        for u in range(4):
            xexp_ref[u >> 1, :, (u & 1) * 1024:(u & 1) * 1024 + 1024] = expand(
                xb32[:, 128 * u:128 * u + 128])

    def qa_item(n):
        hg = n >> 2
        col = pl.multiple_of(n * 256, 256)
        r = _dot(xa32_ref[...], wq_buf[:, pl.ds(col, 256)])
        j0 = (n & 3) * 2
        new = jnp.where(row32 == j0, r[:, :128], qa_ref[hg])
        new = jnp.where(row32 == j0 + 1, r[:, 128:], new)
        qa_ref[hg] = new

    def qb_item(n):
        hg = n >> 1
        half = n & 1
        w = wbq_buf[pl.ds(half * 256, 256), hg].reshape(2048, 128)
        qb_ref[hg] = qb_ref[hg] + _dot(xexp_ref[half], w)

    def qabs_item(n):
        hg = n >> 2
        u = n & 3
        q = qb_ref[hg].astype(BF16)
        w = wuk_buf[pl.ds(u * 128, 128), hg].reshape(1024, 128)
        r = _dot_nt(q, w)
        r = jnp.concatenate(
            [jnp.where(row32 == lane32, r[:, 128 * k:128 * k + 128], 0.0).astype(BF16)
             for k in range(8)], axis=1)
        qa = _dot_nt(r, e0_ref[...])
        for b in range(4):
            qabs_ref[u, b, hg] = qa[8 * b:8 * b + 8, :]

    def score_item(b, n):
        qa = jnp.concatenate(
            [qabs_ref[u, b].reshape(32, 128).astype(BF16) for u in range(4)], axis=1)
        row = pl.multiple_of((n & 1) * 512, 512)
        c = cbuf[b * 4 + (n >> 1), pl.ds(row, 512), :]
        s = _dot_nt(qa, c)
        sb_ref[n] = s
        m = jnp.maximum(jnp.maximum(s[:, :128], s[:, 128:256]),
                        jnp.maximum(s[:, 256:384], s[:, 384:]))
        mb_ref[...] = jnp.maximum(m, jnp.where(n == 0, -jnp.inf, mb_ref[...]))

    def pv_item(b, n):
        s = sb_ref[n]
        m = jnp.max(mb_ref[...], axis=1, keepdims=True)
        p = jnp.exp((s - m) * scale)
        lsum = (p[:, :128] + p[:, 128:256]) + (p[:, 256:384] + p[:, 384:])
        row = pl.multiple_of((n & 1) * 512, 512)
        c = cbuf[b * 4 + (n >> 1), pl.ds(row, 512), :]
        acc = _dot(p.astype(BF16), c)

        @pl.when(n == 0)
        def _():
            lb_ref[...] = lsum
            cacc_ref[...] = acc

        @pl.when(n > 0)
        def _():
            lb_ref[...] = lb_ref[...] + lsum
            cacc_ref[...] = cacc_ref[...] + acc

        @pl.when(n == 7)
        def _():
            inv = 1.0 / jnp.sum(lb_ref[...], axis=1, keepdims=True)
            res = cacc_ref[...] * inv
            for u in range(4):
                cc_ref[u, b] = res[:, 128 * u:128 * u + 128].reshape(4, 8, 128)

    def ctx_item(n):
        hg = n >> 2
        u = n & 3
        c32 = jnp.concatenate([cc_ref[u, bb, hg] for bb in range(4)], axis=0)
        w = wuv_buf[pl.ds(u * 128, 128), hg].reshape(1024, 128)
        ctx_ref[hg] = ctx_ref[hg] + _dot(expand(c32), w)

    def out_item(o_ref, w_buf, n, acc_ref):
        o32 = o_ref[n >> 1]
        j0 = (n & 1) * 4
        lhs = jnp.concatenate(
            [jnp.where(row32 == j0 + j, o32, 0.0).astype(BF16) for j in range(4)], axis=1)
        row = pl.multiple_of(n * 512, 512)
        acc_ref[...] = acc_ref[...] + _dot(lhs, w_buf[pl.ds(row, 512), :])

    def finish(acc):
        return jnp.sum(acc.reshape(4, 8, 512), axis=1).astype(out_ref.dtype)

    def k_work(g, r):
        q = qa_ref[g >> 2, pl.ds(_mo((g & 3) * 8, 8), 8), :].astype(BF16)
        row = pl.multiple_of(r * 128, 128)
        s = jnp.zeros((8, 128), F32)
        for j in range(8):
            sj = _dot_nt(q, kbuf[j, pl.ds(row, 128), :])
            s = jnp.where(row8 == j, sj, s)
        sa_ref[r] = s

    def v_work(r):
        p = pa_ref[r].astype(BF16)
        row = pl.multiple_of(r * 128, 128)
        o = jnp.zeros((8, 128), F32)
        for j in range(8):
            oj = _dot(p, vbuf[j, pl.ds(row, 128), :])
            o = jnp.where(row8 == j, oj, o)
        oacc_ref[...] = oacc_ref[...] + o

    def finalize_o(g):
        l = jnp.sum(psum_ref[...], axis=1, keepdims=True)
        oa_ref[g >> 2, pl.ds(_mo((g & 3) * 8, 8), 8), :] = oacc_ref[...] * (1.0 / l)

    def softmax_a():
        s = sa_ref[...]
        m = jnp.max(jnp.max(s, axis=0), axis=1, keepdims=True)
        p = jnp.exp((s - m[None]) * scale)
        pa_ref[...] = p
        psum_ref[...] = jnp.sum(p, axis=0)
        oacc_ref[...] = jnp.zeros((8, 128), F32)

    def k0a_body(r, carry):
        for t in range(4):
            low_kv(k_hbm, kbuf, 0, r, t, r * 4 + t).wait()
            high_2d(wo_hbm, wo_buf, 128 + r * 32 + t * 8, 8, S_WO).start(priority=HI)
            low_kv(k_hbm, kbuf, 0, r + 4, t, r * 4 + t).start(priority=LO)
        return carry
    lax.fori_loop(0, 4, k0a_body, 0)

    x_prep()

    def k0b_body(r, carry):
        for t in range(4):
            low_kv(k_hbm, kbuf, 0, r + 4, t, r * 4 + t).wait()
            high_2d(wo_hbm, wo_buf, 256 + r * 32 + t * 8, 8, S_WO).start(priority=HI)
            low_c(0, r, t, r * 4 + t).start(priority=LO)
        return carry
    lax.fori_loop(0, 4, k0b_body, 0)

    def c0_body(it, carry):
        nx = it + 4
        s0 = (it & 3) * 4
        for t in range(4):
            low_c(0, it, t, s0 + t).wait()
            high_wq(it, t).start(priority=HI)
            high_3d(wbq_hbm, wbq_buf, it * 8 + t * 2, 2, S_WBQ).start(priority=HI)
            low_c(nx >> 5, nx & 31, t, s0 + t).start(priority=LO)
        return carry
    lax.fori_loop(0, 32, c0_body, 0)

    def c1_tick(it, t, s0):
        low_c(1, it, t, s0 + t).wait()
        high_3d(wuk_hbm, wuk_buf, it * 16 + t * 4, 4, S_WUK).start(priority=HI)
        high_3d(wbq_hbm, wbq_buf, 256 + it * 8 + t * 2, 2, S_WBQ).start(priority=HI)

    def c1_body(it, carry):
        s0 = (it & 3) * 4
        for t in range(4):
            c1_tick(it, t, s0)
            low_c(1, it + 4, t, s0 + t).start(priority=LO)

        @pl.when(it == 2)
        def _():
            wait_all(wq_buf, S_WQ)

        @pl.when(jnp.logical_and(it >= 2, it < 18))
        def _():
            qa_item(it - 2)

        @pl.when(jnp.logical_and(it >= 18, it < 26))
        def _():
            k_work(0, it - 18)

        @pl.when(it == 26)
        def _():
            softmax_a()
        return carry
    lax.fori_loop(0, 28, c1_body, 0)

    for it in range(28, 32):
        s0 = (it & 3) * 4
        for t in range(4):
            c1_tick(it, t, s0)
            if it & 1 == 0:
                low_kv(k_hbm, kbuf, head_of(1), (it - 28) >> 1, t, s0 + t).start(priority=LO)
            else:
                low_kv(v_hbm, vbuf, head_of(0), (it - 28) >> 1, t, s0 + t).start(priority=LO)

    def make_main(high, hook, last):
        def body(i, carry):
            g = i >> 3
            r = i & 7
            i2 = i + 2
            g2 = i2 >> 3
            r2 = i2 & 7
            hk = head_of(g2 + 1)
            hv = head_of(g2)
            s0 = (i & 1) * 8
            if last:
                more = i2 < N_MAIN
                rv = jnp.where(more, r2, 2 * r2 + 1)
            else:
                rv = r2

            def tick(t):
                if t < 4:
                    low_kv(k_hbm, kbuf, 0, r, t, s0 + t).wait()
                else:
                    low_kv(v_hbm, vbuf, 0, r, t - 4, s0 + t).wait()
                high(i, t).start(priority=HI)
                if t >= 4:
                    low_kv(v_hbm, vbuf, hv, rv, t - 4, s0 + t).start(priority=LO)
                elif not last:
                    low_kv(k_hbm, kbuf, hk, r2, t, s0 + t).start(priority=LO)
                else:
                    @pl.when(more)
                    def _():
                        low_kv(k_hbm, kbuf, hk, r2, t, s0 + t).start(priority=LO)

                    @pl.when(jnp.logical_not(more))
                    def _():
                        low_kv(v_hbm, vbuf, hv, 2 * r2, t, s0 + t).start(priority=LO)

            tick(0)
            tick(1)

            @pl.when(jnp.logical_and(r == 0, i > 0))
            def _():
                finalize_o(g - 1)
                softmax_a()

            tick(2)
            tick(3)
            hook(i)
            for t in range(4, 8):
                tick(t)
            k_work(g + 1, r)
            v_work(r)
            return carry
        return body

    def attn_b_hook(n):
        @pl.when((n & 8) == 0)
        def _():
            score_item(n >> 4, n & 7)

        @pl.when((n & 8) != 0)
        def _():
            pv_item(n >> 4, n & 7)

    def hook0(i):
        @pl.when(i == 1)
        def _():
            wait_all(wbq_buf, S_WBQ)
            wait_all(wuk_buf, S_WUK)

        @pl.when(jnp.logical_and(i >= 1, i < 9))
        def _():
            qb_item(i - 1)

        @pl.when(jnp.logical_and(i >= 9, i < 25))
        def _():
            qabs_item(i - 9)

        @pl.when(i >= 25)
        def _():
            score_item(0, i - 25)

    def hook1(i):
        attn_b_hook(i - 25)

    def hook2(i):
        @pl.when(i < 89)
        def _():
            attn_b_hook(i - 25)

        @pl.when(i == 89)
        def _():
            wait_all(wuv_buf, S_WUV)
            wait_all(wbo_buf, S_WBO)

        @pl.when(jnp.logical_and(i >= 89, i < 105))
        def _():
            ctx_item(i - 89)

        @pl.when(jnp.logical_and(i >= 105, i < 113))
        def _():
            out_item(ctx_ref, wbo_buf, i - 105, accb_ref)

        @pl.when(i == 113)
        def _():
            for q in range(3):
                wait_all(wo_buf.at[pl.ds(q * 1024, 1024), :], S_WO + q)

        @pl.when(jnp.logical_and(i >= 113, i < 119))
        def _():
            out_item(oa_ref, wo_buf, i - 113, acca_ref)

        @pl.when(i == 119)
        def _():
            out_ref[:, 512:] = finish(accb_ref[...])

    def high0(i, t):
        return high_3d(wuv_hbm, wuv_buf, i * 16 + t * 2, 2, S_WUV)

    def high1(i, t):
        return high_2d(wbo_hbm, wbo_buf, (i - 32) * 128 + t * 16, 16, S_WBO)

    def high2(i, t):
        return high_2d(wo_hbm, wo_buf, (i - 58) * 64 + t * 8, 8, S_WO + ((i - 58) >> 4))

    lax.fori_loop(0, 32, make_main(high0, hook0, False), 0)
    lax.fori_loop(32, 64, make_main(high1, hook1, False), 0)
    lax.fori_loop(64, N_MAIN, make_main(high2, hook2, True), 0)

    finalize_o(14)
    softmax_a()

    def v15_body(r, carry):
        s0 = (r & 3) * 4
        for t in range(4):
            low_kv(v_hbm, vbuf, 0, r, t, s0 + t).wait()

            @pl.when(r < 4)
            def _():
                high_2d(wo_hbm, wo_buf, 3968 + r * 32 + t * 8, 8, S_WO + 3).start(priority=HI)
                low_kv(v_hbm, vbuf, head_of(15), r + 4, t, s0 + t).start(priority=LO)
        v_work(r)
        return carry
    lax.fori_loop(0, 8, v15_body, 0)

    wait_all(wo_buf.at[pl.ds(3072, 1024), :], S_WO + 3)
    finalize_o(15)
    o32 = oa_ref[3]
    lhs = jnp.concatenate(
        [jnp.where(row32 == j, o32, 0.0).astype(BF16) for j in range(8)], axis=1)
    acc = acca_ref[...] + _dot(lhs, wo_buf[3072:4096, :])
    out_ref[:, :512] = finish(acc)


@jax.jit
def pallas_concat_heads__sliding_block_cached__compressed_kv_cla__decode_kernel(
    A_x: jax.Array,
    A_k_cache: jax.Array,
    A_v_cache: jax.Array,
    A_wq: jax.Array,
    A_wo: jax.Array,
    B_x: jax.Array,
    B_c_kv: jax.Array,
    B_w_q: jax.Array,
    B_w_uk: jax.Array,
    B_w_uv: jax.Array,
    B_w_o: jax.Array,
):
    B, Sq, D = A_x.shape
    _, H, Sk, Dh = A_k_cache.shape
    W = min(4096, max(256, Sk // 4))
    assert (B, Sq, D, H, Sk, Dh, W) == (4, 1, 512, 32, 4096, 128, 1024)
    assert B_c_kv.shape == (4, 4096, 512) and B_w_q.shape == (512, 32, 128)

    def body(*refs):
        _kernel(*refs, win_off=Sk - W, scale=float(Dh) ** -0.5)

    vm = pltpu.VMEM
    scratch = [
        vm((8, 1024, 128), BF16),
        vm((8, 1024, 128), BF16),
        vm((16, 1024, 512), BF16),
        vm((512, 4096), BF16),
        vm((4096, 512), BF16),
        vm((512, 4, 8, 128), BF16),
        vm((512, 4, 8, 128), BF16),
        vm((512, 4, 8, 128), BF16),
        vm((4096, 512), BF16),
        vm((4, 512), BF16),
        vm((4, 512), BF16),
        vm((128, 1024), BF16),
        vm((32, 512), BF16),
        vm((2, 32, 2048), BF16),
        vm((4, 32, 128), F32),
        vm((8, 8, 128), F32),
        vm((8, 8, 128), F32),
        vm((8, 128), F32),
        vm((8, 128), F32),
        vm((4, 32, 128), F32),
        vm((4, 32, 128), F32),
        vm((4, 4, 4, 8, 128), F32),
        vm((8, 32, 512), F32),
        vm((32, 128), F32),
        vm((32, 128), F32),
        vm((32, 512), F32),
        vm((4, 4, 4, 8, 128), F32),
        vm((4, 32, 128), F32),
        vm((32, 512), F32),
        vm((32, 512), F32),
        pltpu.SemaphoreType.DMA((NS,)),
        pltpu.SemaphoreType.DMA((9,)),
        pltpu.SemaphoreType.DMA((2,)),
    ]
    out = pl.pallas_call(
        body,
        out_shape=jax.ShapeDtypeStruct((B, 2 * D), A_x.dtype),
        in_specs=[pl.BlockSpec(memory_space=pl.ANY)] * 11,
        scratch_shapes=scratch,
        compiler_params=pltpu.CompilerParams(
            vmem_limit_bytes=64 * 1024 * 1024,
            disable_bounds_checks=True,
            disable_semaphore_checks=True,
        ),
    )(
        A_x.reshape(B, D),
        A_k_cache.reshape(B * H, Sk, Dh),
        A_v_cache.reshape(B * H, Sk, Dh),
        A_wq,
        A_wo,
        B_x.reshape(B, D),
        B_c_kv.reshape(16, 1024, 512),
        B_w_q.reshape(512, 4, 8, 128),
        B_w_uk.reshape(512, 4, 8, 128),
        B_w_uv.reshape(512, 4, 8, 128),
        B_w_o.reshape(4096, 512),
    )
    return out.reshape(B, Sq, 2 * D)
```

```python
import jax
import jax.numpy as jnp
from jax import lax
import jax.experimental.pallas as pl
import jax.experimental.pallas.tpu as pltpu

F32 = jnp.float32
BF16 = jnp.bfloat16
_NT = (((1,), (1,)), ((), ()))
_NN = (((1,), (0,)), ((), ()))

LO, HI = 1, 0
NS = 16
N_MAIN = 120
FLOAT_HOOK = True
PIN = False

S_WQ = 0
S_WBQ = 4
S_WUK = 5
S_WUV = 6
S_WBO = 7
S_WO = 8
N_HSEM = 11


def _dot(a, b):
    return lax.dot_general(a, b, _NN, preferred_element_type=F32)


def _dot_nt(a, b):
    return lax.dot_general(a, b, _NT, preferred_element_type=F32)


def _mo(x, m):
    return x if isinstance(x, int) else pl.multiple_of(x, m)


def _nop(_=None):
    return None


def _kernel(xa_hbm, k_hbm, v_hbm, wq_hbm, wo_hbm, xb_hbm, c_hbm, wbq_hbm, wuk_hbm,
            wuv_hbm, wbo_hbm, out_ref,
            kbuf, vbuf, cbuf, wq_buf, wo_buf, wbq_buf, wuk_buf, wuv_buf, wbo_buf,
            xa_buf, xb_buf, e0_ref, xa32_ref, xexp_ref,
            qa_ref, sa_ref, pa_ref, psum_ref, oacc_ref, oa_ref,
            qb_ref, qabs_ref, sb_ref, mb_ref, lb_ref, cacc_ref, cc_ref, ctx_ref,
            acca_ref, accb_ref,
            lsem, hsem, xsem, *, win_off, scale):

    def low_c(pair, it, t, sem):
        row = _mo(it * 32 + t * 8, 8)
        return pltpu.make_async_copy(
            c_hbm.at[pl.ds(pair * 8, 8), pl.ds(row, 8), :],
            cbuf.at[pl.ds(pair * 8, 8), pl.ds(row, 8), :],
            lsem.at[sem])

    def head_of(g):
        return (g & 3) * 32 + (g >> 2) * 8

    def low_kv(src, dst, head, r, t, sem):
        row = _mo(r * 128 + t * 32, 32)
        return pltpu.make_async_copy(
            src.at[pl.ds(head, 8), pl.ds(_mo(win_off + row, 32), 32), :],
            dst.at[:, pl.ds(row, 32), :],
            lsem.at[sem])

    def low_wo(n, sem):
        row = _mo(512 + n * 64, 64)
        return pltpu.make_async_copy(
            wo_hbm.at[3, pl.ds(row, 64), :], wo_buf.at[3, pl.ds(row, 64), :], lsem.at[sem])

    def high_wq(hg, row, col, cols):
        row = _mo(row, 8)
        return pltpu.make_async_copy(
            wq_hbm.at[:, pl.ds(row, 8), pl.ds(_mo(hg * 1024 + col, 128), cols)],
            wq_buf.at[hg, :, pl.ds(row, 8), pl.ds(col, cols)], hsem.at[S_WQ + hg])

    def high_3d(src, dst, row, hg, nhg, sem):
        return pltpu.make_async_copy(
            src.at[:, row, pl.ds(hg, nhg)], dst.at[pl.ds(0, 4), row, pl.ds(hg, nhg)], hsem.at[sem])

    def high_2d(src, dst, nq, row, col, sem):
        row = _mo(row, 8)
        return pltpu.make_async_copy(
            src.at[pl.ds(0, nq), pl.ds(row, 8), pl.ds(col, 256)],
            dst.at[pl.ds(0, nq), pl.ds(row, 8), pl.ds(col, 256)], hsem.at[sem])

    def wait_all(buf, sem):
        pltpu.make_async_copy(buf, buf, hsem.at[sem]).wait()

    for r in range(4):
        for t in range(4):
            low_kv(k_hbm, kbuf, 0, r, t, r * 4 + t).start(priority=LO)
    cp_xa = pltpu.make_async_copy(xa_hbm, xa_buf, xsem.at[0])
    cp_xb = pltpu.make_async_copy(xb_hbm, xb_buf, xsem.at[1])
    cp_xa.start(priority=HI)
    cp_xb.start(priority=HI)

    row8 = lax.broadcasted_iota(jnp.int32, (8, 128), 0)
    row32 = lax.broadcasted_iota(jnp.int32, (32, 128), 0) & 7
    lane32 = lax.broadcasted_iota(jnp.int32, (32, 128), 1) & 7

    def e0_body(i, c):
        r0 = pl.multiple_of(i * 16, 16)
        rr = lax.broadcasted_iota(jnp.int32, (16, 1024), 0) + r0
        cc = lax.broadcasted_iota(jnp.int32, (16, 1024), 1) >> 3
        e0_ref[pl.ds(r0, 16), :] = jnp.where(rr == cc, 1.0, 0.0).astype(BF16)
        return c
    lax.fori_loop(0, 8, e0_body, 0)

    qa_ref[...] = jnp.zeros(qa_ref.shape, F32)
    qb_ref[...] = jnp.zeros(qb_ref.shape, F32)
    ctx_ref[...] = jnp.zeros(ctx_ref.shape, F32)
    acca_ref[...] = jnp.zeros(acca_ref.shape, F32)
    accb_ref[...] = jnp.zeros(accb_ref.shape, F32)
    mb_ref[...] = jnp.zeros(mb_ref.shape, F32)
    lb_ref[...] = jnp.zeros(lb_ref.shape, F32)
    cacc_ref[...] = jnp.zeros(cacc_ref.shape, F32)

    def expand(c32, fl=_nop):
        ce = _dot(c32.astype(BF16), e0_ref[...])
        fl(ce)
        return jnp.concatenate(
            [jnp.where(row32 == lane32, ce[:, 128 * k:128 * k + 128], 0.0).astype(BF16)
             for k in range(8)], axis=1)

    def x_prep():
        cp_xa.wait()
        cp_xb.wait()
        xa = xa_buf[...].astype(F32)
        xb = xb_buf[...].astype(F32)
        xa32_ref[...] = jnp.concatenate(
            [jnp.broadcast_to(xa[b:b + 1, :], (8, 512)) for b in range(4)], axis=0).astype(BF16)
        xb32 = jnp.concatenate(
            [jnp.broadcast_to(xb[b:b + 1, :], (8, 512)) for b in range(4)], axis=0)
        for u in range(4):
            xexp_ref[u >> 1, :, (u & 1) * 1024:(u & 1) * 1024 + 1024] = expand(
                xb32[:, 128 * u:128 * u + 128])

    def qa_item(hg, half):
        col = pl.multiple_of(half * 512, 512)
        w = wq_buf[hg, :, :, pl.ds(col, 512)].reshape(512, 512)
        r = _dot(xa32_ref[...], w)
        new = qa_ref[hg]
        for j in range(4):
            new = jnp.where(row32 == half * 4 + j, r[:, 128 * j:128 * j + 128], new)
        qa_ref[hg] = new

    def qb_item(n):
        hg = n >> 1
        half = n & 1
        w = wbq_buf[pl.ds(half * 2, 2), :, hg].reshape(2048, 128)
        qb_ref[hg] = qb_ref[hg] + _dot(xexp_ref[half], w)

    def qabs_item(n):
        hg = n & 3
        u = n >> 2
        q = qb_ref[hg].astype(BF16)
        w = wuk_buf[u, :, hg].reshape(1024, 128)
        r = _dot_nt(q, w)
        r = jnp.concatenate(
            [jnp.where(row32 == lane32, r[:, 128 * k:128 * k + 128], 0.0).astype(BF16)
             for k in range(8)], axis=1)
        qa = _dot_nt(r, e0_ref[...])
        for b in range(4):
            qabs_ref[u, b, hg] = qa[8 * b:8 * b + 8, :]

    def score_item(b, n, fl):
        qa = jnp.concatenate(
            [qabs_ref[u, b].reshape(32, 128).astype(BF16) for u in range(4)], axis=1)
        seg = b * 4 + (n >> 1)
        m = jnp.where(n == 0, -jnp.inf, mb_ref[...])
        for k in range(4):
            row = pl.multiple_of((n & 1) * 512 + k * 128, 128)
            s = _dot_nt(qa, cbuf[seg, pl.ds(row, 128), :])
            if k == 0:
                fl(s)
            sb_ref[n, :, 128 * k:128 * k + 128] = s
            m = jnp.maximum(m, s)
        mb_ref[...] = m

    def max_b():
        mb_ref[...] = jnp.broadcast_to(jnp.max(mb_ref[...], axis=1, keepdims=True), (32, 128))

    def pv_item(b, n, fl):
        m = mb_ref[...]
        ps = [jnp.exp((sb_ref[n, :, 128 * k:128 * k + 128] - m) * scale) for k in range(4)]
        first = n == 0
        lb_ref[...] = jnp.where(first, 0.0, lb_ref[...]) + ((ps[0] + ps[1]) + (ps[2] + ps[3]))
        seg = b * 4 + (n >> 1)
        acc = jnp.where(first, 0.0, cacc_ref[...])
        for k in range(4):
            row = pl.multiple_of((n & 1) * 512 + k * 128, 128)
            d = _dot(ps[k].astype(BF16), cbuf[seg, pl.ds(row, 128), :])
            if k == 0:
                fl(d)
            acc = acc + d
        cacc_ref[...] = acc

    def norm_b(b):
        inv = 1.0 / jnp.sum(lb_ref[...], axis=1, keepdims=True)
        res = cacc_ref[...] * inv
        for u in range(4):
            cc_ref[u, b] = res[:, 128 * u:128 * u + 128].reshape(4, 8, 128)

    def ctx_item(n, fl):
        hg = n >> 2
        u = n & 3
        c32 = jnp.concatenate([cc_ref[u, bb, hg] for bb in range(4)], axis=0)
        w = wuv_buf[u, :, hg].reshape(1024, 128)
        ctx_ref[hg] = ctx_ref[hg] + _dot(expand(c32, fl), w)

    def out_part(o32, w_buf, hg, j0, nj, fl=_nop):
        acc = None
        for j in range(nj):
            row = _mo((j0 + j) * 128, 128)
            d = _dot(jnp.where(row32 == j0 + j, o32, 0.0).astype(BF16),
                     w_buf[hg, pl.ds(row, 128), :])
            if j == 0:
                fl(d)
            acc = d if acc is None else acc + d
        return acc

    def out_item(o_ref, w_buf, hg, half, acc_ref, fl=_nop):
        acc_ref[...] = acc_ref[...] + out_part(o_ref[hg], w_buf, hg, half * 4, 4, fl)

    def rowsum(acc):
        return jnp.sum(acc.reshape(4, 8, 512), axis=1)

    def k_work(g, r):
        q = qa_ref[g >> 2, pl.ds(_mo((g & 3) * 8, 8), 8), :].astype(BF16)
        row = pl.multiple_of(r * 128, 128)
        s = jnp.zeros((8, 128), F32)
        for j in range(8):
            sj = _dot_nt(q, kbuf[j, pl.ds(row, 128), :])
            s = jnp.where(row8 == j, sj, s)
        sa_ref[r] = s

    def v_part(r, fl=_nop):
        p = pa_ref[r].astype(BF16)
        row = _mo(r * 128, 128)
        o = jnp.zeros((8, 128), F32)
        for j in range(8):
            oj = _dot(p, vbuf[j, pl.ds(row, 128), :])
            if j == 0:
                fl(oj)
            o = jnp.where(row8 == j, oj, o)
        return oacc_ref[...] + o

    def finalize_o(g):
        l = jnp.sum(psum_ref[...], axis=1, keepdims=True)
        oa_ref[g >> 2, pl.ds(_mo((g & 3) * 8, 8), 8), :] = oacc_ref[...] * (1.0 / l)

    def softmax_a():
        s = sa_ref[...]
        m = jnp.max(jnp.max(s, axis=0), axis=1, keepdims=True)
        p = jnp.exp((s - m[None]) * scale)
        pa_ref[...] = p
        psum_ref[...] = jnp.sum(p, axis=0)
        oacc_ref[...] = jnp.zeros((8, 128), F32)

    def k0a_body(r, carry):
        for t in range(4):
            low_kv(k_hbm, kbuf, 0, r, t, r * 4 + t).wait()
            high_wq(0, r * 16 + (t >> 1) * 8, (t & 1) * 512, 512).start(priority=HI)
            low_kv(k_hbm, kbuf, 0, r + 4, t, r * 4 + t).start(priority=LO)
        return carry
    lax.fori_loop(0, 4, k0a_body, 0)

    x_prep()

    def k0b_body(r, carry):
        for t in range(4):
            low_kv(k_hbm, kbuf, 0, r + 4, t, r * 4 + t).wait()
            high_wq(0, 64 + r * 16 + (t >> 1) * 8, (t & 1) * 512, 512).start(priority=HI)
            low_c(0, r, t, r * 4 + t).start(priority=LO)
        return carry
    lax.fori_loop(0, 4, k0b_body, 0)

    def c0_body(it, carry):
        nx = it + 4
        s0 = (it & 3) * 4
        for t in range(4):
            low_c(0, it, t, s0 + t).wait()
            high_3d(wbq_hbm, wbq_buf, it * 4 + t, 0, 4, S_WBQ).start(priority=HI)
            low_c(nx >> 5, nx & 31, t, s0 + t).start(priority=LO)

        @pl.when(it == 1)
        def _():
            wait_all(wq_buf.at[0], S_WQ)

        @pl.when(jnp.logical_and(it >= 1, it < 3))
        def _():
            qa_item(0, it - 1)

        @pl.when(jnp.logical_and(it >= 3, it < 11))
        def _():
            k_work(0, it - 3)

        @pl.when(it == 11)
        def _():
            softmax_a()
        return carry
    lax.fori_loop(0, 32, c0_body, 0)

    def c1_tick(it, t, s0):
        low_c(1, it, t, s0 + t).wait()
        high_3d(wuk_hbm, wuk_buf, it * 4 + t, 0, 4, S_WUK).start(priority=HI)

    def c1_body(it, carry):
        s0 = (it & 3) * 4
        for t in range(4):
            c1_tick(it, t, s0)
            low_c(1, it + 4, t, s0 + t).start(priority=LO)

        @pl.when(it == 1)
        def _():
            wait_all(wbq_buf, S_WBQ)

        @pl.when(jnp.logical_and(it >= 1, it < 9))
        def _():
            qb_item(it - 1)
        return carry
    lax.fori_loop(0, 28, c1_body, 0)

    for it in range(28, 32):
        s0 = (it & 3) * 4
        for t in range(4):
            c1_tick(it, t, s0)
            if it % 2 == 0:
                low_kv(k_hbm, kbuf, head_of(1), (it - 28) >> 1, t, s0 + t).start(priority=LO)
            else:
                low_kv(v_hbm, vbuf, head_of(0), (it - 28) >> 1, t, s0 + t).start(priority=LO)

    def make_main(high, pin, hook, hook_floats, extra, last):
        def body(i, carry):
            g = i >> 3
            r = i & 7
            i2 = i + 2
            g2 = i2 >> 3
            r2 = i2 & 7
            hk = head_of(g2 + 1)
            hv = head_of(g2)
            s0 = (i & 1) * 8
            if last:
                more = i2 < N_MAIN
                rv = jnp.where(more, r2, 2 * r2 + 1)
            else:
                rv = r2

            def floater(t):
                def fl(val=None):
                    if PIN and val is not None:
                        pin(val)
                    high(i, t)
                return fl

            def tick(t, with_high=True):
                if t < 4:
                    low_kv(k_hbm, kbuf, 0, r, t, s0 + t).wait()
                else:
                    low_kv(v_hbm, vbuf, 0, r, t - 4, s0 + t).wait()
                if with_high:
                    high(i, t)
                if t >= 4:
                    low_kv(v_hbm, vbuf, hv, rv, t - 4, s0 + t).start(priority=LO)
                elif not last:
                    low_kv(k_hbm, kbuf, hk, r2, t, s0 + t).start(priority=LO)
                else:
                    @pl.when(more)
                    def _():
                        low_kv(k_hbm, kbuf, hk, r2, t, s0 + t).start(priority=LO)

                    @pl.when(jnp.logical_not(more))
                    def _():
                        low_kv(v_hbm, vbuf, hv, 2 * r2, t, s0 + t).start(priority=LO)

            tick(0)
            tick(1, not PIN)

            @pl.when(jnp.logical_and(r == 0, i > 0))
            def _():
                finalize_o(g - 1)
                softmax_a()

            extra(i)
            tick(2)
            tick(3)
            hook(i, floater(5) if hook_floats else _nop)
            tick(4)
            tick(5, not hook_floats)
            tick(6)
            tick(7)
            oacc_ref[...] = v_part(r, floater(1) if PIN else _nop)
            k_work(g + 1, r)
            return carry
        return body

    def pin_to(buf_view):
        def pin(val):
            buf_view[...] = val[:8, :128].astype(BF16)
        return pin

    def high0(i, t):
        high_wq(1 + (i >> 3), (i & 7) * 16 + (t >> 2) * 8, (t & 3) * 256, 256).start(priority=HI)

    def hook0(i, fl):
        @pl.when(i == 1)
        def _():
            wait_all(wuk_buf, S_WUK)

        @pl.when(jnp.logical_and(i >= 1, i < 17))
        def _():
            qabs_item(i - 1)

        @pl.when(i == 18)
        def _():
            wait_all(wq_buf.at[1], S_WQ + 1)
            wait_all(wq_buf.at[2], S_WQ + 2)

        @pl.when(jnp.logical_and(i >= 18, i < 22))
        def _():
            qa_item((i >> 1) - 8, i & 1)

    def high1(i, t):
        @pl.when(i < 56)
        def _():
            high_3d(wuv_hbm, wuv_buf, (i - 24) * 4 + (t >> 1), (t & 1) * 2, 2, S_WUV).start(priority=HI)

        @pl.when(i >= 56)
        def _():
            high_2d(wbo_hbm, wbo_buf, 4, (i - 56) * 32 + (t >> 1) * 8, (t & 1) * 256,
                    S_WBO).start(priority=HI)

    def pin1(val):
        wuv_buf[4, 0, 0] = val[:8, :128].astype(BF16)
        wbo_buf[4, 0:8, 0:128] = val[:8, :128].astype(BF16)

    def extra1(i):
        n = i - 24

        @pl.when(i == 25)
        def _():
            wait_all(wq_buf.at[3], S_WQ + 3)

        @pl.when(jnp.logical_and(i >= 25, i < 27))
        def _():
            qa_item(3, i - 25)

        @pl.when((n & 15) == 8)
        def _():
            max_b()

        @pl.when(jnp.logical_and((n & 15) == 1, n > 16))
        def _():
            norm_b((n >> 4) - 1)

    def hook1(i, fl):
        n = i - 24

        @pl.when((n & 8) == 0)
        def _():
            score_item(n >> 4, n & 7, fl)

        @pl.when((n & 8) != 0)
        def _():
            pv_item(n >> 4, n & 7, fl)

    def high2(i, t):
        high_2d(wo_hbm, wo_buf, 3, (i - 88) * 32 + (t >> 1) * 8, (t & 1) * 256,
                S_WO + ((i - 88) >> 4)).start(priority=HI)

    def extra2(i):
        @pl.when(i == 88)
        def _():
            wait_all(wuv_buf.at[pl.ds(0, 4)], S_WUV)
            norm_b(3)

        @pl.when(i == 104)
        def _():
            wait_all(wbo_buf.at[pl.ds(0, 4)], S_WBO)

        @pl.when(i == 113)
        def _():
            wait_all(wo_buf.at[pl.ds(0, 3), pl.ds(0, 512), :], S_WO)
            out_ref[:, 512:] = rowsum(accb_ref[...]).astype(out_ref.dtype)

    def hook2(i, fl):
        @pl.when(i < 104)
        def _():
            ctx_item(i - 88, fl)

        @pl.when(jnp.logical_and(i >= 104, i < 112))
        def _():
            out_item(ctx_ref, wbo_buf, (i - 104) >> 1, i & 1, accb_ref, fl)

        @pl.when(jnp.logical_and(i >= 113, i < 116))
        def _():
            out_item(oa_ref, wo_buf, i - 113, 0, acca_ref, fl)

        @pl.when(jnp.logical_or(i == 112, i >= 116))
        def _():
            fl()

    lax.fori_loop(0, 24, make_main(high0, pin_to(wq_buf.at[4, 0, 0:8, 0:128]), hook0, False,
                                   _nop, False), 0)
    lax.fori_loop(24, 88, make_main(high1, pin1, hook1, FLOAT_HOOK, extra1, False), 0)
    lax.fori_loop(88, N_MAIN, make_main(high2, pin_to(wo_buf.at[4, 0:8, 0:128]), hook2,
                                        FLOAT_HOOK, extra2, True), 0)

    finalize_o(14)
    softmax_a()

    def v15_body(r, carry):
        s0 = (r & 3) * 4
        for t in range(4):
            low_kv(v_hbm, vbuf, 0, r, t, s0 + t).wait()

            @pl.when(r < 4)
            def _():
                row = pl.multiple_of(r * 128 + t * 32, 32)
                pltpu.make_async_copy(
                    wo_hbm.at[3, pl.ds(row, 32), :], wo_buf.at[3, pl.ds(row, 32), :],
                    hsem.at[S_WO + 2]).start(priority=HI)
                low_kv(v_hbm, vbuf, head_of(15), r + 4, t, s0 + t).start(priority=LO)

            @pl.when(jnp.logical_and(r >= 4, r < 6))
            def _():
                low_wo(s0 + t, s0 + t).start(priority=LO)

            if t == 1:
                @pl.when(r == 1)
                def _():
                    wait_all(wo_buf.at[pl.ds(0, 3), pl.ds(512, 512), :], S_WO + 1)

                @pl.when(jnp.logical_and(r >= 1, r < 4))
                def _():
                    out_item(oa_ref, wo_buf, r - 1, 1, acca_ref)

                @pl.when(r == 4)
                def _():
                    l = jnp.sum(psum_ref[...], axis=1, keepdims=True)
                    psum_ref[...] = jnp.broadcast_to(1.0 / l, (8, 128))
        oacc_ref[...] = v_part(r)
        return carry
    lax.fori_loop(0, 7, v15_body, 0)

    wait_all(wo_buf.at[3, pl.ds(0, 512), :], S_WO + 2)
    for t in range(4):
        low_kv(v_hbm, vbuf, 0, 7, t, 12 + t).wait()
    oa_ref[3, 24:32, :] = v_part(7) * psum_ref[...]
    o32 = oa_ref[3]
    acca_ref[...] = acca_ref[...] + out_part(o32, wo_buf, 3, 0, 4)
    for n in range(6):
        low_wo(n, n).wait()
    part = rowsum(acca_ref[...] + out_part(o32, wo_buf, 3, 4, 3))
    o_last = oa_ref[3, pl.ds(7, 4, stride=8), :].astype(BF16)
    for n in range(6, 8):
        low_wo(n, n).wait()
    out_ref[:, :512] = (part + _dot(o_last, wo_buf[3, 896:1024, :])).astype(out_ref.dtype)


@jax.jit
def pallas_concat_heads__sliding_block_cached__compressed_kv_cla__decode_kernel(
    A_x: jax.Array,
    A_k_cache: jax.Array,
    A_v_cache: jax.Array,
    A_wq: jax.Array,
    A_wo: jax.Array,
    B_x: jax.Array,
    B_c_kv: jax.Array,
    B_w_q: jax.Array,
    B_w_uk: jax.Array,
    B_w_uv: jax.Array,
    B_w_o: jax.Array,
):
    B, Sq, D = A_x.shape
    _, H, Sk, Dh = A_k_cache.shape
    W = min(4096, max(256, Sk // 4))
    assert (B, Sq, D, H, Sk, Dh, W) == (4, 1, 512, 32, 4096, 128, 1024)
    assert B_c_kv.shape == (4, 4096, 512) and B_w_q.shape == (512, 32, 128)

    def body(*refs):
        _kernel(*refs, win_off=Sk - W, scale=float(Dh) ** -0.5)

    vm = pltpu.VMEM
    scratch = [
        vm((8, 1024, 128), BF16),
        vm((8, 1024, 128), BF16),
        vm((16, 1024, 512), BF16),
        vm((5, 4, 128, 1024), BF16),
        vm((5, 1024, 512), BF16),
        vm((4, 128, 4, 8, 128), BF16),
        vm((4, 128, 4, 8, 128), BF16),
        vm((5, 128, 4, 8, 128), BF16),
        vm((5, 1024, 512), BF16),
        vm((4, 512), BF16),
        vm((4, 512), BF16),
        vm((128, 1024), BF16),
        vm((32, 512), BF16),
        vm((2, 32, 2048), BF16),
        vm((4, 32, 128), F32),
        vm((8, 8, 128), F32),
        vm((8, 8, 128), F32),
        vm((8, 128), F32),
        vm((8, 128), F32),
        vm((4, 32, 128), F32),
        vm((4, 32, 128), F32),
        vm((4, 4, 4, 8, 128), F32),
        vm((8, 32, 512), F32),
        vm((32, 128), F32),
        vm((32, 128), F32),
        vm((32, 512), F32),
        vm((4, 4, 4, 8, 128), F32),
        vm((4, 32, 128), F32),
        vm((32, 512), F32),
        vm((32, 512), F32),
        pltpu.SemaphoreType.DMA((NS,)),
        pltpu.SemaphoreType.DMA((N_HSEM,)),
        pltpu.SemaphoreType.DMA((2,)),
    ]
    out = pl.pallas_call(
        body,
        out_shape=jax.ShapeDtypeStruct((B, 2 * D), A_x.dtype),
        in_specs=[pl.BlockSpec(memory_space=pl.ANY)] * 11,
        scratch_shapes=scratch,
        compiler_params=pltpu.CompilerParams(
            vmem_limit_bytes=64 * 1024 * 1024,
            disable_bounds_checks=True,
            disable_semaphore_checks=True,
        ),
    )(
        A_x.reshape(B, D),
        A_k_cache.reshape(B * H, Sk, Dh),
        A_v_cache.reshape(B * H, Sk, Dh),
        A_wq.reshape(4, 128, 4096),
        A_wo.reshape(4, 1024, 512),
        B_x.reshape(B, D),
        B_c_kv.reshape(16, 1024, 512),
        B_w_q.reshape(4, 128, 4, 8, 128),
        B_w_uk.reshape(4, 128, 4, 8, 128),
        B_w_uv.reshape(4, 128, 4, 8, 128),
        B_w_o.reshape(4, 1024, 512),
    )
    return out.reshape(B, Sq, 2 * D)
```

```python
import jax
import jax.numpy as jnp
from jax import lax
import jax.experimental.pallas as pl
import jax.experimental.pallas.tpu as pltpu

F32 = jnp.float32
BF16 = jnp.bfloat16
_NT = (((1,), (1,)), ((), ()))
_NN = (((1,), (0,)), ((), ()))

LO, HI = 1, 0
NS = 16
N_MAIN = 120
FLOAT_HOOK = True
PIN = False
CMODE = 0

S_WQ = 0
S_WBQ = 4
S_WUK = 5
S_WUV = 6
S_WBO = 7
S_WO = 8
N_HSEM = 11


def _dot(a, b):
    return lax.dot_general(a, b, _NN, preferred_element_type=F32)


def _dot_nt(a, b):
    return lax.dot_general(a, b, _NT, preferred_element_type=F32)


def _mo(x, m):
    return x if isinstance(x, int) else pl.multiple_of(x, m)


def _nop(_=None):
    return None


def _kernel(xa_hbm, k_hbm, v_hbm, wq_hbm, wo_hbm, xb_hbm, c_hbm, wbq_hbm, wuk_hbm,
            wuv_hbm, wbo_hbm, out_ref,
            kvbuf, cbuf, wq_buf, wo_buf, wbq_buf, wuk_buf, wuv_buf, wbo_buf,
            xa_buf, xb_buf, e0_ref, xa32_ref, xexp_ref,
            qa_ref, sa_ref, pa_ref, psum_ref, oacc_ref, oa_ref,
            qb_ref, qabs_ref, sb_ref, mb_ref, lb_ref, cacc_ref, cc_ref, ctx_ref,
            acca_ref, accb_ref,
            lsem, hsem, xsem, *, win_off, scale):

    kbuf = kvbuf.at[0]
    vbuf = kvbuf.at[1]

    def low_c(pair, it, t, sem):
        if CMODE == 1:
            row = _mo(pair * 512 + it * 16 + (t >> 1) * 8, 8)
            col = (t & 1) * 256
            return pltpu.make_async_copy(
                c_hbm.at[:, pl.ds(row, 8), pl.ds(col, 256)],
                cbuf.at[:, pl.ds(row, 8), pl.ds(col, 256)],
                lsem.at[sem])
        row = _mo(it * 32 + t * 8, 8)
        return pltpu.make_async_copy(
            c_hbm.at[pl.ds(pair * 8, 8), pl.ds(row, 8), :],
            cbuf.at[pl.ds(pair * 8, 8), pl.ds(row, 8), :],
            lsem.at[sem])

    def head_of(g):
        return (g & 3) * 32 + (g >> 2) * 8

    def low_kv(src, dst, head, r, t, sem):
        row = _mo(r * 128 + t * 32, 32)
        return pltpu.make_async_copy(
            src.at[pl.ds(head, 8), pl.ds(_mo(win_off + row, 32), 32), :],
            dst.at[:, pl.ds(row, 32), :],
            lsem.at[sem])

    def start_pair(hk, hv, r, t, sem):
        row = _mo(r * 128 + t * 16, 16)
        for src, dst, head in ((k_hbm, kbuf, hk), (v_hbm, vbuf, hv)):
            pltpu.make_async_copy(
                src.at[pl.ds(head, 8), pl.ds(_mo(win_off + row, 16), 16), :],
                dst.at[:, pl.ds(row, 16), :],
                lsem.at[sem]).start(priority=LO)

    def wait_pair(r, t, sem):
        both = kvbuf.at[:, :, pl.ds(_mo(r * 128 + t * 16, 16), 16), :]
        pltpu.make_async_copy(both, both, lsem.at[sem]).wait()

    def low_wo(n, sem):
        row = _mo(512 + n * 64, 64)
        return pltpu.make_async_copy(
            wo_hbm.at[3, pl.ds(row, 64), :], wo_buf.at[3, pl.ds(row, 64), :], lsem.at[sem])

    def high_wq(hg, row, col, cols):
        row = _mo(row, 8)
        return pltpu.make_async_copy(
            wq_hbm.at[:, pl.ds(row, 8), pl.ds(_mo(hg * 1024 + col, 128), cols)],
            wq_buf.at[hg, :, pl.ds(row, 8), pl.ds(col, cols)], hsem.at[S_WQ + hg])

    def high_3d(src, dst, row, hg, nhg, sem):
        return pltpu.make_async_copy(
            src.at[:, row, pl.ds(hg, nhg)], dst.at[pl.ds(0, 4), row, pl.ds(hg, nhg)], hsem.at[sem])

    def high_2d(src, dst, nq, row, col, sem):
        row = _mo(row, 8)
        return pltpu.make_async_copy(
            src.at[pl.ds(0, nq), pl.ds(row, 8), pl.ds(col, 256)],
            dst.at[pl.ds(0, nq), pl.ds(row, 8), pl.ds(col, 256)], hsem.at[sem])

    def wait_all(buf, sem):
        pltpu.make_async_copy(buf, buf, hsem.at[sem]).wait()

    for r in range(4):
        for t in range(4):
            low_kv(k_hbm, kbuf, 0, r, t, r * 4 + t).start(priority=LO)
    cp_xa = pltpu.make_async_copy(xa_hbm, xa_buf, xsem.at[0])
    cp_xb = pltpu.make_async_copy(xb_hbm, xb_buf, xsem.at[1])
    cp_xa.start(priority=HI)
    cp_xb.start(priority=HI)

    row8 = lax.broadcasted_iota(jnp.int32, (8, 128), 0)
    row32 = lax.broadcasted_iota(jnp.int32, (32, 128), 0) & 7
    lane32 = lax.broadcasted_iota(jnp.int32, (32, 128), 1) & 7

    def e0_body(i, c):
        r0 = pl.multiple_of(i * 16, 16)
        rr = lax.broadcasted_iota(jnp.int32, (16, 1024), 0) + r0
        cc = lax.broadcasted_iota(jnp.int32, (16, 1024), 1) >> 3
        e0_ref[pl.ds(r0, 16), :] = jnp.where(rr == cc, 1.0, 0.0).astype(BF16)
        return c
    lax.fori_loop(0, 8, e0_body, 0)

    qa_ref[...] = jnp.zeros(qa_ref.shape, F32)
    qb_ref[...] = jnp.zeros(qb_ref.shape, F32)
    ctx_ref[...] = jnp.zeros(ctx_ref.shape, F32)
    acca_ref[...] = jnp.zeros(acca_ref.shape, F32)
    accb_ref[...] = jnp.zeros(accb_ref.shape, F32)
    mb_ref[...] = jnp.zeros(mb_ref.shape, F32)
    lb_ref[...] = jnp.zeros(lb_ref.shape, F32)
    cacc_ref[...] = jnp.zeros(cacc_ref.shape, F32)

    def expand(c32, fl=_nop):
        ce = _dot(c32.astype(BF16), e0_ref[...])
        fl(ce)
        return jnp.concatenate(
            [jnp.where(row32 == lane32, ce[:, 128 * k:128 * k + 128], 0.0).astype(BF16)
             for k in range(8)], axis=1)

    def x_prep():
        cp_xa.wait()
        cp_xb.wait()
        xa = xa_buf[...].astype(F32)
        xb = xb_buf[...].astype(F32)
        xa32_ref[...] = jnp.concatenate(
            [jnp.broadcast_to(xa[b:b + 1, :], (8, 512)) for b in range(4)], axis=0).astype(BF16)
        xb32 = jnp.concatenate(
            [jnp.broadcast_to(xb[b:b + 1, :], (8, 512)) for b in range(4)], axis=0)
        for u in range(4):
            xexp_ref[u >> 1, :, (u & 1) * 1024:(u & 1) * 1024 + 1024] = expand(
                xb32[:, 128 * u:128 * u + 128])

    def qa_item(hg, half):
        col = pl.multiple_of(half * 512, 512)
        w = wq_buf[hg, :, :, pl.ds(col, 512)].reshape(512, 512)
        r = _dot(xa32_ref[...], w)
        new = qa_ref[hg]
        for j in range(4):
            new = jnp.where(row32 == half * 4 + j, r[:, 128 * j:128 * j + 128], new)
        qa_ref[hg] = new

    def qb_item(n):
        hg = n >> 1
        half = n & 1
        w = wbq_buf[pl.ds(half * 2, 2), :, hg].reshape(2048, 128)
        qb_ref[hg] = qb_ref[hg] + _dot(xexp_ref[half], w)

    def qabs_item(n):
        hg = n & 3
        u = n >> 2
        q = qb_ref[hg].astype(BF16)
        w = wuk_buf[u, :, hg].reshape(1024, 128)
        r = _dot_nt(q, w)
        r = jnp.concatenate(
            [jnp.where(row32 == lane32, r[:, 128 * k:128 * k + 128], 0.0).astype(BF16)
             for k in range(8)], axis=1)
        qa = _dot_nt(r, e0_ref[...])
        for b in range(4):
            qabs_ref[u, b, hg] = qa[8 * b:8 * b + 8, :]

    def score_item(b, n, fl):
        qa = jnp.concatenate(
            [qabs_ref[u, b].reshape(32, 128).astype(BF16) for u in range(4)], axis=1)
        seg = b * 4 + (n >> 1)
        m = jnp.where(n == 0, -jnp.inf, mb_ref[...])
        for k in range(4):
            row = pl.multiple_of((n & 1) * 512 + k * 128, 128)
            s = _dot_nt(qa, cbuf[seg, pl.ds(row, 128), :])
            if k == 0:
                fl(s)
            sb_ref[n, :, 128 * k:128 * k + 128] = s
            m = jnp.maximum(m, s)
        mb_ref[...] = m

    def max_b():
        mb_ref[...] = jnp.broadcast_to(jnp.max(mb_ref[...], axis=1, keepdims=True), (32, 128))

    def pv_item(b, n, fl):
        m = mb_ref[...]
        ps = [jnp.exp((sb_ref[n, :, 128 * k:128 * k + 128] - m) * scale) for k in range(4)]
        first = n == 0
        lb_ref[...] = jnp.where(first, 0.0, lb_ref[...]) + ((ps[0] + ps[1]) + (ps[2] + ps[3]))
        seg = b * 4 + (n >> 1)
        acc = jnp.where(first, 0.0, cacc_ref[...])
        for k in range(4):
            row = pl.multiple_of((n & 1) * 512 + k * 128, 128)
            d = _dot(ps[k].astype(BF16), cbuf[seg, pl.ds(row, 128), :])
            if k == 0:
                fl(d)
            acc = acc + d
        cacc_ref[...] = acc

    def norm_b(b):
        inv = 1.0 / jnp.sum(lb_ref[...], axis=1, keepdims=True)
        res = cacc_ref[...] * inv
        for u in range(4):
            cc_ref[u, b] = res[:, 128 * u:128 * u + 128].reshape(4, 8, 128)

    def ctx_item(n, fl):
        hg = n >> 2
        u = n & 3
        c32 = jnp.concatenate([cc_ref[u, bb, hg] for bb in range(4)], axis=0)
        w = wuv_buf[u, :, hg].reshape(1024, 128)
        ctx_ref[hg] = ctx_ref[hg] + _dot(expand(c32, fl), w)

    def out_part(o32, w_buf, hg, j0, nj, fl=_nop):
        acc = None
        for j in range(nj):
            row = _mo((j0 + j) * 128, 128)
            d = _dot(jnp.where(row32 == j0 + j, o32, 0.0).astype(BF16),
                     w_buf[hg, pl.ds(row, 128), :])
            if j == 0:
                fl(d)
            acc = d if acc is None else acc + d
        return acc

    def out_item(o_ref, w_buf, hg, half, acc_ref, fl=_nop):
        acc_ref[...] = acc_ref[...] + out_part(o_ref[hg], w_buf, hg, half * 4, 4, fl)

    def rowsum(acc):
        return jnp.sum(acc.reshape(4, 8, 512), axis=1)

    def k_work(g, r):
        q = qa_ref[g >> 2, pl.ds(_mo((g & 3) * 8, 8), 8), :].astype(BF16)
        row = pl.multiple_of(r * 128, 128)
        s = jnp.zeros((8, 128), F32)
        for j in range(8):
            sj = _dot_nt(q, kbuf[j, pl.ds(row, 128), :])
            s = jnp.where(row8 == j, sj, s)
        sa_ref[r] = s

    def v_part(r, fl=_nop):
        p = pa_ref[r].astype(BF16)
        row = _mo(r * 128, 128)
        o = jnp.zeros((8, 128), F32)
        for j in range(8):
            oj = _dot(p, vbuf[j, pl.ds(row, 128), :])
            if j == 0:
                fl(oj)
            o = jnp.where(row8 == j, oj, o)
        return oacc_ref[...] + o

    def finalize_o(g):
        l = jnp.sum(psum_ref[...], axis=1, keepdims=True)
        oa_ref[g >> 2, pl.ds(_mo((g & 3) * 8, 8), 8), :] = oacc_ref[...] * (1.0 / l)

    def softmax_a():
        s = sa_ref[...]
        m = jnp.max(jnp.max(s, axis=0), axis=1, keepdims=True)
        p = jnp.exp((s - m[None]) * scale)
        pa_ref[...] = p
        psum_ref[...] = jnp.sum(p, axis=0)
        oacc_ref[...] = jnp.zeros((8, 128), F32)

    def k0a_body(r, carry):
        for t in range(4):
            low_kv(k_hbm, kbuf, 0, r, t, r * 4 + t).wait()
            high_wq(0, r * 16 + (t >> 1) * 8, (t & 1) * 512, 512).start(priority=HI)
            low_kv(k_hbm, kbuf, 0, r + 4, t, r * 4 + t).start(priority=LO)
        return carry
    lax.fori_loop(0, 4, k0a_body, 0)

    x_prep()

    def k0b_body(r, carry):
        for t in range(4):
            low_kv(k_hbm, kbuf, 0, r + 4, t, r * 4 + t).wait()
            high_wq(0, 64 + r * 16 + (t >> 1) * 8, (t & 1) * 512, 512).start(priority=HI)
            low_c(0, r, t, r * 4 + t).start(priority=LO)
        return carry
    lax.fori_loop(0, 4, k0b_body, 0)

    def c0_body(it, carry):
        nx = it + 4
        s0 = (it & 3) * 4
        for t in range(4):
            low_c(0, it, t, s0 + t).wait()
            high_3d(wbq_hbm, wbq_buf, it * 4 + t, 0, 4, S_WBQ).start(priority=HI)
            low_c(nx >> 5, nx & 31, t, s0 + t).start(priority=LO)

        @pl.when(it == 1)
        def _():
            wait_all(wq_buf.at[0], S_WQ)

        @pl.when(jnp.logical_and(it >= 1, it < 3))
        def _():
            qa_item(0, it - 1)

        @pl.when(jnp.logical_and(it >= 3, it < 11))
        def _():
            k_work(0, it - 3)

        @pl.when(it == 11)
        def _():
            softmax_a()
        return carry
    lax.fori_loop(0, 32, c0_body, 0)

    def c1_tick(it, t, s0):
        low_c(1, it, t, s0 + t).wait()
        high_3d(wuk_hbm, wuk_buf, it * 4 + t, 0, 4, S_WUK).start(priority=HI)

    def c1_body(it, carry):
        s0 = (it & 3) * 4
        for t in range(4):
            c1_tick(it, t, s0)
            low_c(1, it + 4, t, s0 + t).start(priority=LO)

        @pl.when(it == 1)
        def _():
            wait_all(wbq_buf, S_WBQ)

        @pl.when(jnp.logical_and(it >= 1, it < 9))
        def _():
            qb_item(it - 1)
        return carry
    lax.fori_loop(0, 28, c1_body, 0)

    for it in range(28, 32):
        s0 = (it & 3) * 4
        for t in range(4):
            c1_tick(it, t, s0)
            start_pair(head_of(1), head_of(0), (it - 28) >> 1, (it & 1) * 4 + t, s0 + t)

    def make_main(high, pin, hook, hook_floats, extra, last):
        def body(i, carry):
            g = i >> 3
            r = i & 7
            i2 = i + 2
            g2 = i2 >> 3
            r2 = i2 & 7
            hk = head_of(g2 + 1)
            hv = head_of(g2)
            s0 = (i & 1) * 8
            more = i2 < N_MAIN

            def floater(t):
                def fl(val=None):
                    if PIN and val is not None:
                        pin(val)
                    high(i, t)
                return fl

            def tick(t, with_high=True):
                wait_pair(r, t, s0 + t)
                if with_high:
                    high(i, t)
                if not last:
                    start_pair(hk, hv, r2, t, s0 + t)
                else:
                    @pl.when(more)
                    def _():
                        start_pair(hk, hv, r2, t, s0 + t)

                    @pl.when(jnp.logical_not(more))
                    def _():
                        low_kv(v_hbm, vbuf, hv, 2 * r2 + (t >> 2), t & 3, s0 + t).start(priority=LO)

            tick(0)
            tick(1, not PIN)

            @pl.when(jnp.logical_and(r == 0, i > 0))
            def _():
                finalize_o(g - 1)
                softmax_a()

            extra(i)
            tick(2)
            tick(3)
            hook(i, floater(5) if hook_floats else _nop)
            tick(4)
            tick(5, not hook_floats)
            tick(6)
            tick(7)
            oacc_ref[...] = v_part(r, floater(1) if PIN else _nop)
            k_work(g + 1, r)
            return carry
        return body

    def pin_to(buf_view):
        def pin(val):
            buf_view[...] = val[:8, :128].astype(BF16)
        return pin

    def high0(i, t):
        high_wq(1 + (i >> 3), (i & 7) * 16 + (t >> 2) * 8, (t & 3) * 256, 256).start(priority=HI)

    def hook0(i, fl):
        @pl.when(i == 1)
        def _():
            wait_all(wuk_buf, S_WUK)

        @pl.when(jnp.logical_and(i >= 1, i < 17))
        def _():
            qabs_item(i - 1)

        @pl.when(i == 18)
        def _():
            wait_all(wq_buf.at[1], S_WQ + 1)
            wait_all(wq_buf.at[2], S_WQ + 2)

        @pl.when(jnp.logical_and(i >= 18, i < 22))
        def _():
            qa_item((i >> 1) - 8, i & 1)

    def high1(i, t):
        @pl.when(i < 56)
        def _():
            high_3d(wuv_hbm, wuv_buf, (i - 24) * 4 + (t >> 1), (t & 1) * 2, 2, S_WUV).start(priority=HI)

        @pl.when(i >= 56)
        def _():
            high_2d(wbo_hbm, wbo_buf, 4, (i - 56) * 32 + (t >> 1) * 8, (t & 1) * 256,
                    S_WBO).start(priority=HI)

    def pin1(val):
        wuv_buf[4, 0, 0] = val[:8, :128].astype(BF16)
        wbo_buf[4, 0:8, 0:128] = val[:8, :128].astype(BF16)

    def extra1(i):
        n = i - 24

        @pl.when(i == 25)
        def _():
            wait_all(wq_buf.at[3], S_WQ + 3)

        @pl.when(jnp.logical_and(i >= 25, i < 27))
        def _():
            qa_item(3, i - 25)

        @pl.when((n & 15) == 8)
        def _():
            max_b()

        @pl.when(jnp.logical_and((n & 15) == 1, n > 16))
        def _():
            norm_b((n >> 4) - 1)

    def hook1(i, fl):
        n = i - 24

        @pl.when((n & 8) == 0)
        def _():
            score_item(n >> 4, n & 7, fl)

        @pl.when((n & 8) != 0)
        def _():
            pv_item(n >> 4, n & 7, fl)

    def high2(i, t):
        high_2d(wo_hbm, wo_buf, 3, (i - 88) * 32 + (t >> 1) * 8, (t & 1) * 256,
                S_WO + ((i - 88) >> 4)).start(priority=HI)

    def extra2(i):
        @pl.when(i == 88)
        def _():
            wait_all(wuv_buf.at[pl.ds(0, 4)], S_WUV)
            norm_b(3)

        @pl.when(i == 104)
        def _():
            wait_all(wbo_buf.at[pl.ds(0, 4)], S_WBO)

        @pl.when(i == 113)
        def _():
            wait_all(wo_buf.at[pl.ds(0, 3), pl.ds(0, 512), :], S_WO)
            out_ref[:, 512:] = rowsum(accb_ref[...]).astype(out_ref.dtype)

    def hook2(i, fl):
        @pl.when(i < 104)
        def _():
            ctx_item(i - 88, fl)

        @pl.when(jnp.logical_and(i >= 104, i < 112))
        def _():
            out_item(ctx_ref, wbo_buf, (i - 104) >> 1, i & 1, accb_ref, fl)

        @pl.when(jnp.logical_and(i >= 113, i < 116))
        def _():
            out_item(oa_ref, wo_buf, i - 113, 0, acca_ref, fl)

        @pl.when(jnp.logical_or(i == 112, i >= 116))
        def _():
            fl()

    lax.fori_loop(0, 24, make_main(high0, pin_to(wq_buf.at[4, 0, 0:8, 0:128]), hook0, False,
                                   _nop, False), 0)
    lax.fori_loop(24, 88, make_main(high1, pin1, hook1, FLOAT_HOOK, extra1, False), 0)
    lax.fori_loop(88, N_MAIN, make_main(high2, pin_to(wo_buf.at[4, 0:8, 0:128]), hook2,
                                        FLOAT_HOOK, extra2, True), 0)

    finalize_o(14)
    softmax_a()

    def v15_body(r, carry):
        s0 = (r & 3) * 4
        for t in range(4):
            low_kv(v_hbm, vbuf, 0, r, t, s0 + t).wait()

            @pl.when(r < 4)
            def _():
                row = pl.multiple_of(r * 128 + t * 32, 32)
                pltpu.make_async_copy(
                    wo_hbm.at[3, pl.ds(row, 32), :], wo_buf.at[3, pl.ds(row, 32), :],
                    hsem.at[S_WO + 2]).start(priority=HI)
                low_kv(v_hbm, vbuf, head_of(15), r + 4, t, s0 + t).start(priority=LO)

            @pl.when(jnp.logical_and(r >= 4, r < 6))
            def _():
                low_wo(s0 + t, s0 + t).start(priority=LO)

            if t == 1:
                @pl.when(r == 1)
                def _():
                    wait_all(wo_buf.at[pl.ds(0, 3), pl.ds(512, 512), :], S_WO + 1)

                @pl.when(jnp.logical_and(r >= 1, r < 4))
                def _():
                    out_item(oa_ref, wo_buf, r - 1, 1, acca_ref)

                @pl.when(r == 4)
                def _():
                    l = jnp.sum(psum_ref[...], axis=1, keepdims=True)
                    psum_ref[...] = jnp.broadcast_to(1.0 / l, (8, 128))
        oacc_ref[...] = v_part(r)
        return carry
    lax.fori_loop(0, 7, v15_body, 0)

    wait_all(wo_buf.at[3, pl.ds(0, 512), :], S_WO + 2)
    for t in range(4):
        low_kv(v_hbm, vbuf, 0, 7, t, 12 + t).wait()
    oa_ref[3, 24:32, :] = v_part(7) * psum_ref[...]
    o32 = oa_ref[3]
    acca_ref[...] = acca_ref[...] + out_part(o32, wo_buf, 3, 0, 4)
    for n in range(6):
        low_wo(n, n).wait()
    part = rowsum(acca_ref[...] + out_part(o32, wo_buf, 3, 4, 3))
    o_last = oa_ref[3, pl.ds(7, 4, stride=8), :].astype(BF16)
    for n in range(6, 8):
        low_wo(n, n).wait()
    out_ref[:, :512] = (part + _dot(o_last, wo_buf[3, 896:1024, :])).astype(out_ref.dtype)


@jax.jit
def pallas_concat_heads__sliding_block_cached__compressed_kv_cla__decode_kernel(
    A_x: jax.Array,
    A_k_cache: jax.Array,
    A_v_cache: jax.Array,
    A_wq: jax.Array,
    A_wo: jax.Array,
    B_x: jax.Array,
    B_c_kv: jax.Array,
    B_w_q: jax.Array,
    B_w_uk: jax.Array,
    B_w_uv: jax.Array,
    B_w_o: jax.Array,
):
    B, Sq, D = A_x.shape
    _, H, Sk, Dh = A_k_cache.shape
    W = min(4096, max(256, Sk // 4))
    assert (B, Sq, D, H, Sk, Dh, W) == (4, 1, 512, 32, 4096, 128, 1024)
    assert B_c_kv.shape == (4, 4096, 512) and B_w_q.shape == (512, 32, 128)

    def body(*refs):
        _kernel(*refs, win_off=Sk - W, scale=float(Dh) ** -0.5)

    vm = pltpu.VMEM
    scratch = [
        vm((2, 8, 1024, 128), BF16),
        vm((16, 1024, 512), BF16),
        vm((5, 4, 128, 1024), BF16),
        vm((5, 1024, 512), BF16),
        vm((4, 128, 4, 8, 128), BF16),
        vm((4, 128, 4, 8, 128), BF16),
        vm((5, 128, 4, 8, 128), BF16),
        vm((5, 1024, 512), BF16),
        vm((4, 512), BF16),
        vm((4, 512), BF16),
        vm((128, 1024), BF16),
        vm((32, 512), BF16),
        vm((2, 32, 2048), BF16),
        vm((4, 32, 128), F32),
        vm((8, 8, 128), F32),
        vm((8, 8, 128), F32),
        vm((8, 128), F32),
        vm((8, 128), F32),
        vm((4, 32, 128), F32),
        vm((4, 32, 128), F32),
        vm((4, 4, 4, 8, 128), F32),
        vm((8, 32, 512), F32),
        vm((32, 128), F32),
        vm((32, 128), F32),
        vm((32, 512), F32),
        vm((4, 4, 4, 8, 128), F32),
        vm((4, 32, 128), F32),
        vm((32, 512), F32),
        vm((32, 512), F32),
        pltpu.SemaphoreType.DMA((NS,)),
        pltpu.SemaphoreType.DMA((N_HSEM,)),
        pltpu.SemaphoreType.DMA((2,)),
    ]
    out = pl.pallas_call(
        body,
        out_shape=jax.ShapeDtypeStruct((B, 2 * D), A_x.dtype),
        in_specs=[pl.BlockSpec(memory_space=pl.ANY)] * 11,
        scratch_shapes=scratch,
        compiler_params=pltpu.CompilerParams(
            vmem_limit_bytes=64 * 1024 * 1024,
            disable_bounds_checks=True,
            disable_semaphore_checks=True,
        ),
    )(
        A_x.reshape(B, D),
        A_k_cache.reshape(B * H, Sk, Dh),
        A_v_cache.reshape(B * H, Sk, Dh),
        A_wq.reshape(4, 128, 4096),
        A_wo.reshape(4, 1024, 512),
        B_x.reshape(B, D),
        B_c_kv.reshape(16, 1024, 512),
        B_w_q.reshape(4, 128, 4, 8, 128),
        B_w_uk.reshape(4, 128, 4, 8, 128),
        B_w_uv.reshape(4, 128, 4, 8, 128),
        B_w_o.reshape(4, 1024, 512),
    )
    return out.reshape(B, Sq, 2 * D)
```

```python
import jax
import jax.numpy as jnp
from jax import lax
import jax.experimental.pallas as pl
import jax.experimental.pallas.tpu as pltpu

F32 = jnp.float32
BF16 = jnp.bfloat16
_NT = (((1,), (1,)), ((), ()))
_NN = (((1,), (0,)), ((), ()))

LO, HI = 1, 0
NS = 16
N_MAIN = 112
FLOAT_HOOK = True
PIN = False
CMODE = 1

S_WQ = 0
S_WBQ = 4
S_WUK = 5
S_WUV = 6
S_WBO = 7
S_WO = 8
N_HSEM = 11


def _dot(a, b):
    return lax.dot_general(a, b, _NN, preferred_element_type=F32)


def _dot_nt(a, b):
    return lax.dot_general(a, b, _NT, preferred_element_type=F32)


def _mo(x, m):
    return x if isinstance(x, int) else pl.multiple_of(x, m)


def _nop(_=None):
    return None


def _kernel(xa_hbm, k_hbm, v_hbm, wq_hbm, wo_hbm, xb_hbm, c_hbm, wbq_hbm, wuk_hbm,
            wuv_hbm, wbo_hbm, out_ref,
            kvbuf, cbuf, wq_buf, wo_buf, wbq_buf, wuk_buf, wuv_buf, wbo_buf,
            xa_buf, xb_buf, e0_ref, xa32_ref, xexp_ref,
            qa_ref, sa_ref, pa_ref, psum_ref, oacc_ref, oa_ref,
            qb_ref, qabs_ref, sb_ref, mb_ref, lb_ref, cacc_ref, cc_ref, ctx_ref,
            acca_ref, accb_ref,
            lsem, hsem, xsem, *, win_off, scale):

    def low_c(pair, it, t, sem):
        if CMODE == 1:
            row = _mo(pair * 512 + it * 16 + (t >> 1) * 8, 8)
            col = (t & 1) * 256
            return pltpu.make_async_copy(
                c_hbm.at[:, pl.ds(row, 8), pl.ds(col, 256)],
                cbuf.at[:, pl.ds(row, 8), pl.ds(col, 256)],
                lsem.at[sem])
        row = _mo(it * 32 + t * 8, 8)
        return pltpu.make_async_copy(
            c_hbm.at[pl.ds(pair * 8, 8), pl.ds(row, 8), :],
            cbuf.at[pl.ds(pair * 8, 8), pl.ds(row, 8), :],
            lsem.at[sem])

    def batch_of(g):
        return (g >> 1) & 3

    def hg_of(g):
        return (g >> 3) * 2 + (g & 1)

    def low16(src, kv, sg, r, t, sem):
        row = _mo(r * 128 + t * 16, 16)
        head = (sg & 3) * 32 + (sg >> 2) * 16
        return pltpu.make_async_copy(
            src.at[pl.ds(head, 16), pl.ds(_mo(win_off + row, 16), 16), :],
            kvbuf.at[kv, :, pl.ds(row, 16), :],
            lsem.at[sem])

    def low_v8(e, r, t, sem):
        row = _mo(r * 128 + t * 32, 32)
        return pltpu.make_async_copy(
            v_hbm.at[pl.ds(112 + e * 8, 8), pl.ds(_mo(win_off + row, 32), 32), :],
            kvbuf.at[1, pl.ds(e * 8, 8), pl.ds(row, 32), :],
            lsem.at[sem])

    def low_wo(n, sem):
        row = _mo(n * 64, 64)
        return pltpu.make_async_copy(
            wo_hbm.at[7, pl.ds(row, 64), :], wo_buf.at[7, pl.ds(row, 64), :], lsem.at[sem])

    def high_wq(row, col, cols, sem):
        row = _mo(row, 8)
        return pltpu.make_async_copy(
            wq_hbm.at[:, pl.ds(row, 8), pl.ds(col, cols)],
            wq_buf.at[pl.ds(0, 4), pl.ds(row, 8), pl.ds(col, cols)], hsem.at[sem])

    def high_3d(src, dst, row, hg, nhg, sem):
        return pltpu.make_async_copy(
            src.at[:, row, pl.ds(hg, nhg)], dst.at[pl.ds(0, 4), row, pl.ds(hg, nhg)], hsem.at[sem])

    def high_wbo(half, row, col):
        row = _mo(row, 8)
        return pltpu.make_async_copy(
            wbo_hbm.at[:, half, pl.ds(row, 8), pl.ds(col, 256)],
            wbo_buf.at[pl.ds(0, 4), half, pl.ds(row, 8), pl.ds(col, 256)], hsem.at[S_WBO])

    def high_wo(p0, np_, row, rows, col, cols, sem):
        row = _mo(row, 8)
        return pltpu.make_async_copy(
            wo_hbm.at[pl.ds(p0, np_), pl.ds(row, rows), pl.ds(col, cols)],
            wo_buf.at[pl.ds(p0, np_), pl.ds(row, rows), pl.ds(col, cols)], hsem.at[sem])

    def wait_all(buf, sem):
        pltpu.make_async_copy(buf, buf, hsem.at[sem]).wait()

    for r in range(2):
        for t in range(8):
            low16(k_hbm, 0, 0, r, t, r * 8 + t).start(priority=LO)
    cp_xa = pltpu.make_async_copy(xa_hbm, xa_buf, xsem.at[0])
    cp_xb = pltpu.make_async_copy(xb_hbm, xb_buf, xsem.at[1])
    cp_xa.start(priority=HI)
    cp_xb.start(priority=HI)

    row8 = lax.broadcasted_iota(jnp.int32, (8, 128), 0)
    row32 = lax.broadcasted_iota(jnp.int32, (32, 128), 0) & 7
    lane32 = lax.broadcasted_iota(jnp.int32, (32, 128), 1) & 7

    def e0_body(i, c):
        r0 = pl.multiple_of(i * 16, 16)
        rr = lax.broadcasted_iota(jnp.int32, (16, 1024), 0) + r0
        cc = lax.broadcasted_iota(jnp.int32, (16, 1024), 1) >> 3
        e0_ref[pl.ds(r0, 16), :] = jnp.where(rr == cc, 1.0, 0.0).astype(BF16)
        return c
    lax.fori_loop(0, 8, e0_body, 0)

    qa_ref[...] = jnp.zeros(qa_ref.shape, F32)
    qb_ref[...] = jnp.zeros(qb_ref.shape, F32)
    ctx_ref[...] = jnp.zeros(ctx_ref.shape, F32)
    acca_ref[...] = jnp.zeros(acca_ref.shape, F32)
    accb_ref[...] = jnp.zeros(accb_ref.shape, F32)
    mb_ref[...] = jnp.zeros(mb_ref.shape, F32)
    lb_ref[...] = jnp.zeros(lb_ref.shape, F32)
    cacc_ref[...] = jnp.zeros(cacc_ref.shape, F32)

    def expand(c32, fl=_nop):
        ce = _dot(c32.astype(BF16), e0_ref[...])
        fl(ce)
        return jnp.concatenate(
            [jnp.where(row32 == lane32, ce[:, 128 * k:128 * k + 128], 0.0).astype(BF16)
             for k in range(8)], axis=1)

    def x_prep():
        cp_xa.wait()
        cp_xb.wait()
        xa = xa_buf[...].astype(F32)
        xb = xb_buf[...].astype(F32)
        xa32_ref[...] = jnp.concatenate(
            [jnp.broadcast_to(xa[b:b + 1, :], (8, 512)) for b in range(4)], axis=0).astype(BF16)
        xb32 = jnp.concatenate(
            [jnp.broadcast_to(xb[b:b + 1, :], (8, 512)) for b in range(4)], axis=0)
        for u in range(4):
            xexp_ref[u >> 1, :, (u & 1) * 1024:(u & 1) * 1024 + 1024] = expand(
                xb32[:, 128 * u:128 * u + 128])

    def qa_item(hg, half):
        col = pl.multiple_of(hg * 1024 + half * 512, 512)
        w = wq_buf[0:4, :, pl.ds(col, 512)].reshape(512, 512)
        r = _dot(xa32_ref[...], w)
        new = qa_ref[hg]
        for j in range(4):
            new = jnp.where(row32 == half * 4 + j, r[:, 128 * j:128 * j + 128], new)
        qa_ref[hg] = new

    def qb_item(n):
        hg = n >> 1
        half = n & 1
        w = wbq_buf[pl.ds(half * 2, 2), :, hg].reshape(2048, 128)
        qb_ref[hg] = qb_ref[hg] + _dot(xexp_ref[half], w)

    def qabs_item(n, fl):
        hg = n & 3
        u = n >> 2
        q = qb_ref[hg].astype(BF16)
        w = wuk_buf[u, :, hg].reshape(1024, 128)
        r = _dot_nt(q, w)
        fl(r)
        r = jnp.concatenate(
            [jnp.where(row32 == lane32, r[:, 128 * k:128 * k + 128], 0.0).astype(BF16)
             for k in range(8)], axis=1)
        qa = _dot_nt(r, e0_ref[...])
        for b in range(4):
            qabs_ref[u, b, hg] = qa[8 * b:8 * b + 8, :]

    def score_item(b, n, fl):
        qa = jnp.concatenate(
            [qabs_ref[u, b].reshape(32, 128).astype(BF16) for u in range(4)], axis=1)
        seg = b * 4 + (n >> 1)
        m = jnp.where(n == 0, -jnp.inf, mb_ref[...])
        for k in range(4):
            row = pl.multiple_of((n & 1) * 512 + k * 128, 128)
            s = _dot_nt(qa, cbuf[seg, pl.ds(row, 128), :])
            if k == 0:
                fl(s)
            sb_ref[n, :, 128 * k:128 * k + 128] = s
            m = jnp.maximum(m, s)
        mb_ref[...] = m

    def max_b():
        mb_ref[...] = jnp.broadcast_to(jnp.max(mb_ref[...], axis=1, keepdims=True), (32, 128))

    def pv_item(b, n, fl):
        m = mb_ref[...]
        ps = [jnp.exp((sb_ref[n, :, 128 * k:128 * k + 128] - m) * scale) for k in range(4)]
        first = n == 0
        lb_ref[...] = jnp.where(first, 0.0, lb_ref[...]) + ((ps[0] + ps[1]) + (ps[2] + ps[3]))
        seg = b * 4 + (n >> 1)
        acc = jnp.where(first, 0.0, cacc_ref[...])
        for k in range(4):
            row = pl.multiple_of((n & 1) * 512 + k * 128, 128)
            d = _dot(ps[k].astype(BF16), cbuf[seg, pl.ds(row, 128), :])
            if k == 0:
                fl(d)
            acc = acc + d
        cacc_ref[...] = acc

    def norm_b(b):
        inv = 1.0 / jnp.sum(lb_ref[...], axis=1, keepdims=True)
        res = cacc_ref[...] * inv
        for u in range(4):
            cc_ref[u, b] = res[:, 128 * u:128 * u + 128].reshape(4, 8, 128)

    def ctx_item(n, fl):
        hg = n >> 2
        u = n & 3
        c32 = jnp.concatenate([cc_ref[u, bb, hg] for bb in range(4)], axis=0)
        w = wuv_buf[u, :, hg].reshape(1024, 128)
        ctx_ref[hg] = ctx_ref[hg] + _dot(expand(c32, fl), w)

    def out_part(o32, w_half, j0, jj, nj, fl=_nop):
        acc = None
        for j in range(jj, jj + nj):
            d = _dot(jnp.where(row32 == j0 + j, o32, 0.0).astype(BF16),
                     w_half[j * 128:j * 128 + 128, :])
            if j == jj:
                fl(d)
            acc = d if acc is None else acc + d
        return acc

    def out_a_item(n, fl=_nop):
        acca_ref[...] = acca_ref[...] + out_part(
            oa_ref[n >> 1], wo_buf.at[n], (n & 1) * 4, 0, 4, fl)

    def out_b_item(n, fl=_nop):
        accb_ref[...] = accb_ref[...] + out_part(
            ctx_ref[n >> 1], wbo_buf.at[n >> 1, n & 1], (n & 1) * 4, 0, 4, fl)

    def rowsum(acc):
        return jnp.sum(acc.reshape(4, 8, 512), axis=1)

    def k_work(g, r):
        q = qa_ref[hg_of(g), pl.ds(_mo(batch_of(g) * 8, 8), 8), :].astype(BF16)
        row = pl.multiple_of(r * 128, 128)
        h0 = (g & 1) * 8
        s = jnp.zeros((8, 128), F32)
        for j in range(8):
            sj = _dot_nt(q, kvbuf[0, h0 + j, pl.ds(row, 128), :])
            s = jnp.where(row8 == j, sj, s)
        sa_ref[r] = s

    def v_part(g, r, fl=_nop):
        p = pa_ref[r].astype(BF16)
        row = _mo(r * 128, 128)
        h0 = (g & 1) * 8
        o = jnp.zeros((8, 128), F32)
        for j in range(8):
            oj = _dot(p, kvbuf[1, h0 + j, pl.ds(row, 128), :])
            if j == 0:
                fl(oj)
            o = jnp.where(row8 == j, oj, o)
        return oacc_ref[...] + o

    def finalize_o(g):
        l = jnp.sum(psum_ref[...], axis=1, keepdims=True)
        oa_ref[hg_of(g), pl.ds(_mo(batch_of(g) * 8, 8), 8), :] = oacc_ref[...] * (1.0 / l)

    def softmax_a():
        s = sa_ref[...]
        m = jnp.max(jnp.max(s, axis=0), axis=1, keepdims=True)
        p = jnp.exp((s - m[None]) * scale)
        pa_ref[...] = p
        psum_ref[...] = jnp.sum(p, axis=0)
        oacc_ref[...] = jnp.zeros((8, 128), F32)

    def k0_tick(r, t, s0):
        low16(k_hbm, 0, 0, r, t, s0 + t).wait()
        high_wq(r * 16 + (t >> 2) * 8, (t & 3) * 512, 512, S_WQ).start(priority=HI)

    def k0a_body(r, carry):
        s0 = (r & 1) * 8
        for t in range(8):
            k0_tick(r, t, s0)
            low16(k_hbm, 0, 0, r + 2, t, s0 + t).start(priority=LO)
        return carry
    lax.fori_loop(0, 6, k0a_body, 0)

    x_prep()

    def k0b_body(r, carry):
        s0 = r * 8
        for t in range(8):
            k0_tick(r + 6, t, s0)
            low_c(0, r * 2 + (t >> 2), t & 3, s0 + t).start(priority=LO)
        return carry
    lax.fori_loop(0, 2, k0b_body, 0)

    def c0_body(it, carry):
        nx = it + 4
        s0 = (it & 3) * 4
        for t in range(4):
            low_c(0, it, t, s0 + t).wait()
            high_3d(wbq_hbm, wbq_buf, it * 4 + t, 0, 4, S_WBQ).start(priority=HI)
            low_c(nx >> 5, nx & 31, t, s0 + t).start(priority=LO)

        @pl.when(it == 1)
        def _():
            wait_all(wq_buf.at[pl.ds(0, 4), :, pl.ds(0, 2048)], S_WQ)

        @pl.when(jnp.logical_and(it >= 1, it < 5))
        def _():
            qa_item((it - 1) >> 1, (it - 1) & 1)

        @pl.when(jnp.logical_and(it >= 5, it < 13))
        def _():
            k_work(0, it - 5)

        @pl.when(it == 13)
        def _():
            softmax_a()
        return carry
    lax.fori_loop(0, 32, c0_body, 0)

    def c1_tick(it, t, s0):
        low_c(1, it, t, s0 + t).wait()
        high_3d(wuk_hbm, wuk_buf, it * 4 + t, 0, 4, S_WUK).start(priority=HI)

    def c1_body(it, carry):
        s0 = (it & 3) * 4
        for t in range(4):
            c1_tick(it, t, s0)
            low_c(1, it + 4, t, s0 + t).start(priority=LO)

        @pl.when(it == 1)
        def _():
            wait_all(wbq_buf, S_WBQ)

        @pl.when(jnp.logical_and(it >= 1, it < 9))
        def _():
            qb_item(it - 1)
        return carry
    lax.fori_loop(0, 28, c1_body, 0)

    def c1b_body(r, carry):
        for t in range(8):
            c1_tick(28 + r * 2 + (t >> 2), t & 3, r * 8 + (t >> 2) * 4)
            low16(v_hbm, 1, 0, r, t, r * 8 + t).start(priority=LO)
        return carry
    lax.fori_loop(0, 2, c1b_body, 0)

    def make_main(high, pin, hook, hook_floats, extra, last):
        def body(i, carry):
            g = i >> 3
            r = i & 7
            i2 = i + 2
            g2 = i2 >> 3
            r2 = i2 & 7
            sg2 = (g2 + 1) >> 1
            odd2 = (g2 & 1) == 1
            s0 = (i & 1) * 8
            kv = 1 - (g & 1)

            def floater(t):
                def fl(val=None):
                    if PIN and val is not None:
                        pin(val)
                    high(i, t)
                return fl

            def tick(t, with_high=True):
                low16(k_hbm, kv, 0, r, t, s0 + t).wait()
                if with_high:
                    high(i, t)

                @pl.when(odd2)
                def _():
                    low16(k_hbm, 0, sg2, r2, t, s0 + t).start(priority=LO)

                if not last:
                    @pl.when(jnp.logical_not(odd2))
                    def _():
                        low16(v_hbm, 1, sg2, r2, t, s0 + t).start(priority=LO)
                else:
                    @pl.when(jnp.logical_and(jnp.logical_not(odd2), i2 < N_MAIN))
                    def _():
                        low16(v_hbm, 1, sg2, r2, t, s0 + t).start(priority=LO)

                    @pl.when(i2 >= N_MAIN)
                    def _():
                        low_v8(0, 2 * r2 + (t >> 2), t & 3, s0 + t).start(priority=LO)

            tick(0)
            tick(1, not PIN)

            @pl.when(jnp.logical_and(r == 0, i > 0))
            def _():
                finalize_o(g - 1)
                softmax_a()

            extra(i)
            tick(2)
            tick(3)
            hook(i, floater(5) if hook_floats else _nop)
            tick(4)
            tick(5, not hook_floats)
            tick(6)
            tick(7)
            oacc_ref[...] = v_part(g, r, floater(1) if PIN else _nop)
            k_work(g + 1, r)
            return carry
        return body

    def pin_to(buf_view):
        def pin(val):
            buf_view[...] = val[:8, :128].astype(BF16)
        return pin

    def high0(i, t):
        high_wq(i * 8, 2048 + t * 256, 256, S_WQ + 1).start(priority=HI)

    def hook0(i, fl):
        @pl.when(i == 0)
        def _():
            wait_all(wuk_buf, S_WUK)

        qabs_item(i, fl)

    def high1(i, t):
        @pl.when(i < 48)
        def _():
            high_3d(wuv_hbm, wuv_buf, (i - 16) * 4 + (t >> 1), (t & 1) * 2, 2,
                    S_WUV).start(priority=HI)

        @pl.when(i >= 48)
        def _():
            high_wbo((i >> 4) - 3, (i & 15) * 32 + (t >> 1) * 8, (t & 1) * 256).start(priority=HI)

    def pin1(val):
        wuv_buf[4, 0, 0] = val[:8, :128].astype(BF16)
        wbo_buf[4, 0, 0:8, 0:128] = val[:8, :128].astype(BF16)

    def extra1(i):
        n = i - 16

        @pl.when(i == 25)
        def _():
            wait_all(wq_buf.at[pl.ds(0, 4), :, pl.ds(2048, 2048)], S_WQ + 1)

        @pl.when(jnp.logical_and(i >= 25, i < 29))
        def _():
            qa_item(2 + ((i - 25) >> 1), (i - 25) & 1)

        @pl.when((n & 15) == 8)
        def _():
            max_b()

        @pl.when(jnp.logical_and((n & 15) == 1, n > 16))
        def _():
            norm_b((n >> 4) - 1)

    def hook1(i, fl):
        n = i - 16

        @pl.when((n & 8) == 0)
        def _():
            score_item(n >> 4, n & 7, fl)

        @pl.when((n & 8) != 0)
        def _():
            pv_item(n >> 4, n & 7, fl)

    def high2(i, t):
        row = (i & 15) * 32 + (t >> 1) * 8

        @pl.when(i < 96)
        def _():
            high_wo(0, 4, row, 8, (t & 1) * 256, 256, S_WO).start(priority=HI)

        @pl.when(i >= 96)
        def _():
            high_wo(4, 2, row, 8, (t & 1) * 256, 256, S_WO + 1).start(priority=HI)

    def extra2(i):
        @pl.when(i == 80)
        def _():
            wait_all(wuv_buf.at[pl.ds(0, 4)], S_WUV)
            norm_b(3)

        @pl.when(i == 96)
        def _():
            wait_all(wbo_buf.at[pl.ds(0, 4)], S_WBO)

        @pl.when(i == 105)
        def _():
            wait_all(wo_buf.at[pl.ds(0, 4)], S_WO)
            out_ref[:, 512:] = rowsum(accb_ref[...]).astype(out_ref.dtype)

    def hook2(i, fl):
        @pl.when(i < 96)
        def _():
            ctx_item(i - 80, fl)

        @pl.when(jnp.logical_and(i >= 96, i < 104))
        def _():
            out_b_item(i - 96, fl)

        @pl.when(jnp.logical_and(i >= 105, i < 109))
        def _():
            out_a_item(i - 105, fl)

        @pl.when(jnp.logical_or(i == 104, i >= 109))
        def _():
            fl()

    lax.fori_loop(0, 16, make_main(high0, pin_to(wq_buf.at[4, 0:8, 0:128]), hook0, FLOAT_HOOK,
                                   _nop, False), 0)
    lax.fori_loop(16, 80, make_main(high1, pin1, hook1, FLOAT_HOOK, extra1, False), 0)
    lax.fori_loop(80, N_MAIN, make_main(high2, pin_to(wo_buf.at[8, 0:8, 0:128]), hook2,
                                        FLOAT_HOOK, extra2, True), 0)

    finalize_o(13)
    softmax_a()

    def g14_body(r, carry):
        s0 = (r & 3) * 4
        nx = r + 4
        for t in range(4):
            low_v8(0, r, t, s0 + t).wait()
            high_wo(6, 1, r * 32 + t * 8, 8, 0, 512, S_WO + 2).start(priority=HI)
            low_v8(nx >> 3, nx & 7, t, s0 + t).start(priority=LO)
        oacc_ref[...] = v_part(14, r)
        k_work(15, r)
        return carry
    lax.fori_loop(0, 8, g14_body, 0)

    finalize_o(14)
    softmax_a()

    def v15_body(r, carry):
        s0 = (r & 3) * 4
        for t in range(4):
            low_v8(1, r, t, s0 + t).wait()

            @pl.when(r < 4)
            def _():
                high_wo(6, 1, 256 + r * 64 + t * 16, 16, 0, 512, S_WO + 2).start(priority=HI)
                low_v8(1, r + 4, t, s0 + t).start(priority=LO)

            @pl.when(jnp.logical_and(r >= 4, r < 6))
            def _():
                low_wo(s0 + t, s0 + t).start(priority=LO)

            if t == 1:
                @pl.when(r == 1)
                def _():
                    wait_all(wo_buf.at[pl.ds(4, 2)], S_WO + 1)

                @pl.when(jnp.logical_and(r >= 1, r < 3))
                def _():
                    out_a_item(r + 3)

                @pl.when(r == 4)
                def _():
                    l = jnp.sum(psum_ref[...], axis=1, keepdims=True)
                    psum_ref[...] = jnp.broadcast_to(1.0 / l, (8, 128))
        oacc_ref[...] = v_part(15, r)
        return carry
    lax.fori_loop(0, 7, v15_body, 0)

    wait_all(wo_buf.at[pl.ds(6, 1)], S_WO + 2)
    for t in range(4):
        low_v8(1, 7, t, 12 + t).wait()
    oa_ref[3, 24:32, :] = v_part(15, 7) * psum_ref[...]
    o32 = oa_ref[3]
    acca_ref[...] = acca_ref[...] + out_part(o32, wo_buf.at[6], 0, 0, 4)
    for n in range(6):
        low_wo(n, n).wait()
    part = rowsum(acca_ref[...] + out_part(o32, wo_buf.at[7], 4, 0, 3))
    o_last = oa_ref[3, pl.ds(7, 4, stride=8), :].astype(BF16)
    for n in range(6, 8):
        low_wo(n, n).wait()
    out_ref[:, :512] = (part + _dot(o_last, wo_buf[7, 384:512, :])).astype(out_ref.dtype)


@jax.jit
def pallas_concat_heads__sliding_block_cached__compressed_kv_cla__decode_kernel(
    A_x: jax.Array,
    A_k_cache: jax.Array,
    A_v_cache: jax.Array,
    A_wq: jax.Array,
    A_wo: jax.Array,
    B_x: jax.Array,
    B_c_kv: jax.Array,
    B_w_q: jax.Array,
    B_w_uk: jax.Array,
    B_w_uv: jax.Array,
    B_w_o: jax.Array,
):
    B, Sq, D = A_x.shape
    _, H, Sk, Dh = A_k_cache.shape
    W = min(4096, max(256, Sk // 4))
    assert (B, Sq, D, H, Sk, Dh, W) == (4, 1, 512, 32, 4096, 128, 1024)
    assert B_c_kv.shape == (4, 4096, 512) and B_w_q.shape == (512, 32, 128)

    def body(*refs):
        _kernel(*refs, win_off=Sk - W, scale=float(Dh) ** -0.5)

    vm = pltpu.VMEM
    scratch = [
        vm((2, 16, 1024, 128), BF16),
        vm((16, 1024, 512), BF16),
        vm((5, 128, 4096), BF16),
        vm((9, 512, 512), BF16),
        vm((4, 128, 4, 8, 128), BF16),
        vm((4, 128, 4, 8, 128), BF16),
        vm((5, 128, 4, 8, 128), BF16),
        vm((5, 2, 512, 512), BF16),
        vm((4, 512), BF16),
        vm((4, 512), BF16),
        vm((128, 1024), BF16),
        vm((32, 512), BF16),
        vm((2, 32, 2048), BF16),
        vm((4, 32, 128), F32),
        vm((8, 8, 128), F32),
        vm((8, 8, 128), F32),
        vm((8, 128), F32),
        vm((8, 128), F32),
        vm((4, 32, 128), F32),
        vm((4, 32, 128), F32),
        vm((4, 4, 4, 8, 128), F32),
        vm((8, 32, 512), F32),
        vm((32, 128), F32),
        vm((32, 128), F32),
        vm((32, 512), F32),
        vm((4, 4, 4, 8, 128), F32),
        vm((4, 32, 128), F32),
        vm((32, 512), F32),
        vm((32, 512), F32),
        pltpu.SemaphoreType.DMA((NS,)),
        pltpu.SemaphoreType.DMA((N_HSEM,)),
        pltpu.SemaphoreType.DMA((2,)),
    ]
    out = pl.pallas_call(
        body,
        out_shape=jax.ShapeDtypeStruct((B, 2 * D), A_x.dtype),
        in_specs=[pl.BlockSpec(memory_space=pl.ANY)] * 11,
        scratch_shapes=scratch,
        compiler_params=pltpu.CompilerParams(
            vmem_limit_bytes=64 * 1024 * 1024,
            disable_bounds_checks=True,
            disable_semaphore_checks=True,
        ),
    )(
        A_x.reshape(B, D),
        A_k_cache.reshape(B * H, Sk, Dh),
        A_v_cache.reshape(B * H, Sk, Dh),
        A_wq.reshape(4, 128, 4096),
        A_wo.reshape(8, 512, 512),
        B_x.reshape(B, D),
        B_c_kv.reshape(16, 1024, 512),
        B_w_q.reshape(4, 128, 4, 8, 128),
        B_w_uk.reshape(4, 128, 4, 8, 128),
        B_w_uv.reshape(4, 128, 4, 8, 128),
        B_w_o.reshape(4, 2, 512, 512),
    )
    return out.reshape(B, Sq, 2 * D)
```

```python
import jax
import jax.numpy as jnp
from jax import lax
import jax.experimental.pallas as pl
import jax.experimental.pallas.tpu as pltpu

F32 = jnp.float32
BF16 = jnp.bfloat16
_NT = (((1,), (1,)), ((), ()))
_NN = (((1,), (0,)), ((), ()))

LO, HI = 1, 0
NS = 16
N_MAIN = 112

S_WQ = 0
S_WBQ = 4
S_WUK = 5
S_WUV = 6
S_WBO = 7
S_WO = 8
N_HSEM = 11
NSPLIT = 6


def _dot(a, b):
    return lax.dot_general(a, b, _NN, preferred_element_type=F32)


def _dot_nt(a, b):
    return lax.dot_general(a, b, _NT, preferred_element_type=F32)


def _mo(x, m):
    return x if isinstance(x, int) else pl.multiple_of(x, m)


def _nop(_=None):
    return None


def _kernel(xa_hbm, k_hbm, v_hbm, wq_hbm, wo_hbm, xb_hbm, c_hbm, wbq_hbm, wuk_hbm,
            wuv_hbm, wbo_hbm, out_hbm,
            kvbuf, cbuf, wq_buf, wo_buf, wbq_buf, wuk_buf, wuv_buf, wbo_buf,
            xa_buf, xb_buf, e0_ref, xa32_ref, xexp_ref,
            qa_ref, sa_ref, pa_ref, psum_ref, oacc_ref, oa_ref,
            qb_ref, qabs_ref, sb_ref, mb_ref, lb_ref, cacc_ref, cc_ref, ctx_ref,
            acca_ref, accb_ref, olast_ref, part_ref, obuf,
            lsem, hsem, xsem, *, win_off, scale):

    def low_c(it, t, sem):
        row = _mo(it * 16 + (t >> 1) * 8, 8)
        col = (t & 1) * 256
        return pltpu.make_async_copy(
            c_hbm.at[:, pl.ds(row, 8), pl.ds(col, 256)],
            cbuf.at[:, pl.ds(row, 8), pl.ds(col, 256)],
            lsem.at[sem])

    def batch_of(g):
        return (g >> 1) & 3

    def hg_of(g):
        return (g >> 3) * 2 + (g & 1)

    def low16(src, kv, sg, r, t, sem):
        row = _mo(r * 128 + t * 16, 16)
        head = (sg & 3) * 32 + (sg >> 2) * 16
        return pltpu.make_async_copy(
            src.at[pl.ds(head, 16), pl.ds(_mo(win_off + row, 16), 16), :],
            kvbuf.at[kv, :, pl.ds(row, 16), :],
            lsem.at[sem])

    def low_v8(e, r, t, sem):
        row = _mo(r * 128 + t * 32, 32)
        return pltpu.make_async_copy(
            v_hbm.at[pl.ds(112 + e * 8, 8), pl.ds(_mo(win_off + row, 32), 32), :],
            kvbuf.at[1, pl.ds(e * 8, 8), pl.ds(row, 32), :],
            lsem.at[sem])

    def low_wo(n, sem):
        row = _mo(n * 64, 64)
        return pltpu.make_async_copy(
            wo_hbm.at[7, pl.ds(row, 64), :], wo_buf.at[7, pl.ds(row, 64), :], lsem.at[sem])

    def high_wq(row, col, cols, sem):
        row = _mo(row, 8)
        return pltpu.make_async_copy(
            wq_hbm.at[:, pl.ds(row, 8), pl.ds(col, cols)],
            wq_buf.at[:, pl.ds(row, 8), pl.ds(col, cols)], hsem.at[sem])

    def high_3d(src, dst, row, hg, nhg, sem):
        return pltpu.make_async_copy(
            src.at[:, row, pl.ds(hg, nhg)], dst.at[:, row, pl.ds(hg, nhg)], hsem.at[sem])

    def high_wbo(half, row, col):
        row = _mo(row, 8)
        return pltpu.make_async_copy(
            wbo_hbm.at[:, half, pl.ds(row, 8), pl.ds(col, 256)],
            wbo_buf.at[:, half, pl.ds(row, 8), pl.ds(col, 256)], hsem.at[S_WBO])

    def high_wo(p0, np_, row, rows, col, cols, sem):
        row = _mo(row, 8)
        return pltpu.make_async_copy(
            wo_hbm.at[pl.ds(p0, np_), pl.ds(row, rows), pl.ds(col, cols)],
            wo_buf.at[pl.ds(p0, np_), pl.ds(row, rows), pl.ds(col, cols)], hsem.at[sem])

    def out_copy(h):
        return pltpu.make_async_copy(
            obuf.at[h], out_hbm.at[:, pl.ds(h * 512, 512)], xsem.at[2 + h])

    def wait_all(buf, sem):
        pltpu.make_async_copy(buf, buf, hsem.at[sem]).wait()

    for r in range(2):
        for t in range(8):
            low16(k_hbm, 0, 0, r, t, r * 8 + t).start(priority=LO)
    cp_xa = pltpu.make_async_copy(xa_hbm, xa_buf, xsem.at[0])
    cp_xb = pltpu.make_async_copy(xb_hbm, xb_buf, xsem.at[1])
    cp_xa.start(priority=HI)
    cp_xb.start(priority=HI)

    row8 = lax.broadcasted_iota(jnp.int32, (8, 128), 0)
    row32 = lax.broadcasted_iota(jnp.int32, (32, 128), 0) & 7
    lane32 = lax.broadcasted_iota(jnp.int32, (32, 128), 1) & 7

    def e0_body(i, c):
        r0 = pl.multiple_of(i * 16, 16)
        rr = lax.broadcasted_iota(jnp.int32, (16, 1024), 0) + r0
        cc = lax.broadcasted_iota(jnp.int32, (16, 1024), 1) >> 3
        e0_ref[pl.ds(r0, 16), :] = jnp.where(rr == cc, 1.0, 0.0).astype(BF16)
        return c
    lax.fori_loop(0, 8, e0_body, 0)

    qa_ref[...] = jnp.zeros(qa_ref.shape, F32)
    qb_ref[...] = jnp.zeros(qb_ref.shape, F32)
    ctx_ref[...] = jnp.zeros(ctx_ref.shape, F32)
    acca_ref[...] = jnp.zeros(acca_ref.shape, F32)
    accb_ref[...] = jnp.zeros(accb_ref.shape, F32)
    mb_ref[...] = jnp.zeros(mb_ref.shape, F32)
    lb_ref[...] = jnp.zeros(lb_ref.shape, F32)
    cacc_ref[...] = jnp.zeros(cacc_ref.shape, F32)
    olast_ref[...] = jnp.zeros(olast_ref.shape, F32)
    part_ref[...] = jnp.zeros(part_ref.shape, F32)

    def expand(c32, fl=_nop):
        ce = _dot(c32.astype(BF16), e0_ref[...])
        fl()
        return jnp.concatenate(
            [jnp.where(row32 == lane32, ce[:, 128 * k:128 * k + 128], 0.0).astype(BF16)
             for k in range(8)], axis=1)

    def x_prep():
        cp_xa.wait()
        cp_xb.wait()
        xa = xa_buf[...].astype(F32)
        xb = xb_buf[...].astype(F32)
        xa32_ref[...] = jnp.concatenate(
            [jnp.broadcast_to(xa[b:b + 1, :], (8, 512)) for b in range(4)], axis=0).astype(BF16)
        xb32 = jnp.concatenate(
            [jnp.broadcast_to(xb[b:b + 1, :], (8, 512)) for b in range(4)], axis=0)
        for u in range(4):
            xexp_ref[u >> 1, :, (u & 1) * 1024:(u & 1) * 1024 + 1024] = expand(
                xb32[:, 128 * u:128 * u + 128])

    def qa_item(hg, half):
        col = pl.multiple_of(hg * 1024 + half * 512, 512)
        w = wq_buf[:, :, pl.ds(col, 512)].reshape(512, 512)
        r = _dot(xa32_ref[...], w)
        new = qa_ref[hg]
        for j in range(4):
            new = jnp.where(row32 == half * 4 + j, r[:, 128 * j:128 * j + 128], new)
        qa_ref[hg] = new

    def qb_item(n):
        hg = n >> 1
        half = n & 1
        w = wbq_buf[pl.ds(half * 2, 2), :, hg].reshape(2048, 128)
        qb_ref[hg] = qb_ref[hg] + _dot(xexp_ref[half], w)

    def qabs_item(n, fl):
        hg = n & 3
        u = n >> 2
        q = qb_ref[hg].astype(BF16)
        w = wuk_buf[u, :, hg].reshape(1024, 128)
        r = _dot_nt(q, w)
        fl()
        r = jnp.concatenate(
            [jnp.where(row32 == lane32, r[:, 128 * k:128 * k + 128], 0.0).astype(BF16)
             for k in range(8)], axis=1)
        qa = _dot_nt(r, e0_ref[...])
        for b in range(4):
            qabs_ref[u, b, hg] = qa[8 * b:8 * b + 8, :]

    def score_item(b, n, fl):
        qa = jnp.concatenate(
            [qabs_ref[u, b].reshape(32, 128).astype(BF16) for u in range(4)], axis=1)
        seg = b * 4 + (n >> 1)
        m = jnp.where(n == 0, -jnp.inf, mb_ref[...])
        for k in range(4):
            row = pl.multiple_of((n & 1) * 512 + k * 128, 128)
            s = _dot_nt(qa, cbuf[seg, pl.ds(row, 128), :])
            if k == 0:
                fl()
            sb_ref[n, :, 128 * k:128 * k + 128] = s
            m = jnp.maximum(m, s)
        mb_ref[...] = m

    def max_b():
        mb_ref[...] = jnp.broadcast_to(jnp.max(mb_ref[...], axis=1, keepdims=True), (32, 128))

    def pv_item(b, n, fl):
        m = mb_ref[...]
        ps = [jnp.exp((sb_ref[n, :, 128 * k:128 * k + 128] - m) * scale) for k in range(4)]
        first = n == 0
        lb_ref[...] = jnp.where(first, 0.0, lb_ref[...]) + ((ps[0] + ps[1]) + (ps[2] + ps[3]))
        seg = b * 4 + (n >> 1)
        acc = jnp.where(first, 0.0, cacc_ref[...])
        for k in range(4):
            row = pl.multiple_of((n & 1) * 512 + k * 128, 128)
            d = _dot(ps[k].astype(BF16), cbuf[seg, pl.ds(row, 128), :])
            if k == 0:
                fl()
            acc = acc + d
        cacc_ref[...] = acc

    def norm_b(b):
        inv = 1.0 / jnp.sum(lb_ref[...], axis=1, keepdims=True)
        res = cacc_ref[...] * inv
        for u in range(4):
            cc_ref[u, b] = res[:, 128 * u:128 * u + 128].reshape(4, 8, 128)

    def ctx_item(n, fl):
        hg = n >> 2
        u = n & 3
        c32 = jnp.concatenate([cc_ref[u, bb, hg] for bb in range(4)], axis=0)
        w = wuv_buf[u, :, hg].reshape(1024, 128)
        ctx_ref[hg] = ctx_ref[hg] + _dot(expand(c32, fl), w)

    def out_part(o32, w_half, j0, jj, nj, fl=_nop):
        acc = None
        for j in range(jj, jj + nj):
            d = _dot(jnp.where(row32 == j0 + j, o32, 0.0).astype(BF16),
                     w_half[j * 128:j * 128 + 128, :])
            if j == jj:
                fl()
            acc = d if acc is None else acc + d
        return acc

    def out_a_item(n, fl=_nop):
        acca_ref[...] = acca_ref[...] + out_part(
            oa_ref[n >> 1], wo_buf.at[n], (n & 1) * 4, 0, 4, fl)

    def out_b_item(n, fl=_nop):
        accb_ref[...] = accb_ref[...] + out_part(
            ctx_ref[n >> 1], wbo_buf.at[n >> 1, n & 1], (n & 1) * 4, 0, 4, fl)

    def rowsum(acc):
        return jnp.sum(acc.reshape(4, 8, 512), axis=1)

    def k_work(g, r):
        q = qa_ref[hg_of(g), pl.ds(_mo(batch_of(g) * 8, 8), 8), :].astype(BF16)
        row = pl.multiple_of(r * 128, 128)
        h0 = (g & 1) * 8
        s = jnp.zeros((8, 128), F32)
        for j in range(8):
            sj = _dot_nt(q, kvbuf[0, h0 + j, pl.ds(row, 128), :])
            s = jnp.where(row8 == j, sj, s)
        sa_ref[r] = s

    def v_part(g, r):
        p = pa_ref[r].astype(BF16)
        row = _mo(r * 128, 128)
        h0 = (g & 1) * 8
        o = jnp.zeros((8, 128), F32)
        for j in range(8):
            oj = _dot(p, kvbuf[1, h0 + j, pl.ds(row, 128), :])
            o = jnp.where(row8 == j, oj, o)
        return oacc_ref[...] + o

    def finalize_o(g):
        l = jnp.sum(psum_ref[...], axis=1, keepdims=True)
        oa_ref[hg_of(g), pl.ds(_mo(batch_of(g) * 8, 8), 8), :] = oacc_ref[...] * (1.0 / l)

    def softmax_a():
        s = sa_ref[...]
        m = jnp.max(jnp.max(s, axis=0), axis=1, keepdims=True)
        p = jnp.exp((s - m[None]) * scale)
        pa_ref[...] = p
        psum_ref[...] = jnp.sum(p, axis=0)
        oacc_ref[...] = jnp.zeros((8, 128), F32)

    def k0_tick(r, t, s0):
        low16(k_hbm, 0, 0, r, t, s0 + t).wait()
        high_wq(r * 16 + (t >> 2) * 8, (t & 3) * 512, 512, S_WQ).start(priority=HI)

    def k0a_body(r, carry):
        s0 = (r & 1) * 8
        for t in range(8):
            k0_tick(r, t, s0)
            low16(k_hbm, 0, 0, r + 2, t, s0 + t).start(priority=LO)
        return carry
    lax.fori_loop(0, 6, k0a_body, 0)

    x_prep()

    def k0b_body(r, carry):
        s0 = r * 8
        for t in range(8):
            k0_tick(r + 6, t, s0)
            low_c(r * 2 + (t >> 2), t & 3, s0 + t).start(priority=LO)
        return carry
    lax.fori_loop(0, 2, k0b_body, 0)

    def c0_body(it, carry):
        s0 = (it & 3) * 4
        for t in range(4):
            low_c(it, t, s0 + t).wait()
            high_3d(wbq_hbm, wbq_buf, it * 4 + t, 0, 4, S_WBQ).start(priority=HI)
            low_c(it + 4, t, s0 + t).start(priority=LO)

        @pl.when(it == 1)
        def _():
            wait_all(wq_buf.at[:, :, pl.ds(0, 2048)], S_WQ)

        @pl.when(jnp.logical_and(it >= 1, it < 5))
        def _():
            qa_item((it - 1) >> 1, (it - 1) & 1)

        @pl.when(jnp.logical_and(it >= 5, it < 13))
        def _():
            k_work(0, it - 5)

        @pl.when(it == 13)
        def _():
            softmax_a()
        return carry
    lax.fori_loop(0, 32, c0_body, 0)

    def c1_tick(it, t, s0):
        low_c(32 + it, t, s0 + t).wait()
        high_3d(wuk_hbm, wuk_buf, it * 4 + t, 0, 4, S_WUK).start(priority=HI)

    def c1_body(it, carry):
        s0 = (it & 3) * 4
        for t in range(4):
            c1_tick(it, t, s0)
            low_c(36 + it, t, s0 + t).start(priority=LO)

        @pl.when(it == 1)
        def _():
            wait_all(wbq_buf, S_WBQ)

        @pl.when(jnp.logical_and(it >= 1, it < 9))
        def _():
            qb_item(it - 1)
        return carry
    lax.fori_loop(0, 28, c1_body, 0)

    def c1b_body(r, carry):
        for t in range(8):
            c1_tick(28 + r * 2 + (t >> 2), t & 3, r * 8 + (t >> 2) * 4)
            low16(v_hbm, 1, 0, r, t, r * 8 + t).start(priority=LO)
        return carry
    lax.fori_loop(0, 2, c1b_body, 0)

    def make_main(high, hook, extra, last):
        def body(i, carry):
            g = i >> 3
            r = i & 7
            i2 = i + 2
            g2 = i2 >> 3
            r2 = i2 & 7
            sg2 = (g2 + 1) >> 1
            odd2 = (g2 & 1) == 1
            s0 = (i & 1) * 8
            kv = 1 - (g & 1)

            def tick(t, with_high=True):
                low16(k_hbm, kv, 0, r, t, s0 + t).wait()
                if with_high:
                    high(i, t)

                @pl.when(odd2)
                def _():
                    low16(k_hbm, 0, sg2, r2, t, s0 + t).start(priority=LO)

                if not last:
                    @pl.when(jnp.logical_not(odd2))
                    def _():
                        low16(v_hbm, 1, sg2, r2, t, s0 + t).start(priority=LO)
                else:
                    @pl.when(jnp.logical_and(jnp.logical_not(odd2), i2 < N_MAIN))
                    def _():
                        low16(v_hbm, 1, sg2, r2, t, s0 + t).start(priority=LO)

                    @pl.when(i2 >= N_MAIN)
                    def _():
                        low_v8(0, 2 * r2 + (t >> 2), t & 3, s0 + t).start(priority=LO)

            tick(0)
            tick(1)

            @pl.when(jnp.logical_and(r == 0, i > 0))
            def _():
                finalize_o(g - 1)
                softmax_a()

            extra(i)
            tick(2)
            tick(3)
            hook(i, lambda: high(i, 5))
            tick(4)
            tick(5, False)
            tick(6)
            tick(7)
            oacc_ref[...] = v_part(g, r)
            k_work(g + 1, r)
            return carry
        return body

    def high0(i, t):
        high_wq(i * 8, 2048 + t * 256, 256, S_WQ + 1).start(priority=HI)

    def hook0(i, fl):
        @pl.when(i == 0)
        def _():
            wait_all(wuk_buf, S_WUK)

        qabs_item(i, fl)

    def high1(i, t):
        @pl.when(i < 48)
        def _():
            high_3d(wuv_hbm, wuv_buf, (i - 16) * 4 + (t >> 1), (t & 1) * 2, 2,
                    S_WUV).start(priority=HI)

        @pl.when(i >= 48)
        def _():
            high_wbo((i >> 4) - 3, (i & 15) * 32 + (t >> 1) * 8, (t & 1) * 256).start(priority=HI)

    def extra1(i):
        n = i - 16

        @pl.when(i == 25)
        def _():
            wait_all(wq_buf.at[:, :, pl.ds(2048, 2048)], S_WQ + 1)

        @pl.when(jnp.logical_and(i >= 25, i < 29))
        def _():
            qa_item(2 + ((i - 25) >> 1), (i - 25) & 1)

        @pl.when((n & 15) == 8)
        def _():
            max_b()

        @pl.when(jnp.logical_and((n & 15) == 1, n > 16))
        def _():
            norm_b((n >> 4) - 1)

    def hook1(i, fl):
        n = i - 16

        @pl.when((n & 8) == 0)
        def _():
            score_item(n >> 4, n & 7, fl)

        @pl.when((n & 8) != 0)
        def _():
            pv_item(n >> 4, n & 7, fl)

    def high2(i, t):
        row = (i & 15) * 32 + (t >> 1) * 8

        @pl.when(i < 96)
        def _():
            high_wo(0, 4, row, 8, (t & 1) * 256, 256, S_WO).start(priority=HI)

        @pl.when(i >= 96)
        def _():
            high_wo(4, 2, row, 8, (t & 1) * 256, 256, S_WO + 1).start(priority=HI)

    def extra2(i):
        @pl.when(i == 80)
        def _():
            wait_all(wuv_buf, S_WUV)
            norm_b(3)

        @pl.when(i == 96)
        def _():
            wait_all(wbo_buf, S_WBO)

        @pl.when(i == 105)
        def _():
            wait_all(wo_buf.at[pl.ds(0, 4)], S_WO)
            obuf[1] = rowsum(accb_ref[...]).astype(obuf.dtype)
            out_copy(1).start(priority=HI)

    def hook2(i, fl):
        @pl.when(i < 96)
        def _():
            ctx_item(i - 80, fl)

        @pl.when(jnp.logical_and(i >= 96, i < 104))
        def _():
            out_b_item(i - 96, fl)

        @pl.when(jnp.logical_and(i >= 105, i < 109))
        def _():
            out_a_item(i - 105, fl)

        @pl.when(jnp.logical_or(i == 104, i >= 109))
        def _():
            fl()

    lax.fori_loop(0, 16, make_main(high0, hook0, _nop, False), 0)
    lax.fori_loop(16, 80, make_main(high1, hook1, extra1, False), 0)
    lax.fori_loop(80, N_MAIN, make_main(high2, hook2, extra2, True), 0)

    finalize_o(13)
    softmax_a()

    def g14_body(r, carry):
        s0 = (r & 3) * 4
        nx = r + 4
        for t in range(4):
            low_v8(0, r, t, s0 + t).wait()
            high_wo(6, 1, r * 32 + t * 8, 8, 0, 512, S_WO + 2).start(priority=HI)
            low_v8(nx >> 3, nx & 7, t, s0 + t).start(priority=LO)
        oacc_ref[...] = v_part(14, r)
        k_work(15, r)
        return carry
    lax.fori_loop(0, 8, g14_body, 0)

    finalize_o(14)
    softmax_a()

    def v15_body(r, carry):
        s0 = (r & 3) * 4
        for t in range(4):
            low_v8(1, r, t, s0 + t).wait()

            @pl.when(r < 4)
            def _():
                high_wo(6, 1, 256 + r * 64 + t * 16, 16, 0, 512, S_WO + 2).start(priority=HI)
                low_v8(1, r + 4, t, s0 + t).start(priority=LO)

            @pl.when(jnp.logical_and(r >= 4, r < 6))
            def _():
                low_wo(s0 + t, s0 + t).start(priority=LO)

            if t == 1:
                @pl.when(r == 1)
                def _():
                    wait_all(wo_buf.at[pl.ds(4, 2)], S_WO + 1)

                @pl.when(jnp.logical_and(r >= 1, r < 3))
                def _():
                    out_a_item(r + 3)

                @pl.when(r == 4)
                def _():
                    l = jnp.sum(psum_ref[...], axis=1, keepdims=True)
                    psum_ref[...] = jnp.broadcast_to(1.0 / l, (8, 128))
        oacc_ref[...] = v_part(15, r)
        return carry
    lax.fori_loop(0, 7, v15_body, 0)

    wait_all(wo_buf.at[pl.ds(6, 1)], S_WO + 2)
    for t in range(4):
        low_v8(1, 7, t, 12 + t).wait()
    oa_ref[3, 24:32, :] = v_part(15, 7) * psum_ref[...]
    for n in range(2):
        low_wo(n, n).wait()
    o32 = oa_ref[3]
    part_ref[0:4, :] = rowsum(acca_ref[...] + out_part(o32, wo_buf.at[6], 0, 0, 4)
                              + out_part(o32, wo_buf.at[7], 4, 0, 1))
    for j in range(5, 8):
        olast_ref[0:4, (j - 5) * 128:(j - 4) * 128] = o32.reshape(4, 8, 128)[:, j, :]
    for n in range(2, NSPLIT):
        low_wo(n, n).wait()
    k1 = NSPLIT * 64
    part_ref[...] = part_ref[...] + _dot(
        olast_ref[:, 0:k1 - 128].astype(BF16), wo_buf[7, 128:k1, :])
    lhs = olast_ref[:, k1 - 128:384].astype(BF16)
    for n in range(NSPLIT, 8):
        low_wo(n, n).wait()
    res = part_ref[...] + _dot(lhs, wo_buf[7, k1:512, :])
    obuf[0] = res[0:4, :].astype(obuf.dtype)
    out_copy(0).start(priority=HI)
    out_copy(1).wait()
    out_copy(0).wait()


@jax.jit
def pallas_concat_heads__sliding_block_cached__compressed_kv_cla__decode_kernel(
    A_x: jax.Array,
    A_k_cache: jax.Array,
    A_v_cache: jax.Array,
    A_wq: jax.Array,
    A_wo: jax.Array,
    B_x: jax.Array,
    B_c_kv: jax.Array,
    B_w_q: jax.Array,
    B_w_uk: jax.Array,
    B_w_uv: jax.Array,
    B_w_o: jax.Array,
):
    B, Sq, D = A_x.shape
    _, H, Sk, Dh = A_k_cache.shape
    W = min(4096, max(256, Sk // 4))
    assert (B, Sq, D, H, Sk, Dh, W) == (4, 1, 512, 32, 4096, 128, 1024)
    assert B_c_kv.shape == (4, 4096, 512) and B_w_q.shape == (512, 32, 128)

    def body(*refs):
        _kernel(*refs, win_off=Sk - W, scale=float(Dh) ** -0.5)

    vm = pltpu.VMEM
    scratch = [
        vm((2, 16, 1024, 128), BF16),
        vm((16, 1024, 512), BF16),
        vm((4, 128, 4096), BF16),
        vm((8, 512, 512), BF16),
        vm((4, 128, 4, 8, 128), BF16),
        vm((4, 128, 4, 8, 128), BF16),
        vm((4, 128, 4, 8, 128), BF16),
        vm((4, 2, 512, 512), BF16),
        vm((4, 512), BF16),
        vm((4, 512), BF16),
        vm((128, 1024), BF16),
        vm((32, 512), BF16),
        vm((2, 32, 2048), BF16),
        vm((4, 32, 128), F32),
        vm((8, 8, 128), F32),
        vm((8, 8, 128), F32),
        vm((8, 128), F32),
        vm((8, 128), F32),
        vm((4, 32, 128), F32),
        vm((4, 32, 128), F32),
        vm((4, 4, 4, 8, 128), F32),
        vm((8, 32, 512), F32),
        vm((32, 128), F32),
        vm((32, 128), F32),
        vm((32, 512), F32),
        vm((4, 4, 4, 8, 128), F32),
        vm((4, 32, 128), F32),
        vm((32, 512), F32),
        vm((32, 512), F32),
        vm((8, 384), F32),
        vm((8, 512), F32),
        vm((2, 4, 512), A_x.dtype),
        pltpu.SemaphoreType.DMA((NS,)),
        pltpu.SemaphoreType.DMA((N_HSEM,)),
        pltpu.SemaphoreType.DMA((4,)),
    ]
    out = pl.pallas_call(
        body,
        out_shape=jax.ShapeDtypeStruct((B, 2 * D), A_x.dtype),
        in_specs=[pl.BlockSpec(memory_space=pl.ANY)] * 11,
        out_specs=pl.BlockSpec(memory_space=pl.ANY),
        scratch_shapes=scratch,
        compiler_params=pltpu.CompilerParams(
            vmem_limit_bytes=64 * 1024 * 1024,
            disable_bounds_checks=True,
            disable_semaphore_checks=True,
        ),
    )(
        A_x.reshape(B, D),
        A_k_cache.reshape(B * H, Sk, Dh),
        A_v_cache.reshape(B * H, Sk, Dh),
        A_wq.reshape(4, 128, 4096),
        A_wo.reshape(8, 512, 512),
        B_x.reshape(B, D),
        B_c_kv.reshape(16, 1024, 512),
        B_w_q.reshape(4, 128, 4, 8, 128),
        B_w_uk.reshape(4, 128, 4, 8, 128),
        B_w_uv.reshape(4, 128, 4, 8, 128),
        B_w_o.reshape(4, 2, 512, 512),
    )
    return out.reshape(B, Sq, 2 * D)
```

```python
import jax
import jax.numpy as jnp
from jax import lax
import jax.experimental.pallas as pl
import jax.experimental.pallas.tpu as pltpu

F32 = jnp.float32
BF16 = jnp.bfloat16
_NT = (((1,), (1,)), ((), ()))
_NN = (((1,), (0,)), ((), ()))

LO, HI = 1, 0
NS = 16
N_MAIN = 112

S_WQ = 0
S_WBQ = 4
S_WUK = 5
S_WUV = 6
S_WBO = 7
S_WO = 8
N_HSEM = 11
NSPLIT = 6
NBIG = 3


def _dot(a, b):
    return lax.dot_general(a, b, _NN, preferred_element_type=F32)


def _dot_nt(a, b):
    return lax.dot_general(a, b, _NT, preferred_element_type=F32)


def _mo(x, m):
    return x if isinstance(x, int) else pl.multiple_of(x, m)


def _nop(_=None):
    return None


def _kernel(xa_hbm, k_hbm, v_hbm, wq_hbm, wo_hbm, xb_hbm, c_hbm, wbq_hbm, wuk_hbm,
            wuv_hbm, wbo_hbm, out_hbm,
            kvbuf, cbuf, wq_buf, wo_buf, wbq_buf, wuk_buf, wuv_buf, wbo_buf,
            xa_buf, xb_buf, e0_ref, xa32_ref, xexp_ref,
            qa_ref, sa_ref, pa_ref, psum_ref, oacc_ref, oa_ref,
            qb_ref, qabs_ref, sb_ref, mb_ref, lb_ref, cacc_ref, cc_ref, ctx_ref,
            acca_ref, accb_ref, olast_ref, part_ref, obuf,
            lsem, hsem, xsem, *, win_off, scale):

    def low_c(it, t, sem):
        row = _mo(it * 16 + (t >> 1) * 8, 8)
        col = (t & 1) * 256
        return pltpu.make_async_copy(
            c_hbm.at[:, pl.ds(row, 8), pl.ds(col, 256)],
            cbuf.at[:, pl.ds(row, 8), pl.ds(col, 256)],
            lsem.at[sem])

    def batch_of(g):
        return (g >> 1) & 3

    def hg_of(g):
        return (g >> 3) * 2 + (g & 1)

    def low16(src, kv, sg, r, t, sem):
        row = _mo(r * 128 + t * 16, 16)
        head = (sg & 3) * 32 + (sg >> 2) * 16
        return pltpu.make_async_copy(
            src.at[pl.ds(head, 16), pl.ds(_mo(win_off + row, 16), 16), :],
            kvbuf.at[kv, :, pl.ds(row, 16), :],
            lsem.at[sem])

    def low_v8(e, r, t, sem):
        row = _mo(r * 128 + t * 32, 32)
        return pltpu.make_async_copy(
            v_hbm.at[pl.ds(112 + e * 8, 8), pl.ds(_mo(win_off + row, 32), 32), :],
            kvbuf.at[1, pl.ds(e * 8, 8), pl.ds(row, 32), :],
            lsem.at[sem])

    def low_wo(n, sem):
        row = _mo(n * 64, 64)
        return pltpu.make_async_copy(
            wo_hbm.at[7, pl.ds(row, 64), :], wo_buf.at[7, pl.ds(row, 64), :], lsem.at[sem])

    def high_wq(row, col, cols, sem):
        row = _mo(row, 8)
        return pltpu.make_async_copy(
            wq_hbm.at[:, pl.ds(row, 8), pl.ds(col, cols)],
            wq_buf.at[:, pl.ds(row, 8), pl.ds(col, cols)], hsem.at[sem])

    def high_3d(src, dst, row, hg, nhg, sem):
        return pltpu.make_async_copy(
            src.at[:, row, pl.ds(hg, nhg)], dst.at[:, row, pl.ds(hg, nhg)], hsem.at[sem])

    def high_wbo(half, row, col):
        row = _mo(row, 8)
        return pltpu.make_async_copy(
            wbo_hbm.at[:, half, pl.ds(row, 8), pl.ds(col, 256)],
            wbo_buf.at[:, half, pl.ds(row, 8), pl.ds(col, 256)], hsem.at[S_WBO])

    def high_wo(p0, np_, row, rows, col, cols, sem):
        row = _mo(row, 8)
        return pltpu.make_async_copy(
            wo_hbm.at[pl.ds(p0, np_), pl.ds(row, rows), pl.ds(col, cols)],
            wo_buf.at[pl.ds(p0, np_), pl.ds(row, rows), pl.ds(col, cols)], hsem.at[sem])

    def out_copy(h):
        return pltpu.make_async_copy(
            obuf.at[h], out_hbm.at[:, pl.ds(h * 512, 512)], xsem.at[2 + h])

    def wait_all(buf, sem):
        pltpu.make_async_copy(buf, buf, hsem.at[sem]).wait()

    for r in range(2):
        for t in range(8):
            low16(k_hbm, 0, 0, r, t, r * 8 + t).start(priority=LO)
    cp_xa = pltpu.make_async_copy(xa_hbm, xa_buf, xsem.at[0])
    cp_xb = pltpu.make_async_copy(xb_hbm, xb_buf, xsem.at[1])
    cp_xa.start(priority=HI)
    cp_xb.start(priority=HI)

    row8 = lax.broadcasted_iota(jnp.int32, (8, 128), 0)
    row32 = lax.broadcasted_iota(jnp.int32, (32, 128), 0) & 7
    lane32 = lax.broadcasted_iota(jnp.int32, (32, 128), 1) & 7

    def e0_body(i, c):
        r0 = pl.multiple_of(i * 16, 16)
        rr = lax.broadcasted_iota(jnp.int32, (16, 1024), 0) + r0
        cc = lax.broadcasted_iota(jnp.int32, (16, 1024), 1) >> 3
        e0_ref[pl.ds(r0, 16), :] = jnp.where(rr == cc, 1.0, 0.0).astype(BF16)
        return c
    lax.fori_loop(0, 8, e0_body, 0)

    qa_ref[...] = jnp.zeros(qa_ref.shape, F32)
    qb_ref[...] = jnp.zeros(qb_ref.shape, F32)
    ctx_ref[...] = jnp.zeros(ctx_ref.shape, F32)
    acca_ref[...] = jnp.zeros(acca_ref.shape, F32)
    accb_ref[...] = jnp.zeros(accb_ref.shape, F32)
    mb_ref[...] = jnp.zeros(mb_ref.shape, F32)
    lb_ref[...] = jnp.zeros(lb_ref.shape, F32)
    cacc_ref[...] = jnp.zeros(cacc_ref.shape, F32)
    olast_ref[...] = jnp.zeros(olast_ref.shape, F32)
    part_ref[...] = jnp.zeros(part_ref.shape, F32)

    def expand(c32, fl=_nop):
        ce = _dot(c32.astype(BF16), e0_ref[...])
        fl()
        return jnp.concatenate(
            [jnp.where(row32 == lane32, ce[:, 128 * k:128 * k + 128], 0.0).astype(BF16)
             for k in range(8)], axis=1)

    def x_prep():
        cp_xa.wait()
        cp_xb.wait()
        xa = xa_buf[...].astype(F32)
        xb = xb_buf[...].astype(F32)
        xa32_ref[...] = jnp.concatenate(
            [jnp.broadcast_to(xa[b:b + 1, :], (8, 512)) for b in range(4)], axis=0).astype(BF16)
        xb32 = jnp.concatenate(
            [jnp.broadcast_to(xb[b:b + 1, :], (8, 512)) for b in range(4)], axis=0)
        for u in range(4):
            xexp_ref[u >> 1, :, (u & 1) * 1024:(u & 1) * 1024 + 1024] = expand(
                xb32[:, 128 * u:128 * u + 128])

    def qa_item(hg, half):
        col = pl.multiple_of(hg * 1024 + half * 512, 512)
        w = wq_buf[:, :, pl.ds(col, 512)].reshape(512, 512)
        r = _dot(xa32_ref[...], w)
        new = qa_ref[hg]
        for j in range(4):
            new = jnp.where(row32 == half * 4 + j, r[:, 128 * j:128 * j + 128], new)
        qa_ref[hg] = new

    def qb_item(n):
        hg = n >> 1
        half = n & 1
        w = wbq_buf[pl.ds(half * 2, 2), :, hg].reshape(2048, 128)
        qb_ref[hg] = qb_ref[hg] + _dot(xexp_ref[half], w)

    def qabs_item(n, fl):
        hg = n & 3
        u = n >> 2
        q = qb_ref[hg].astype(BF16)
        w = wuk_buf[u, :, hg].reshape(1024, 128)
        r = _dot_nt(q, w)
        fl()
        r = jnp.concatenate(
            [jnp.where(row32 == lane32, r[:, 128 * k:128 * k + 128], 0.0).astype(BF16)
             for k in range(8)], axis=1)
        qa = _dot_nt(r, e0_ref[...])
        for b in range(4):
            qabs_ref[u, b, hg] = qa[8 * b:8 * b + 8, :]

    def score_item(b, n, fl):
        qa = jnp.concatenate(
            [qabs_ref[u, b].reshape(32, 128).astype(BF16) for u in range(4)], axis=1)
        seg = b * 4 + (n >> 1)
        m = jnp.where(n == 0, -jnp.inf, mb_ref[...])
        for k in range(4):
            row = pl.multiple_of((n & 1) * 512 + k * 128, 128)
            s = _dot_nt(qa, cbuf[seg, pl.ds(row, 128), :])
            if k == 0:
                fl()
            sb_ref[n, :, 128 * k:128 * k + 128] = s
            m = jnp.maximum(m, s)
        mb_ref[...] = m

    def max_b():
        mb_ref[...] = jnp.broadcast_to(jnp.max(mb_ref[...], axis=1, keepdims=True), (32, 128))

    def pv_item(b, n, fl):
        m = mb_ref[...]
        ps = [jnp.exp((sb_ref[n, :, 128 * k:128 * k + 128] - m) * scale) for k in range(4)]
        first = n == 0
        lb_ref[...] = jnp.where(first, 0.0, lb_ref[...]) + ((ps[0] + ps[1]) + (ps[2] + ps[3]))
        seg = b * 4 + (n >> 1)
        acc = jnp.where(first, 0.0, cacc_ref[...])
        for k in range(4):
            row = pl.multiple_of((n & 1) * 512 + k * 128, 128)
            d = _dot(ps[k].astype(BF16), cbuf[seg, pl.ds(row, 128), :])
            if k == 0:
                fl()
            acc = acc + d
        cacc_ref[...] = acc

    def norm_b(b):
        inv = 1.0 / jnp.sum(lb_ref[...], axis=1, keepdims=True)
        res = cacc_ref[...] * inv
        for u in range(4):
            cc_ref[u, b] = res[:, 128 * u:128 * u + 128].reshape(4, 8, 128)

    def ctx_item(n, fl):
        hg = n >> 2
        u = n & 3
        c32 = jnp.concatenate([cc_ref[u, bb, hg] for bb in range(4)], axis=0)
        w = wuv_buf[u, :, hg].reshape(1024, 128)
        ctx_ref[hg] = ctx_ref[hg] + _dot(expand(c32, fl), w)

    def out_part(o32, w_half, j0, jj, nj, fl=_nop):
        acc = None
        for j in range(jj, jj + nj):
            d = _dot(jnp.where(row32 == j0 + j, o32, 0.0).astype(BF16),
                     w_half[j * 128:j * 128 + 128, :])
            if j == jj:
                fl()
            acc = d if acc is None else acc + d
        return acc

    def out_a_item(n, fl=_nop):
        acca_ref[...] = acca_ref[...] + out_part(
            oa_ref[n >> 1], wo_buf.at[n], (n & 1) * 4, 0, 4, fl)

    def out_b_item(n, fl=_nop):
        accb_ref[...] = accb_ref[...] + out_part(
            ctx_ref[n >> 1], wbo_buf.at[n >> 1, n & 1], (n & 1) * 4, 0, 4, fl)

    def rowsum(acc):
        return jnp.sum(acc.reshape(4, 8, 512), axis=1)

    def k_work(g, r):
        q = qa_ref[hg_of(g), pl.ds(_mo(batch_of(g) * 8, 8), 8), :].astype(BF16)
        row = pl.multiple_of(r * 128, 128)
        h0 = (g & 1) * 8
        s = jnp.zeros((8, 128), F32)
        for j in range(8):
            sj = _dot_nt(q, kvbuf[0, h0 + j, pl.ds(row, 128), :])
            s = jnp.where(row8 == j, sj, s)
        sa_ref[r] = s

    def v_part(g, r):
        p = pa_ref[r].astype(BF16)
        row = _mo(r * 128, 128)
        h0 = (g & 1) * 8
        o = jnp.zeros((8, 128), F32)
        for j in range(8):
            oj = _dot(p, kvbuf[1, h0 + j, pl.ds(row, 128), :])
            o = jnp.where(row8 == j, oj, o)
        return oacc_ref[...] + o

    def finalize_o(g):
        l = jnp.sum(psum_ref[...], axis=1, keepdims=True)
        oa_ref[hg_of(g), pl.ds(_mo(batch_of(g) * 8, 8), 8), :] = oacc_ref[...] * (1.0 / l)

    def softmax_a():
        s = sa_ref[...]
        m = jnp.max(jnp.max(s, axis=0), axis=1, keepdims=True)
        p = jnp.exp((s - m[None]) * scale)
        pa_ref[...] = p
        psum_ref[...] = jnp.sum(p, axis=0)
        oacc_ref[...] = jnp.zeros((8, 128), F32)

    def k0_tick(r, t, s0):
        low16(k_hbm, 0, 0, r, t, s0 + t).wait()
        high_wq(r * 16 + (t >> 2) * 8, (t & 3) * 512, 512, S_WQ).start(priority=HI)

    def k0a_body(r, carry):
        s0 = (r & 1) * 8
        for t in range(8):
            k0_tick(r, t, s0)
            low16(k_hbm, 0, 0, r + 2, t, s0 + t).start(priority=LO)
        return carry
    lax.fori_loop(0, 6, k0a_body, 0)

    x_prep()

    def k0b_body(r, carry):
        s0 = r * 8
        for t in range(8):
            k0_tick(r + 6, t, s0)
            low_c(r * 2 + (t >> 2), t & 3, s0 + t).start(priority=LO)
        return carry
    lax.fori_loop(0, 2, k0b_body, 0)

    def c0_body(it, carry):
        s0 = (it & 3) * 4
        for t in range(4):
            low_c(it, t, s0 + t).wait()
            high_3d(wbq_hbm, wbq_buf, it * 4 + t, 0, 4, S_WBQ).start(priority=HI)
            low_c(it + 4, t, s0 + t).start(priority=LO)

        @pl.when(it == 1)
        def _():
            wait_all(wq_buf.at[:, :, pl.ds(0, 2048)], S_WQ)

        @pl.when(jnp.logical_and(it >= 1, it < 5))
        def _():
            qa_item((it - 1) >> 1, (it - 1) & 1)

        @pl.when(jnp.logical_and(it >= 5, it < 13))
        def _():
            k_work(0, it - 5)

        @pl.when(it == 13)
        def _():
            softmax_a()
        return carry
    lax.fori_loop(0, 32, c0_body, 0)

    def c1_tick(it, t, s0):
        low_c(32 + it, t, s0 + t).wait()
        high_3d(wuk_hbm, wuk_buf, it * 4 + t, 0, 4, S_WUK).start(priority=HI)

    def c1_body(it, carry):
        s0 = (it & 3) * 4
        for t in range(4):
            c1_tick(it, t, s0)
            low_c(36 + it, t, s0 + t).start(priority=LO)

        @pl.when(it == 1)
        def _():
            wait_all(wbq_buf, S_WBQ)

        @pl.when(jnp.logical_and(it >= 1, it < 9))
        def _():
            qb_item(it - 1)
        return carry
    lax.fori_loop(0, 28, c1_body, 0)

    def c1b_body(r, carry):
        for t in range(8):
            c1_tick(28 + r * 2 + (t >> 2), t & 3, r * 8 + (t >> 2) * 4)
            low16(v_hbm, 1, 0, r, t, r * 8 + t).start(priority=LO)
        return carry
    lax.fori_loop(0, 2, c1b_body, 0)

    def make_main(high, hook, extra, last):
        def body(i, carry):
            g = i >> 3
            r = i & 7
            i2 = i + 2
            g2 = i2 >> 3
            r2 = i2 & 7
            sg2 = (g2 + 1) >> 1
            odd2 = (g2 & 1) == 1
            s0 = (i & 1) * 8
            kv = 1 - (g & 1)

            def tick(t, with_high=True):
                low16(k_hbm, kv, 0, r, t, s0 + t).wait()
                if with_high:
                    high(i, t)

                @pl.when(odd2)
                def _():
                    low16(k_hbm, 0, sg2, r2, t, s0 + t).start(priority=LO)

                if not last:
                    @pl.when(jnp.logical_not(odd2))
                    def _():
                        low16(v_hbm, 1, sg2, r2, t, s0 + t).start(priority=LO)
                else:
                    @pl.when(jnp.logical_and(jnp.logical_not(odd2), i2 < N_MAIN))
                    def _():
                        low16(v_hbm, 1, sg2, r2, t, s0 + t).start(priority=LO)

                    @pl.when(i2 >= N_MAIN)
                    def _():
                        low_v8(0, 2 * r2 + (t >> 2), t & 3, s0 + t).start(priority=LO)

            tick(0)
            tick(1)

            @pl.when(jnp.logical_and(r == 0, i > 0))
            def _():
                finalize_o(g - 1)
                softmax_a()

            extra(i)
            tick(2)
            tick(3)
            hook(i, lambda: high(i, 5))
            tick(4)
            tick(5, False)
            tick(6)
            tick(7)
            oacc_ref[...] = v_part(g, r)
            k_work(g + 1, r)
            return carry
        return body

    def high0(i, t):
        high_wq(i * 8, 2048 + t * 256, 256, S_WQ + 1).start(priority=HI)

    def hook0(i, fl):
        @pl.when(i == 0)
        def _():
            wait_all(wuk_buf, S_WUK)

        qabs_item(i, fl)

    def high1(i, t):
        @pl.when(i < 48)
        def _():
            high_3d(wuv_hbm, wuv_buf, (i - 16) * 4 + (t >> 1), (t & 1) * 2, 2,
                    S_WUV).start(priority=HI)

        @pl.when(i >= 48)
        def _():
            high_wbo((i >> 4) - 3, (i & 15) * 32 + (t >> 1) * 8, (t & 1) * 256).start(priority=HI)

    def extra1(i):
        n = i - 16

        @pl.when(i == 25)
        def _():
            wait_all(wq_buf.at[:, :, pl.ds(2048, 2048)], S_WQ + 1)

        @pl.when(jnp.logical_and(i >= 25, i < 29))
        def _():
            qa_item(2 + ((i - 25) >> 1), (i - 25) & 1)

        @pl.when((n & 15) == 8)
        def _():
            max_b()

        @pl.when(jnp.logical_and((n & 15) == 1, n > 16))
        def _():
            norm_b((n >> 4) - 1)

    def hook1(i, fl):
        n = i - 16

        @pl.when((n & 8) == 0)
        def _():
            score_item(n >> 4, n & 7, fl)

        @pl.when((n & 8) != 0)
        def _():
            pv_item(n >> 4, n & 7, fl)

    def high2(i, t):
        row = (i & 15) * 32 + (t >> 1) * 8

        @pl.when(i < 96)
        def _():
            high_wo(0, 4, row, 8, (t & 1) * 256, 256, S_WO).start(priority=HI)

        @pl.when(i >= 96)
        def _():
            high_wo(4, 2, row, 8, (t & 1) * 256, 256, S_WO + 1).start(priority=HI)

    def extra2(i):
        @pl.when(i == 80)
        def _():
            wait_all(wuv_buf, S_WUV)
            norm_b(3)

        @pl.when(i == 96)
        def _():
            wait_all(wbo_buf, S_WBO)

        @pl.when(i == 105)
        def _():
            wait_all(wo_buf.at[pl.ds(0, 4)], S_WO)
            obuf[1] = rowsum(accb_ref[...]).astype(obuf.dtype)
            out_copy(1).start(priority=HI)

    def hook2(i, fl):
        @pl.when(i < 96)
        def _():
            ctx_item(i - 80, fl)

        @pl.when(jnp.logical_and(i >= 96, i < 104))
        def _():
            out_b_item(i - 96, fl)

        @pl.when(jnp.logical_and(i >= 105, i < 109))
        def _():
            out_a_item(i - 105, fl)

        @pl.when(jnp.logical_or(i == 104, i >= 109))
        def _():
            fl()

    lax.fori_loop(0, 16, make_main(high0, hook0, _nop, False), 0)
    lax.fori_loop(16, 80, make_main(high1, hook1, extra1, False), 0)
    lax.fori_loop(80, N_MAIN, make_main(high2, hook2, extra2, True), 0)

    finalize_o(13)
    softmax_a()

    def g14_body(r, carry):
        s0 = (r & 3) * 4
        nx = r + 4
        for t in range(4):
            low_v8(0, r, t, s0 + t).wait()
            high_wo(6, 1, r * 32 + t * 8, 8, 0, 512, S_WO + 2).start(priority=HI)
            low_v8(nx >> 3, nx & 7, t, s0 + t).start(priority=LO)
        oacc_ref[...] = v_part(14, r)
        k_work(15, r)
        return carry
    lax.fori_loop(0, 8, g14_body, 0)

    finalize_o(14)
    softmax_a()

    def v15_body(r, carry):
        s0 = (r & 3) * 4
        for t in range(4):
            low_v8(1, r, t, s0 + t).wait()

            @pl.when(r < NBIG)
            def _():
                high_wo(6, 1, 256 + r * 64 + t * 16, 16, 0, 512, S_WO + 2).start(priority=HI)

            @pl.when(jnp.logical_and(r >= NBIG, r < 8 - NBIG))
            def _():
                high_wo(6, 1, 256 + NBIG * 32 + r * 32 + t * 8, 8, 0, 512,
                        S_WO + 2).start(priority=HI)

            @pl.when(r < 4)
            def _():
                low_v8(1, r + 4, t, s0 + t).start(priority=LO)

            @pl.when(jnp.logical_and(r >= 4, r < 6))
            def _():
                low_wo(s0 + t, s0 + t).start(priority=LO)

            if t == 1:
                @pl.when(r == 1)
                def _():
                    wait_all(wo_buf.at[pl.ds(4, 2)], S_WO + 1)

                @pl.when(jnp.logical_and(r >= 1, r < 3))
                def _():
                    out_a_item(r + 3)

                @pl.when(r == 4)
                def _():
                    l = jnp.sum(psum_ref[...], axis=1, keepdims=True)
                    psum_ref[...] = jnp.broadcast_to(1.0 / l, (8, 128))
        oacc_ref[...] = v_part(15, r)
        return carry
    lax.fori_loop(0, 7, v15_body, 0)

    for t in range(4):
        low_v8(1, 7, t, 12 + t).wait()
    oa_ref[3, 24:32, :] = v_part(15, 7) * psum_ref[...]
    wait_all(wo_buf.at[pl.ds(6, 1)], S_WO + 2)
    for n in range(2):
        low_wo(n, n).wait()
    o32 = oa_ref[3]
    part_ref[0:4, :] = rowsum(acca_ref[...] + out_part(o32, wo_buf.at[6], 0, 0, 4)
                              + out_part(o32, wo_buf.at[7], 4, 0, 1))
    for j in range(5, 8):
        olast_ref[0:4, (j - 5) * 128:(j - 4) * 128] = o32.reshape(4, 8, 128)[:, j, :]
    for n in range(2, NSPLIT):
        low_wo(n, n).wait()
    k1 = NSPLIT * 64
    part_ref[...] = part_ref[...] + _dot(
        olast_ref[:, 0:k1 - 128].astype(BF16), wo_buf[7, 128:k1, :])
    lhs = olast_ref[:, k1 - 128:384].astype(BF16)
    for n in range(NSPLIT, 8):
        low_wo(n, n).wait()
    res = part_ref[...] + _dot(lhs, wo_buf[7, k1:512, :])
    obuf[0] = res[0:4, :].astype(obuf.dtype)
    out_copy(0).start(priority=HI)
    out_copy(1).wait()
    out_copy(0).wait()


@jax.jit
def pallas_concat_heads__sliding_block_cached__compressed_kv_cla__decode_kernel(
    A_x: jax.Array,
    A_k_cache: jax.Array,
    A_v_cache: jax.Array,
    A_wq: jax.Array,
    A_wo: jax.Array,
    B_x: jax.Array,
    B_c_kv: jax.Array,
    B_w_q: jax.Array,
    B_w_uk: jax.Array,
    B_w_uv: jax.Array,
    B_w_o: jax.Array,
):
    B, Sq, D = A_x.shape
    _, H, Sk, Dh = A_k_cache.shape
    W = min(4096, max(256, Sk // 4))
    assert (B, Sq, D, H, Sk, Dh, W) == (4, 1, 512, 32, 4096, 128, 1024)
    assert B_c_kv.shape == (4, 4096, 512) and B_w_q.shape == (512, 32, 128)

    def body(*refs):
        _kernel(*refs, win_off=Sk - W, scale=float(Dh) ** -0.5)

    vm = pltpu.VMEM
    scratch = [
        vm((2, 16, 1024, 128), BF16),
        vm((16, 1024, 512), BF16),
        vm((4, 128, 4096), BF16),
        vm((8, 512, 512), BF16),
        vm((4, 128, 4, 8, 128), BF16),
        vm((4, 128, 4, 8, 128), BF16),
        vm((4, 128, 4, 8, 128), BF16),
        vm((4, 2, 512, 512), BF16),
        vm((4, 512), BF16),
        vm((4, 512), BF16),
        vm((128, 1024), BF16),
        vm((32, 512), BF16),
        vm((2, 32, 2048), BF16),
        vm((4, 32, 128), F32),
        vm((8, 8, 128), F32),
        vm((8, 8, 128), F32),
        vm((8, 128), F32),
        vm((8, 128), F32),
        vm((4, 32, 128), F32),
        vm((4, 32, 128), F32),
        vm((4, 4, 4, 8, 128), F32),
        vm((8, 32, 512), F32),
        vm((32, 128), F32),
        vm((32, 128), F32),
        vm((32, 512), F32),
        vm((4, 4, 4, 8, 128), F32),
        vm((4, 32, 128), F32),
        vm((32, 512), F32),
        vm((32, 512), F32),
        vm((8, 384), F32),
        vm((8, 512), F32),
        vm((2, 4, 512), A_x.dtype),
        pltpu.SemaphoreType.DMA((NS,)),
        pltpu.SemaphoreType.DMA((N_HSEM,)),
        pltpu.SemaphoreType.DMA((4,)),
    ]
    out = pl.pallas_call(
        body,
        out_shape=jax.ShapeDtypeStruct((B, 2 * D), A_x.dtype),
        in_specs=[pl.BlockSpec(memory_space=pl.ANY)] * 11,
        out_specs=pl.BlockSpec(memory_space=pl.ANY),
        scratch_shapes=scratch,
        compiler_params=pltpu.CompilerParams(
            vmem_limit_bytes=64 * 1024 * 1024,
            disable_bounds_checks=True,
            disable_semaphore_checks=True,
        ),
    )(
        A_x.reshape(B, D),
        A_k_cache.reshape(B * H, Sk, Dh),
        A_v_cache.reshape(B * H, Sk, Dh),
        A_wq.reshape(4, 128, 4096),
        A_wo.reshape(8, 512, 512),
        B_x.reshape(B, D),
        B_c_kv.reshape(16, 1024, 512),
        B_w_q.reshape(4, 128, 4, 8, 128),
        B_w_uk.reshape(4, 128, 4, 8, 128),
        B_w_uv.reshape(4, 128, 4, 8, 128),
        B_w_o.reshape(4, 2, 512, 512),
    )
    return out.reshape(B, Sq, 2 * D)
```

```python
import jax
import jax.numpy as jnp
from jax import lax
import jax.experimental.pallas as pl
import jax.experimental.pallas.tpu as pltpu

F32 = jnp.float32
BF16 = jnp.bfloat16
_NT = (((1,), (1,)), ((), ()))
_NN = (((1,), (0,)), ((), ()))

LO, HI = 1, 0
NS = 16
N_MAIN = 112

S_WQ = 0
S_WBQ = 4
S_WUK = 5
S_WUV = 6
S_WBO = 7
S_WO = 8
N_HSEM = 11
NSPLIT = 6
NBIG = 3


def _dot(a, b):
    return lax.dot_general(a, b, _NN, preferred_element_type=F32)


def _dot_nt(a, b):
    return lax.dot_general(a, b, _NT, preferred_element_type=F32)


def _mo(x, m):
    return x if isinstance(x, int) else pl.multiple_of(x, m)


def _nop(_=None):
    return None


def _kernel(xa_hbm, k_hbm, v_hbm, wq_hbm, wo_hbm, xb_hbm, c_hbm, wbq_hbm, wuk_hbm,
            wuv_hbm, wbo_hbm, out_hbm,
            kvbuf, cbuf, wq_buf, wo_buf, wbq_buf, wuk_buf, wuv_buf, wbo_buf,
            xa_buf, xb_buf, e0_ref, xa32_ref, xexp_ref,
            qa_ref, sa_ref, pa_ref, psum_ref, oacc_ref, oa_ref,
            qb_ref, qabs_ref, sb_ref, mb_ref, lb_ref, cacc_ref, cc_ref, ctx_ref,
            acca_ref, accb_ref, olast_ref, part_ref, obuf,
            lsem, hsem, xsem, *, win_off, scale):

    def low_c(it, t, sem):
        row = _mo(it * 16 + (t >> 1) * 8, 8)
        col = (t & 1) * 256
        return pltpu.make_async_copy(
            c_hbm.at[:, pl.ds(row, 8), pl.ds(col, 256)],
            cbuf.at[:, pl.ds(row, 8), pl.ds(col, 256)],
            lsem.at[sem])

    def batch_of(g):
        return (g >> 1) & 3

    def hg_of(g):
        return (g >> 3) * 2 + (g & 1)

    def low16(src, kv, sg, r, t, sem):
        row = _mo(r * 128 + t * 16, 16)
        head = (sg & 3) * 32 + (sg >> 2) * 16
        return pltpu.make_async_copy(
            src.at[pl.ds(head, 16), pl.ds(_mo(win_off + row, 16), 16), :],
            kvbuf.at[kv, :, pl.ds(row, 16), :],
            lsem.at[sem])

    def wait16(kv, r, t, sem):
        dst = kvbuf.at[kv, :, pl.ds(_mo(r * 128 + t * 16, 16), 16), :]
        pltpu.make_async_copy(dst, dst, lsem.at[sem]).wait()

    def low_v8(e, r, t, sem):
        row = _mo(r * 128 + t * 32, 32)
        return pltpu.make_async_copy(
            v_hbm.at[pl.ds(112 + e * 8, 8), pl.ds(_mo(win_off + row, 32), 32), :],
            kvbuf.at[1, pl.ds(e * 8, 8), pl.ds(row, 32), :],
            lsem.at[sem])

    def low_wo(n, sem):
        row = _mo(n * 64, 64)
        return pltpu.make_async_copy(
            wo_hbm.at[7, pl.ds(row, 64), :], wo_buf.at[7, pl.ds(row, 64), :], lsem.at[sem])

    def high_wq(row, col, cols, sem):
        row = _mo(row, 8)
        return pltpu.make_async_copy(
            wq_hbm.at[:, pl.ds(row, 8), pl.ds(col, cols)],
            wq_buf.at[:, pl.ds(row, 8), pl.ds(col, cols)], hsem.at[sem])

    def high_3d(src, dst, row, hg, nhg, sem):
        return pltpu.make_async_copy(
            src.at[:, row, pl.ds(hg, nhg)], dst.at[:, row, pl.ds(hg, nhg)], hsem.at[sem])

    def high_wbo(half, row, col):
        row = _mo(row, 8)
        return pltpu.make_async_copy(
            wbo_hbm.at[:, half, pl.ds(row, 8), pl.ds(col, 256)],
            wbo_buf.at[:, half, pl.ds(row, 8), pl.ds(col, 256)], hsem.at[S_WBO])

    def high_wo(p0, np_, row, rows, col, cols, sem):
        row = _mo(row, 8)
        return pltpu.make_async_copy(
            wo_hbm.at[pl.ds(p0, np_), pl.ds(row, rows), pl.ds(col, cols)],
            wo_buf.at[pl.ds(p0, np_), pl.ds(row, rows), pl.ds(col, cols)], hsem.at[sem])

    def out_copy(h):
        return pltpu.make_async_copy(
            obuf.at[h], out_hbm.at[:, pl.ds(h * 512, 512)], xsem.at[2 + h])

    def wait_all(buf, sem):
        pltpu.make_async_copy(buf, buf, hsem.at[sem]).wait()

    for r in range(2):
        for t in range(8):
            low16(k_hbm, 0, 0, r, t, r * 8 + t).start(priority=LO)
    cp_xa = pltpu.make_async_copy(xa_hbm, xa_buf, xsem.at[0])
    cp_xb = pltpu.make_async_copy(xb_hbm, xb_buf, xsem.at[1])
    cp_xa.start(priority=HI)
    cp_xb.start(priority=HI)

    row8 = lax.broadcasted_iota(jnp.int32, (8, 128), 0)
    row32 = lax.broadcasted_iota(jnp.int32, (32, 128), 0) & 7
    lane32 = lax.broadcasted_iota(jnp.int32, (32, 128), 1) & 7

    def e0_body(i, c):
        r0 = pl.multiple_of(i * 16, 16)
        rr = lax.broadcasted_iota(jnp.int32, (16, 1024), 0) + r0
        cc = lax.broadcasted_iota(jnp.int32, (16, 1024), 1) >> 3
        e0_ref[pl.ds(r0, 16), :] = jnp.where(rr == cc, 1.0, 0.0).astype(BF16)
        return c
    lax.fori_loop(0, 8, e0_body, 0)

    qa_ref[...] = jnp.zeros(qa_ref.shape, F32)
    qb_ref[...] = jnp.zeros(qb_ref.shape, F32)
    ctx_ref[...] = jnp.zeros(ctx_ref.shape, F32)
    acca_ref[...] = jnp.zeros(acca_ref.shape, F32)
    accb_ref[...] = jnp.zeros(accb_ref.shape, F32)
    mb_ref[...] = jnp.zeros(mb_ref.shape, F32)
    lb_ref[...] = jnp.zeros(lb_ref.shape, F32)
    cacc_ref[...] = jnp.zeros(cacc_ref.shape, F32)
    olast_ref[...] = jnp.zeros(olast_ref.shape, F32)
    part_ref[...] = jnp.zeros(part_ref.shape, F32)

    def expand(c32, fl=_nop):
        ce = _dot(c32.astype(BF16), e0_ref[...])
        fl()
        return jnp.concatenate(
            [jnp.where(row32 == lane32, ce[:, 128 * k:128 * k + 128], 0.0).astype(BF16)
             for k in range(8)], axis=1)

    def x_prep():
        cp_xa.wait()
        cp_xb.wait()
        xa = xa_buf[...].astype(F32)
        xb = xb_buf[...].astype(F32)
        xa32_ref[...] = jnp.concatenate(
            [jnp.broadcast_to(xa[b:b + 1, :], (8, 512)) for b in range(4)], axis=0).astype(BF16)
        xb32 = jnp.concatenate(
            [jnp.broadcast_to(xb[b:b + 1, :], (8, 512)) for b in range(4)], axis=0)
        for u in range(4):
            xexp_ref[u >> 1, :, (u & 1) * 1024:(u & 1) * 1024 + 1024] = expand(
                xb32[:, 128 * u:128 * u + 128])

    def qa_item(hg, half):
        col = pl.multiple_of(hg * 1024 + half * 512, 512)
        w = wq_buf[:, :, pl.ds(col, 512)].reshape(512, 512)
        r = _dot(xa32_ref[...], w)
        new = qa_ref[hg]
        for j in range(4):
            new = jnp.where(row32 == half * 4 + j, r[:, 128 * j:128 * j + 128], new)
        qa_ref[hg] = new

    def qb_item(n):
        hg = n >> 1
        half = n & 1
        w = wbq_buf[pl.ds(half * 2, 2), :, hg].reshape(2048, 128)
        qb_ref[hg] = qb_ref[hg] + _dot(xexp_ref[half], w)

    def qabs_item(n, fl):
        hg = n & 3
        u = n >> 2
        q = qb_ref[hg].astype(BF16)
        w = wuk_buf[u, :, hg].reshape(1024, 128)
        r = _dot_nt(q, w)
        fl()
        r = jnp.concatenate(
            [jnp.where(row32 == lane32, r[:, 128 * k:128 * k + 128], 0.0).astype(BF16)
             for k in range(8)], axis=1)
        qa = _dot_nt(r, e0_ref[...])
        for b in range(4):
            qabs_ref[u, b, hg] = qa[8 * b:8 * b + 8, :]

    def score_item(b, n, fl):
        qa = jnp.concatenate(
            [qabs_ref[u, b].reshape(32, 128).astype(BF16) for u in range(4)], axis=1)
        seg = b * 4 + (n >> 1)
        m = jnp.where(n == 0, -jnp.inf, mb_ref[...])
        for k in range(4):
            row = pl.multiple_of((n & 1) * 512 + k * 128, 128)
            s = _dot_nt(qa, cbuf[seg, pl.ds(row, 128), :])
            if k == 0:
                fl()
            sb_ref[n, :, 128 * k:128 * k + 128] = s
            m = jnp.maximum(m, s)
        mb_ref[...] = m

    def max_b():
        mb_ref[...] = jnp.broadcast_to(jnp.max(mb_ref[...], axis=1, keepdims=True), (32, 128))

    def pv_item(b, n, fl):
        m = mb_ref[...]
        ps = [jnp.exp((sb_ref[n, :, 128 * k:128 * k + 128] - m) * scale) for k in range(4)]
        first = n == 0
        lb_ref[...] = jnp.where(first, 0.0, lb_ref[...]) + ((ps[0] + ps[1]) + (ps[2] + ps[3]))
        seg = b * 4 + (n >> 1)
        acc = jnp.where(first, 0.0, cacc_ref[...])
        for k in range(4):
            row = pl.multiple_of((n & 1) * 512 + k * 128, 128)
            d = _dot(ps[k].astype(BF16), cbuf[seg, pl.ds(row, 128), :])
            if k == 0:
                fl()
            acc = acc + d
        cacc_ref[...] = acc

    def norm_b(b):
        inv = 1.0 / jnp.sum(lb_ref[...], axis=1, keepdims=True)
        res = cacc_ref[...] * inv
        for u in range(4):
            cc_ref[u, b] = res[:, 128 * u:128 * u + 128].reshape(4, 8, 128)

    def ctx_item(n, fl):
        hg = n >> 2
        u = n & 3
        c32 = jnp.concatenate([cc_ref[u, bb, hg] for bb in range(4)], axis=0)
        w = wuv_buf[u, :, hg].reshape(1024, 128)
        ctx_ref[hg] = ctx_ref[hg] + _dot(expand(c32, fl), w)

    def out_part(o32, w_half, j0, jj, nj, fl=_nop):
        acc = None
        for j in range(jj, jj + nj):
            d = _dot(jnp.where(row32 == j0 + j, o32, 0.0).astype(BF16),
                     w_half[j * 128:j * 128 + 128, :])
            if j == jj:
                fl()
            acc = d if acc is None else acc + d
        return acc

    def out_a_item(n, fl=_nop):
        acca_ref[...] = acca_ref[...] + out_part(
            oa_ref[n >> 1], wo_buf.at[n], (n & 1) * 4, 0, 4, fl)

    def out_b_item(n, fl=_nop):
        accb_ref[...] = accb_ref[...] + out_part(
            ctx_ref[n >> 1], wbo_buf.at[n >> 1, n & 1], (n & 1) * 4, 0, 4, fl)

    def rowsum(acc):
        return jnp.sum(acc.reshape(4, 8, 512), axis=1)

    def k_work(g, r):
        q = qa_ref[hg_of(g), pl.ds(_mo(batch_of(g) * 8, 8), 8), :].astype(BF16)
        row = pl.multiple_of(r * 128, 128)
        h0 = (g & 1) * 8
        s = jnp.zeros((8, 128), F32)
        for j in range(8):
            sj = _dot_nt(q, kvbuf[0, h0 + j, pl.ds(row, 128), :])
            s = jnp.where(row8 == j, sj, s)
        sa_ref[r] = s

    def v_part(g, r):
        p = pa_ref[r].astype(BF16)
        row = _mo(r * 128, 128)
        h0 = (g & 1) * 8
        o = jnp.zeros((8, 128), F32)
        for j in range(8):
            oj = _dot(p, kvbuf[1, h0 + j, pl.ds(row, 128), :])
            o = jnp.where(row8 == j, oj, o)
        return oacc_ref[...] + o

    def finalize_o(g):
        l = jnp.sum(psum_ref[...], axis=1, keepdims=True)
        oa_ref[hg_of(g), pl.ds(_mo(batch_of(g) * 8, 8), 8), :] = oacc_ref[...] * (1.0 / l)

    def softmax_a():
        s = sa_ref[...]
        m = jnp.max(jnp.max(s, axis=0), axis=1, keepdims=True)
        p = jnp.exp((s - m[None]) * scale)
        pa_ref[...] = p
        psum_ref[...] = jnp.sum(p, axis=0)
        oacc_ref[...] = jnp.zeros((8, 128), F32)

    def k0_tick(r, t, s0):
        low16(k_hbm, 0, 0, r, t, s0 + t).wait()
        high_wq(r * 16 + (t >> 2) * 8, (t & 3) * 512, 512, S_WQ).start(priority=HI)

    def k0a_body(r, carry):
        s0 = (r & 1) * 8
        for t in range(8):
            k0_tick(r, t, s0)
            low16(k_hbm, 0, 0, r + 2, t, s0 + t).start(priority=LO)
        return carry
    lax.fori_loop(0, 6, k0a_body, 0)

    x_prep()

    def k0b_body(r, carry):
        s0 = r * 8
        for t in range(8):
            k0_tick(r + 6, t, s0)
            low_c(r * 2 + (t >> 2), t & 3, s0 + t).start(priority=LO)
        return carry
    lax.fori_loop(0, 2, k0b_body, 0)

    def c0_body(it, carry):
        s0 = (it & 3) * 4
        for t in range(4):
            low_c(it, t, s0 + t).wait()
            high_3d(wbq_hbm, wbq_buf, it * 4 + t, 0, 4, S_WBQ).start(priority=HI)
            low_c(it + 4, t, s0 + t).start(priority=LO)

        @pl.when(it == 1)
        def _():
            wait_all(wq_buf.at[:, :, pl.ds(0, 2048)], S_WQ)

        @pl.when(jnp.logical_and(it >= 1, it < 5))
        def _():
            qa_item((it - 1) >> 1, (it - 1) & 1)

        @pl.when(jnp.logical_and(it >= 5, it < 13))
        def _():
            k_work(0, it - 5)

        @pl.when(it == 13)
        def _():
            softmax_a()
        return carry
    lax.fori_loop(0, 32, c0_body, 0)

    def c1_tick(it, t, s0):
        low_c(32 + it, t, s0 + t).wait()
        high_3d(wuk_hbm, wuk_buf, it * 4 + t, 0, 4, S_WUK).start(priority=HI)

    def c1_body(it, carry):
        s0 = (it & 3) * 4
        for t in range(4):
            c1_tick(it, t, s0)
            low_c(36 + it, t, s0 + t).start(priority=LO)

        @pl.when(it == 1)
        def _():
            wait_all(wbq_buf, S_WBQ)

        @pl.when(jnp.logical_and(it >= 1, it < 9))
        def _():
            qb_item(it - 1)
        return carry
    lax.fori_loop(0, 28, c1_body, 0)

    def c1b_body(r, carry):
        for t in range(8):
            c1_tick(28 + r * 2 + (t >> 2), t & 3, r * 8 + (t >> 2) * 4)
            low16(v_hbm, 1, 0, r, t, r * 8 + t).start(priority=LO)
        return carry
    lax.fori_loop(0, 2, c1b_body, 0)

    def make_main(high, hook, extra, last):
        def body(i, carry):
            g = i >> 3
            r = i & 7
            i2 = i + 2
            g2 = i2 >> 3
            r2 = i2 & 7
            sg2 = (g2 + 1) >> 1
            odd2 = (g2 & 1) == 1
            s0 = (i & 1) * 8
            kv = 1 - (g & 1)

            def tick(t, with_high=True):
                wait16(kv, r, t, s0 + t)
                if with_high:
                    high(i, t)

                @pl.when(odd2)
                def _():
                    low16(k_hbm, 0, sg2, r2, t, s0 + t).start(priority=LO)

                if not last:
                    @pl.when(jnp.logical_not(odd2))
                    def _():
                        low16(v_hbm, 1, sg2, r2, t, s0 + t).start(priority=LO)
                else:
                    @pl.when(jnp.logical_and(jnp.logical_not(odd2), i2 < N_MAIN))
                    def _():
                        low16(v_hbm, 1, sg2, r2, t, s0 + t).start(priority=LO)

                    @pl.when(i2 >= N_MAIN)
                    def _():
                        low_v8(0, 2 * r2 + (t >> 2), t & 3, s0 + t).start(priority=LO)

            tick(0)
            tick(1)

            @pl.when(jnp.logical_and(r == 0, i > 0))
            def _():
                finalize_o(g - 1)
                softmax_a()

            extra(i)
            tick(2)
            tick(3)
            hook(i, lambda: high(i, 5))
            tick(4)
            tick(5, False)
            tick(6)
            tick(7)
            oacc_ref[...] = v_part(g, r)
            k_work(g + 1, r)
            return carry
        return body

    def high0(i, t):
        high_wq(i * 8, 2048 + t * 256, 256, S_WQ + 1).start(priority=HI)

    def hook0(i, fl):
        @pl.when(i == 0)
        def _():
            wait_all(wuk_buf, S_WUK)

        qabs_item(i, fl)

    def high1(i, t):
        @pl.when(i < 48)
        def _():
            high_3d(wuv_hbm, wuv_buf, (i - 16) * 4 + (t >> 1), (t & 1) * 2, 2,
                    S_WUV).start(priority=HI)

        @pl.when(i >= 48)
        def _():
            high_wbo((i >> 4) - 3, (i & 15) * 32 + (t >> 1) * 8, (t & 1) * 256).start(priority=HI)

    def extra1(i):
        n = i - 16

        @pl.when(i == 25)
        def _():
            wait_all(wq_buf.at[:, :, pl.ds(2048, 2048)], S_WQ + 1)

        @pl.when(jnp.logical_and(i >= 25, i < 29))
        def _():
            qa_item(2 + ((i - 25) >> 1), (i - 25) & 1)

        @pl.when((n & 15) == 8)
        def _():
            max_b()

        @pl.when(jnp.logical_and((n & 15) == 1, n > 16))
        def _():
            norm_b((n >> 4) - 1)

    def hook1(i, fl):
        n = i - 16

        @pl.when((n & 8) == 0)
        def _():
            score_item(n >> 4, n & 7, fl)

        @pl.when((n & 8) != 0)
        def _():
            pv_item(n >> 4, n & 7, fl)

    def high2(i, t):
        row = (i & 15) * 32 + (t >> 1) * 8

        @pl.when(i < 96)
        def _():
            high_wo(0, 4, row, 8, (t & 1) * 256, 256, S_WO).start(priority=HI)

        @pl.when(i >= 96)
        def _():
            high_wo(4, 2, row, 8, (t & 1) * 256, 256, S_WO + 1).start(priority=HI)

    def extra2(i):
        @pl.when(i == 80)
        def _():
            wait_all(wuv_buf, S_WUV)
            norm_b(3)

        @pl.when(i == 96)
        def _():
            wait_all(wbo_buf, S_WBO)

        @pl.when(i == 105)
        def _():
            wait_all(wo_buf.at[pl.ds(0, 4)], S_WO)
            obuf[1] = rowsum(accb_ref[...]).astype(obuf.dtype)
            out_copy(1).start(priority=HI)

    def hook2(i, fl):
        @pl.when(i < 96)
        def _():
            ctx_item(i - 80, fl)

        @pl.when(jnp.logical_and(i >= 96, i < 104))
        def _():
            out_b_item(i - 96, fl)

        @pl.when(jnp.logical_and(i >= 105, i < 109))
        def _():
            out_a_item(i - 105, fl)

        @pl.when(jnp.logical_or(i == 104, i >= 109))
        def _():
            fl()

    lax.fori_loop(0, 16, make_main(high0, hook0, _nop, False), 0)
    lax.fori_loop(16, 80, make_main(high1, hook1, extra1, False), 0)
    lax.fori_loop(80, N_MAIN, make_main(high2, hook2, extra2, True), 0)

    finalize_o(13)
    softmax_a()

    def g14_body(r, carry):
        s0 = (r & 3) * 4
        nx = r + 4
        for t in range(4):
            low_v8(0, r, t, s0 + t).wait()
            high_wo(6, 1, r * 32 + t * 8, 8, 0, 512, S_WO + 2).start(priority=HI)
            low_v8(nx >> 3, nx & 7, t, s0 + t).start(priority=LO)
        oacc_ref[...] = v_part(14, r)
        k_work(15, r)
        return carry
    lax.fori_loop(0, 8, g14_body, 0)

    finalize_o(14)
    softmax_a()

    def v15_body(r, carry):
        s0 = (r & 3) * 4
        for t in range(4):
            low_v8(1, r, t, s0 + t).wait()

            @pl.when(r < NBIG)
            def _():
                high_wo(6, 1, 256 + r * 64 + t * 16, 16, 0, 512, S_WO + 2).start(priority=HI)

            @pl.when(jnp.logical_and(r >= NBIG, r < 8 - NBIG))
            def _():
                high_wo(6, 1, 256 + NBIG * 32 + r * 32 + t * 8, 8, 0, 512,
                        S_WO + 2).start(priority=HI)

            @pl.when(r < 4)
            def _():
                low_v8(1, r + 4, t, s0 + t).start(priority=LO)

            @pl.when(jnp.logical_and(r >= 4, r < 6))
            def _():
                low_wo(s0 + t, s0 + t).start(priority=LO)

            if t == 1:
                @pl.when(r == 1)
                def _():
                    wait_all(wo_buf.at[pl.ds(4, 2)], S_WO + 1)

                @pl.when(jnp.logical_and(r >= 1, r < 3))
                def _():
                    out_a_item(r + 3)

                @pl.when(r == 4)
                def _():
                    l = jnp.sum(psum_ref[...], axis=1, keepdims=True)
                    psum_ref[...] = jnp.broadcast_to(1.0 / l, (8, 128))
        oacc_ref[...] = v_part(15, r)
        return carry
    lax.fori_loop(0, 7, v15_body, 0)

    for t in range(4):
        low_v8(1, 7, t, 12 + t).wait()
    oa_ref[3, 24:32, :] = v_part(15, 7) * psum_ref[...]
    wait_all(wo_buf.at[pl.ds(6, 1)], S_WO + 2)
    for n in range(2):
        low_wo(n, n).wait()
    o32 = oa_ref[3]
    part_ref[0:4, :] = rowsum(acca_ref[...] + out_part(o32, wo_buf.at[6], 0, 0, 4)
                              + out_part(o32, wo_buf.at[7], 4, 0, 1))
    for j in range(5, 8):
        olast_ref[0:4, (j - 5) * 128:(j - 4) * 128] = o32.reshape(4, 8, 128)[:, j, :]
    for n in range(2, NSPLIT):
        low_wo(n, n).wait()
    k1 = NSPLIT * 64
    part_ref[...] = part_ref[...] + _dot(
        olast_ref[:, 0:k1 - 128].astype(BF16), wo_buf[7, 128:k1, :])
    lhs = olast_ref[:, k1 - 128:384].astype(BF16)
    for n in range(NSPLIT, 8):
        low_wo(n, n).wait()
    res = part_ref[...] + _dot(lhs, wo_buf[7, k1:512, :])
    obuf[0] = res[0:4, :].astype(obuf.dtype)
    out_copy(0).start(priority=HI)
    out_copy(1).wait()
    out_copy(0).wait()


@jax.jit
def pallas_concat_heads__sliding_block_cached__compressed_kv_cla__decode_kernel(
    A_x: jax.Array,
    A_k_cache: jax.Array,
    A_v_cache: jax.Array,
    A_wq: jax.Array,
    A_wo: jax.Array,
    B_x: jax.Array,
    B_c_kv: jax.Array,
    B_w_q: jax.Array,
    B_w_uk: jax.Array,
    B_w_uv: jax.Array,
    B_w_o: jax.Array,
):
    B, Sq, D = A_x.shape
    _, H, Sk, Dh = A_k_cache.shape
    W = min(4096, max(256, Sk // 4))
    assert (B, Sq, D, H, Sk, Dh, W) == (4, 1, 512, 32, 4096, 128, 1024)
    assert B_c_kv.shape == (4, 4096, 512) and B_w_q.shape == (512, 32, 128)

    def body(*refs):
        _kernel(*refs, win_off=Sk - W, scale=float(Dh) ** -0.5)

    vm = pltpu.VMEM
    scratch = [
        vm((2, 16, 1024, 128), BF16),
        vm((16, 1024, 512), BF16),
        vm((4, 128, 4096), BF16),
        vm((8, 512, 512), BF16),
        vm((4, 128, 4, 8, 128), BF16),
        vm((4, 128, 4, 8, 128), BF16),
        vm((4, 128, 4, 8, 128), BF16),
        vm((4, 2, 512, 512), BF16),
        vm((4, 512), BF16),
        vm((4, 512), BF16),
        vm((128, 1024), BF16),
        vm((32, 512), BF16),
        vm((2, 32, 2048), BF16),
        vm((4, 32, 128), F32),
        vm((8, 8, 128), F32),
        vm((8, 8, 128), F32),
        vm((8, 128), F32),
        vm((8, 128), F32),
        vm((4, 32, 128), F32),
        vm((4, 32, 128), F32),
        vm((4, 4, 4, 8, 128), F32),
        vm((8, 32, 512), F32),
        vm((32, 128), F32),
        vm((32, 128), F32),
        vm((32, 512), F32),
        vm((4, 4, 4, 8, 128), F32),
        vm((4, 32, 128), F32),
        vm((32, 512), F32),
        vm((32, 512), F32),
        vm((8, 384), F32),
        vm((8, 512), F32),
        vm((2, 4, 512), A_x.dtype),
        pltpu.SemaphoreType.DMA((NS,)),
        pltpu.SemaphoreType.DMA((N_HSEM,)),
        pltpu.SemaphoreType.DMA((4,)),
    ]
    out = pl.pallas_call(
        body,
        out_shape=jax.ShapeDtypeStruct((B, 2 * D), A_x.dtype),
        in_specs=[pl.BlockSpec(memory_space=pl.ANY)] * 11,
        out_specs=pl.BlockSpec(memory_space=pl.ANY),
        scratch_shapes=scratch,
        compiler_params=pltpu.CompilerParams(
            vmem_limit_bytes=64 * 1024 * 1024,
            disable_bounds_checks=True,
            disable_semaphore_checks=True,
        ),
    )(
        A_x.reshape(B, D),
        A_k_cache.reshape(B * H, Sk, Dh),
        A_v_cache.reshape(B * H, Sk, Dh),
        A_wq.reshape(4, 128, 4096),
        A_wo.reshape(8, 512, 512),
        B_x.reshape(B, D),
        B_c_kv.reshape(16, 1024, 512),
        B_w_q.reshape(4, 128, 4, 8, 128),
        B_w_uk.reshape(4, 128, 4, 8, 128),
        B_w_uv.reshape(4, 128, 4, 8, 128),
        B_w_o.reshape(4, 2, 512, 512),
    )
    return out.reshape(B, Sq, 2 * D)
```

```python
import jax
import jax.numpy as jnp
from jax import lax
import jax.experimental.pallas as pl
import jax.experimental.pallas.tpu as pltpu

F32 = jnp.float32
BF16 = jnp.bfloat16
_NT = (((1,), (1,)), ((), ()))
_NN = (((1,), (0,)), ((), ()))

LO, HI = 1, 0
NS = 16
N_MAIN = 112

S_WQ = 0
S_WBQ = 4
S_WUK = 5
S_WUV = 6
S_WBO = 7
S_WO = 8
N_HSEM = 11
NSPLIT = 6
NBIG = 3
ROT = 14
ROTC = ((32 - ROT) % 32) * 128
_PW = ROT // 4
WO_RUNS = [(a, n) for a, n in ((0, _PW), (_PW, 1), (_PW + 1, 3 - _PW)) if n > 0] if ROT else [(0, 4)]


def _dot(a, b):
    return lax.dot_general(a, b, _NN, preferred_element_type=F32)


def _dot_nt(a, b):
    return lax.dot_general(a, b, _NT, preferred_element_type=F32)


def _mo(x, m):
    return x if isinstance(x, int) else pl.multiple_of(x, m)


def _nop(_=None):
    return None


def _kernel(xa_hbm, k_hbm, v_hbm, wq_hbm, wo_hbm, xb_hbm, c_hbm, wbq_hbm, wuk_hbm,
            wuv_hbm, wbo_hbm, out_hbm,
            kvbuf, cbuf, wq_buf, wo_buf, wbq_buf, wuk_buf, wuv_buf, wbo_buf,
            xa_buf, xb_buf, e0_ref, xa32_ref, xexp_ref,
            qa_ref, sa_ref, pa_ref, psum_ref, oacc_ref, oa_ref,
            qb_ref, qabs_ref, sb_ref, mb_ref, lb_ref, cacc_ref, cc_ref, ctx_ref,
            acca_ref, accb_ref, olast_ref, part_ref, obuf,
            lsem, hsem, xsem, *, win_off, scale):

    def low_c(it, t, sem):
        row = _mo(it * 16 + (t >> 1) * 8, 8)
        col = (t & 1) * 256
        return pltpu.make_async_copy(
            c_hbm.at[:, pl.ds(row, 8), pl.ds(col, 256)],
            cbuf.at[:, pl.ds(row, 8), pl.ds(col, 256)],
            lsem.at[sem])

    def batch_of(g):
        return (g >> 1) & 3

    def hg_of(g):
        return (g >> 3) * 2 + (g & 1)

    def nprev_of(g):
        n = ROT - hg_of(g) * 8
        return max(0, min(8, n)) if isinstance(n, int) else jnp.clip(n, 0, 8)

    def low_heads(src, kv, head, slot, n, r, t, sem):
        row = _mo(r * 128 + t * 16, 16)
        return pltpu.make_async_copy(
            src.at[pl.ds(head, n), pl.ds(_mo(win_off + row, 16), 16), :],
            kvbuf.at[kv, pl.ds(slot, n), pl.ds(row, 16), :],
            lsem.at[sem])

    def start16(src, kv, sg, r, t, sem):
        head = (sg & 3) * 32 + (sg >> 2) * 16 - ROT
        low_heads(src, kv, head, 0, 16, r, t, sem).start(priority=LO)

    def start16_first(src, kv, r, t, sem):
        if ROT:
            low_heads(src, kv, 128 - ROT, 0, ROT, r, t, sem).start(priority=LO)
        low_heads(src, kv, 0, ROT, 16 - ROT, r, t, sem).start(priority=LO)

    def wait16(kv, r, t, sem):
        dst = kvbuf.at[kv, :, pl.ds(_mo(r * 128 + t * 16, 16), 16), :]
        pltpu.make_async_copy(dst, dst, lsem.at[sem]).wait()

    def low_v8(e, r, t, sem):
        row = _mo(r * 128 + t * 32, 32)
        return pltpu.make_async_copy(
            v_hbm.at[pl.ds(112 - ROT + e * 8, 8), pl.ds(_mo(win_off + row, 32), 32), :],
            kvbuf.at[1, pl.ds(e * 8, 8), pl.ds(row, 32), :],
            lsem.at[sem])

    def wo_copy(p0, np_, row, rows, col, cols, sem):
        flat = (p0 * 512 + row + ROTC) & 4095
        return pltpu.make_async_copy(
            wo_hbm.at[pl.ds(flat >> 9, np_), pl.ds(_mo(flat & 511, 8), rows), pl.ds(col, cols)],
            wo_buf.at[pl.ds(p0, np_), pl.ds(_mo(row, 8), rows), pl.ds(col, cols)], sem)

    def low_wo(n, sem):
        return wo_copy(7, 1, n * 64, 64, 0, 512, lsem.at[sem])

    def start_wq(row, col, cols, sem):
        row = _mo(row, 8)
        src = (col + ROTC) % 4096
        first = min(cols, 4096 - src)
        for c0, s0, n in ((col, src, first), (col + first, 0, cols - first)):
            if n:
                pltpu.make_async_copy(
                    wq_hbm.at[:, pl.ds(row, 8), pl.ds(s0, n)],
                    wq_buf.at[:, pl.ds(row, 8), pl.ds(c0, n)], hsem.at[sem]).start(priority=HI)

    def high_3d(src, dst, row, hg, nhg, sem):
        return pltpu.make_async_copy(
            src.at[:, row, pl.ds(hg, nhg)], dst.at[:, row, pl.ds(hg, nhg)], hsem.at[sem])

    def high_wbo(half, row, col):
        row = _mo(row, 8)
        return pltpu.make_async_copy(
            wbo_hbm.at[:, half, pl.ds(row, 8), pl.ds(col, 256)],
            wbo_buf.at[:, half, pl.ds(row, 8), pl.ds(col, 256)], hsem.at[S_WBO])

    def high_wo(p0, np_, row, rows, col, cols, sem):
        return wo_copy(p0, np_, row, rows, col, cols, hsem.at[sem])

    def out_copy(h):
        return pltpu.make_async_copy(
            obuf.at[h], out_hbm.at[:, pl.ds(h * 512, 512)], xsem.at[2 + h])

    def wait_all(buf, sem):
        pltpu.make_async_copy(buf, buf, hsem.at[sem]).wait()

    for r in range(2):
        for t in range(8):
            start16_first(k_hbm, 0, r, t, r * 8 + t)
    cp_xa = pltpu.make_async_copy(xa_hbm, xa_buf, xsem.at[0])
    cp_xb = pltpu.make_async_copy(xb_hbm, xb_buf, xsem.at[1])
    cp_xa.start(priority=HI)
    cp_xb.start(priority=HI)

    row8 = lax.broadcasted_iota(jnp.int32, (8, 128), 0)
    row32 = lax.broadcasted_iota(jnp.int32, (32, 128), 0) & 7
    lane32 = lax.broadcasted_iota(jnp.int32, (32, 128), 1) & 7

    def e0_body(i, c):
        r0 = pl.multiple_of(i * 16, 16)
        rr = lax.broadcasted_iota(jnp.int32, (16, 1024), 0) + r0
        cc = lax.broadcasted_iota(jnp.int32, (16, 1024), 1) >> 3
        e0_ref[pl.ds(r0, 16), :] = jnp.where(rr == cc, 1.0, 0.0).astype(BF16)
        return c
    lax.fori_loop(0, 8, e0_body, 0)

    qa_ref[...] = jnp.zeros(qa_ref.shape, F32)
    qb_ref[...] = jnp.zeros(qb_ref.shape, F32)
    ctx_ref[...] = jnp.zeros(ctx_ref.shape, F32)
    acca_ref[...] = jnp.zeros(acca_ref.shape, F32)
    accb_ref[...] = jnp.zeros(accb_ref.shape, F32)
    mb_ref[...] = jnp.zeros(mb_ref.shape, F32)
    lb_ref[...] = jnp.zeros(lb_ref.shape, F32)
    cacc_ref[...] = jnp.zeros(cacc_ref.shape, F32)
    olast_ref[...] = jnp.zeros(olast_ref.shape, F32)
    part_ref[...] = jnp.zeros(part_ref.shape, F32)
    oa_ref[...] = jnp.zeros(oa_ref.shape, F32)

    def expand(c32, fl=_nop):
        ce = _dot(c32.astype(BF16), e0_ref[...])
        fl()
        return jnp.concatenate(
            [jnp.where(row32 == lane32, ce[:, 128 * k:128 * k + 128], 0.0).astype(BF16)
             for k in range(8)], axis=1)

    def x_prep():
        cp_xa.wait()
        cp_xb.wait()
        xa = xa_buf[...].astype(F32)
        xb = xb_buf[...].astype(F32)
        xa32_ref[...] = jnp.concatenate(
            [jnp.broadcast_to(xa[b:b + 1, :], (8, 512)) for b in range(4)], axis=0).astype(BF16)
        xb32 = jnp.concatenate(
            [jnp.broadcast_to(xb[b:b + 1, :], (8, 512)) for b in range(4)], axis=0)
        for u in range(4):
            xexp_ref[u >> 1, :, (u & 1) * 1024:(u & 1) * 1024 + 1024] = expand(
                xb32[:, 128 * u:128 * u + 128])

    def qa_item(hg, half):
        col = pl.multiple_of(hg * 1024 + half * 512, 512)
        w = wq_buf[:, :, pl.ds(col, 512)].reshape(512, 512)
        r = _dot(xa32_ref[...], w)
        new = qa_ref[hg]
        for j in range(4):
            new = jnp.where(row32 == half * 4 + j, r[:, 128 * j:128 * j + 128], new)
        qa_ref[hg] = new

    def qb_item(n):
        hg = n >> 1
        half = n & 1
        w = wbq_buf[pl.ds(half * 2, 2), :, hg].reshape(2048, 128)
        qb_ref[hg] = qb_ref[hg] + _dot(xexp_ref[half], w)

    def qabs_item(n, fl):
        hg = n & 3
        u = n >> 2
        q = qb_ref[hg].astype(BF16)
        w = wuk_buf[u, :, hg].reshape(1024, 128)
        r = _dot_nt(q, w)
        fl()
        r = jnp.concatenate(
            [jnp.where(row32 == lane32, r[:, 128 * k:128 * k + 128], 0.0).astype(BF16)
             for k in range(8)], axis=1)
        qa = _dot_nt(r, e0_ref[...])
        for b in range(4):
            qabs_ref[u, b, hg] = qa[8 * b:8 * b + 8, :]

    def score_item(b, n, fl):
        qa = jnp.concatenate(
            [qabs_ref[u, b].reshape(32, 128).astype(BF16) for u in range(4)], axis=1)
        seg = b * 4 + (n >> 1)
        m = jnp.where(n == 0, -jnp.inf, mb_ref[...])
        for k in range(4):
            row = pl.multiple_of((n & 1) * 512 + k * 128, 128)
            s = _dot_nt(qa, cbuf[seg, pl.ds(row, 128), :])
            if k == 0:
                fl()
            sb_ref[n, :, 128 * k:128 * k + 128] = s
            m = jnp.maximum(m, s)
        mb_ref[...] = m

    def max_b():
        mb_ref[...] = jnp.broadcast_to(jnp.max(mb_ref[...], axis=1, keepdims=True), (32, 128))

    def pv_item(b, n, fl):
        m = mb_ref[...]
        ps = [jnp.exp((sb_ref[n, :, 128 * k:128 * k + 128] - m) * scale) for k in range(4)]
        first = n == 0
        lb_ref[...] = jnp.where(first, 0.0, lb_ref[...]) + ((ps[0] + ps[1]) + (ps[2] + ps[3]))
        seg = b * 4 + (n >> 1)
        acc = jnp.where(first, 0.0, cacc_ref[...])
        for k in range(4):
            row = pl.multiple_of((n & 1) * 512 + k * 128, 128)
            d = _dot(ps[k].astype(BF16), cbuf[seg, pl.ds(row, 128), :])
            if k == 0:
                fl()
            acc = acc + d
        cacc_ref[...] = acc

    def norm_b(b):
        inv = 1.0 / jnp.sum(lb_ref[...], axis=1, keepdims=True)
        res = cacc_ref[...] * inv
        for u in range(4):
            cc_ref[u, b] = res[:, 128 * u:128 * u + 128].reshape(4, 8, 128)

    def ctx_item(n, fl):
        hg = n >> 2
        u = n & 3
        c32 = jnp.concatenate([cc_ref[u, bb, hg] for bb in range(4)], axis=0)
        w = wuv_buf[u, :, hg].reshape(1024, 128)
        ctx_ref[hg] = ctx_ref[hg] + _dot(expand(c32, fl), w)

    def out_part(o32, w_half, j0, jj, nj, fl=_nop):
        acc = None
        for j in range(jj, jj + nj):
            d = _dot(jnp.where(row32 == j0 + j, o32, 0.0).astype(BF16),
                     w_half[j * 128:j * 128 + 128, :])
            if j == jj:
                fl()
            acc = d if acc is None else acc + d
        return acc

    def out_a_item(n, fl=_nop):
        acca_ref[...] = acca_ref[...] + out_part(
            oa_ref[n >> 1], wo_buf.at[n], (n & 1) * 4, 0, 4, fl)

    def out_b_item(n, fl=_nop):
        accb_ref[...] = accb_ref[...] + out_part(
            ctx_ref[n >> 1], wbo_buf.at[n >> 1, n & 1], (n & 1) * 4, 0, 4, fl)

    def rowsum(acc):
        return jnp.sum(acc.reshape(4, 8, 512), axis=1)

    def k_work(g, r):
        hg, b = hg_of(g), batch_of(g)
        q = jnp.where(row8 < nprev_of(g),
                      qa_ref[hg, pl.ds(_mo(((b + 3) & 3) * 8, 8), 8), :],
                      qa_ref[hg, pl.ds(_mo(b * 8, 8), 8), :]).astype(BF16)
        row = pl.multiple_of(r * 128, 128)
        h0 = (g & 1) * 8
        s = jnp.zeros((8, 128), F32)
        for j in range(8):
            sj = _dot_nt(q, kvbuf[0, h0 + j, pl.ds(row, 128), :])
            s = jnp.where(row8 == j, sj, s)
        sa_ref[r] = s

    def v_part(g, r):
        p = pa_ref[r].astype(BF16)
        row = _mo(r * 128, 128)
        h0 = (g & 1) * 8
        o = jnp.zeros((8, 128), F32)
        for j in range(8):
            oj = _dot(p, kvbuf[1, h0 + j, pl.ds(row, 128), :])
            o = jnp.where(row8 == j, oj, o)
        return oacc_ref[...] + o

    def finalize_o(g):
        l = jnp.sum(psum_ref[...], axis=1, keepdims=True)
        o = oacc_ref[...] * (1.0 / l)
        hg, b = hg_of(g), batch_of(g)
        prev = row8 < nprev_of(g)
        rp = pl.ds(_mo(((b + 3) & 3) * 8, 8), 8)
        rc = pl.ds(_mo(b * 8, 8), 8)
        oa_ref[hg, rp, :] = jnp.where(prev, o, oa_ref[hg, rp, :])
        oa_ref[hg, rc, :] = jnp.where(prev, oa_ref[hg, rc, :], o)

    def softmax_a():
        s = sa_ref[...]
        m = jnp.max(jnp.max(s, axis=0), axis=1, keepdims=True)
        p = jnp.exp((s - m[None]) * scale)
        pa_ref[...] = p
        psum_ref[...] = jnp.sum(p, axis=0)
        oacc_ref[...] = jnp.zeros((8, 128), F32)

    def k0_tick(r, t, s0):
        wait16(0, r, t, s0 + t)
        start_wq(r * 16 + (t >> 2) * 8, (t & 3) * 512, 512, S_WQ)

    def k0a_body(r, carry):
        s0 = (r & 1) * 8
        for t in range(8):
            k0_tick(r, t, s0)
            start16_first(k_hbm, 0, r + 2, t, s0 + t)
        return carry
    lax.fori_loop(0, 6, k0a_body, 0)

    x_prep()

    def k0b_body(r, carry):
        s0 = r * 8
        for t in range(8):
            k0_tick(r + 6, t, s0)
            low_c(r * 2 + (t >> 2), t & 3, s0 + t).start(priority=LO)
        return carry
    lax.fori_loop(0, 2, k0b_body, 0)

    def c0_body(it, carry):
        s0 = (it & 3) * 4
        for t in range(4):
            low_c(it, t, s0 + t).wait()
            high_3d(wbq_hbm, wbq_buf, it * 4 + t, 0, 4, S_WBQ).start(priority=HI)
            low_c(it + 4, t, s0 + t).start(priority=LO)

        @pl.when(it == 1)
        def _():
            wait_all(wq_buf.at[:, :, pl.ds(0, 2048)], S_WQ)

        @pl.when(jnp.logical_and(it >= 1, it < 5))
        def _():
            qa_item((it - 1) >> 1, (it - 1) & 1)

        @pl.when(jnp.logical_and(it >= 5, it < 13))
        def _():
            k_work(0, it - 5)

        @pl.when(it == 13)
        def _():
            softmax_a()
        return carry
    lax.fori_loop(0, 32, c0_body, 0)

    def c1_tick(it, t, s0):
        low_c(32 + it, t, s0 + t).wait()
        high_3d(wuk_hbm, wuk_buf, it * 4 + t, 0, 4, S_WUK).start(priority=HI)

    def c1_body(it, carry):
        s0 = (it & 3) * 4
        for t in range(4):
            c1_tick(it, t, s0)
            low_c(36 + it, t, s0 + t).start(priority=LO)

        @pl.when(it == 1)
        def _():
            wait_all(wbq_buf, S_WBQ)

        @pl.when(jnp.logical_and(it >= 1, it < 9))
        def _():
            qb_item(it - 1)
        return carry
    lax.fori_loop(0, 28, c1_body, 0)

    def c1b_body(r, carry):
        for t in range(8):
            c1_tick(28 + r * 2 + (t >> 2), t & 3, r * 8 + (t >> 2) * 4)
            start16_first(v_hbm, 1, r, t, r * 8 + t)
        return carry
    lax.fori_loop(0, 2, c1b_body, 0)

    def make_main(high, hook, extra, first, last):
        def body(i, carry):
            g = i >> 3
            r = i & 7
            i2 = i + 2
            g2 = i2 >> 3
            r2 = i2 & 7
            sg2 = (g2 + 1) >> 1
            odd2 = (g2 & 1) == 1
            s0 = (i & 1) * 8
            kv = 1 - (g & 1)

            def tick(t, with_high=True):
                wait16(kv, r, t, s0 + t)
                if with_high:
                    high(i, t)

                @pl.when(odd2)
                def _():
                    start16(k_hbm, 0, sg2, r2, t, s0 + t)

                if first:
                    @pl.when(i2 < 8)
                    def _():
                        start16_first(v_hbm, 1, r2, t, s0 + t)

                    @pl.when(i2 >= 16)
                    def _():
                        start16(v_hbm, 1, sg2, r2, t, s0 + t)
                elif not last:
                    @pl.when(jnp.logical_not(odd2))
                    def _():
                        start16(v_hbm, 1, sg2, r2, t, s0 + t)
                else:
                    @pl.when(jnp.logical_and(jnp.logical_not(odd2), i2 < N_MAIN))
                    def _():
                        start16(v_hbm, 1, sg2, r2, t, s0 + t)

                    @pl.when(i2 >= N_MAIN)
                    def _():
                        low_v8(0, 2 * r2 + (t >> 2), t & 3, s0 + t).start(priority=LO)

            tick(0)
            tick(1)

            @pl.when(jnp.logical_and(r == 0, i > 0))
            def _():
                finalize_o(g - 1)
                softmax_a()

            extra(i)
            tick(2)
            tick(3)
            hook(i, lambda: high(i, 5))
            tick(4)
            tick(5, False)
            tick(6)
            tick(7)
            oacc_ref[...] = v_part(g, r)
            k_work(g + 1, r)
            return carry
        return body

    def high0(i, t):
        start_wq(i * 8, 2048 + t * 256, 256, S_WQ + 1)

    def hook0(i, fl):
        @pl.when(i == 0)
        def _():
            wait_all(wuk_buf, S_WUK)

        qabs_item(i, fl)

    def high1(i, t):
        @pl.when(i < 48)
        def _():
            high_3d(wuv_hbm, wuv_buf, (i - 16) * 4 + (t >> 1), (t & 1) * 2, 2,
                    S_WUV).start(priority=HI)

        @pl.when(i >= 48)
        def _():
            high_wbo((i >> 4) - 3, (i & 15) * 32 + (t >> 1) * 8, (t & 1) * 256).start(priority=HI)

    def extra1(i):
        n = i - 16

        @pl.when(i == 25)
        def _():
            wait_all(wq_buf.at[:, :, pl.ds(2048, 2048)], S_WQ + 1)

        @pl.when(jnp.logical_and(i >= 25, i < 29))
        def _():
            qa_item(2 + ((i - 25) >> 1), (i - 25) & 1)

        @pl.when((n & 15) == 8)
        def _():
            max_b()

        @pl.when(jnp.logical_and((n & 15) == 1, n > 16))
        def _():
            norm_b((n >> 4) - 1)

    def hook1(i, fl):
        n = i - 16

        @pl.when((n & 8) == 0)
        def _():
            score_item(n >> 4, n & 7, fl)

        @pl.when((n & 8) != 0)
        def _():
            pv_item(n >> 4, n & 7, fl)

    def high2(i, t):
        row = (i & 15) * 32 + (t >> 1) * 8

        @pl.when(i < 96)
        def _():
            for p0, np_ in WO_RUNS:
                high_wo(p0, np_, row, 8, (t & 1) * 256, 256, S_WO).start(priority=HI)

        @pl.when(i >= 96)
        def _():
            high_wo(4, 2, row, 8, (t & 1) * 256, 256, S_WO + 1).start(priority=HI)

    def extra2(i):
        @pl.when(i == 80)
        def _():
            wait_all(wuv_buf, S_WUV)
            norm_b(3)

        @pl.when(i == 96)
        def _():
            wait_all(wbo_buf, S_WBO)

        @pl.when(i == 105)
        def _():
            wait_all(wo_buf.at[pl.ds(0, 4)], S_WO)
            obuf[1] = rowsum(accb_ref[...]).astype(obuf.dtype)
            out_copy(1).start(priority=HI)

    def hook2(i, fl):
        @pl.when(i < 96)
        def _():
            ctx_item(i - 80, fl)

        @pl.when(jnp.logical_and(i >= 96, i < 104))
        def _():
            out_b_item(i - 96, fl)

        @pl.when(jnp.logical_and(i >= 105, i < 109))
        def _():
            out_a_item(i - 105, fl)

        @pl.when(jnp.logical_or(i == 104, i >= 109))
        def _():
            fl()

    lax.fori_loop(0, 16, make_main(high0, hook0, _nop, True, False), 0)
    lax.fori_loop(16, 80, make_main(high1, hook1, extra1, False, False), 0)
    lax.fori_loop(80, N_MAIN, make_main(high2, hook2, extra2, False, True), 0)

    finalize_o(13)
    softmax_a()

    def g14_body(r, carry):
        s0 = (r & 3) * 4
        nx = r + 4
        for t in range(4):
            low_v8(0, r, t, s0 + t).wait()
            high_wo(6, 1, r * 32 + t * 8, 8, 0, 512, S_WO + 2).start(priority=HI)
            low_v8(nx >> 3, nx & 7, t, s0 + t).start(priority=LO)
        oacc_ref[...] = v_part(14, r)
        k_work(15, r)
        return carry
    lax.fori_loop(0, 8, g14_body, 0)

    finalize_o(14)
    softmax_a()

    def v15_body(r, carry):
        s0 = (r & 3) * 4
        for t in range(4):
            low_v8(1, r, t, s0 + t).wait()

            @pl.when(r < NBIG)
            def _():
                high_wo(6, 1, 256 + r * 64 + t * 16, 16, 0, 512, S_WO + 2).start(priority=HI)

            @pl.when(jnp.logical_and(r >= NBIG, r < 8 - NBIG))
            def _():
                high_wo(6, 1, 256 + NBIG * 32 + r * 32 + t * 8, 8, 0, 512,
                        S_WO + 2).start(priority=HI)

            @pl.when(r < 4)
            def _():
                low_v8(1, r + 4, t, s0 + t).start(priority=LO)

            @pl.when(jnp.logical_and(r >= 4, r < 6))
            def _():
                low_wo(s0 + t, s0 + t).start(priority=LO)

            if t == 1:
                @pl.when(r == 1)
                def _():
                    wait_all(wo_buf.at[pl.ds(4, 2)], S_WO + 1)

                @pl.when(jnp.logical_and(r >= 1, r < 3))
                def _():
                    out_a_item(r + 3)

                @pl.when(r == 4)
                def _():
                    l = jnp.sum(psum_ref[...], axis=1, keepdims=True)
                    psum_ref[...] = jnp.broadcast_to(1.0 / l, (8, 128))
        oacc_ref[...] = v_part(15, r)
        return carry
    lax.fori_loop(0, 7, v15_body, 0)

    for t in range(4):
        low_v8(1, 7, t, 12 + t).wait()
    oa_ref[3, 24:32, :] = v_part(15, 7) * psum_ref[...]
    wait_all(wo_buf.at[pl.ds(6, 1)], S_WO + 2)
    for n in range(2):
        low_wo(n, n).wait()
    o32 = oa_ref[3]
    part_ref[0:4, :] = rowsum(acca_ref[...] + out_part(o32, wo_buf.at[6], 0, 0, 4)
                              + out_part(o32, wo_buf.at[7], 4, 0, 1))
    for j in range(5, 8):
        olast_ref[0:4, (j - 5) * 128:(j - 4) * 128] = o32.reshape(4, 8, 128)[:, j, :]
    for n in range(2, NSPLIT):
        low_wo(n, n).wait()
    k1 = NSPLIT * 64
    part_ref[...] = part_ref[...] + _dot(
        olast_ref[:, 0:k1 - 128].astype(BF16), wo_buf[7, 128:k1, :])
    lhs = olast_ref[:, k1 - 128:384].astype(BF16)
    for n in range(NSPLIT, 8):
        low_wo(n, n).wait()
    res = part_ref[...] + _dot(lhs, wo_buf[7, k1:512, :])
    obuf[0] = res[0:4, :].astype(obuf.dtype)
    out_copy(0).start(priority=HI)
    out_copy(1).wait()
    out_copy(0).wait()


@jax.jit
def pallas_concat_heads__sliding_block_cached__compressed_kv_cla__decode_kernel(
    A_x: jax.Array,
    A_k_cache: jax.Array,
    A_v_cache: jax.Array,
    A_wq: jax.Array,
    A_wo: jax.Array,
    B_x: jax.Array,
    B_c_kv: jax.Array,
    B_w_q: jax.Array,
    B_w_uk: jax.Array,
    B_w_uv: jax.Array,
    B_w_o: jax.Array,
):
    B, Sq, D = A_x.shape
    _, H, Sk, Dh = A_k_cache.shape
    W = min(4096, max(256, Sk // 4))
    assert (B, Sq, D, H, Sk, Dh, W) == (4, 1, 512, 32, 4096, 128, 1024)
    assert B_c_kv.shape == (4, 4096, 512) and B_w_q.shape == (512, 32, 128)

    def body(*refs):
        _kernel(*refs, win_off=Sk - W, scale=float(Dh) ** -0.5)

    vm = pltpu.VMEM
    scratch = [
        vm((2, 16, 1024, 128), BF16),
        vm((16, 1024, 512), BF16),
        vm((4, 128, 4096), BF16),
        vm((8, 512, 512), BF16),
        vm((4, 128, 4, 8, 128), BF16),
        vm((4, 128, 4, 8, 128), BF16),
        vm((4, 128, 4, 8, 128), BF16),
        vm((4, 2, 512, 512), BF16),
        vm((4, 512), BF16),
        vm((4, 512), BF16),
        vm((128, 1024), BF16),
        vm((32, 512), BF16),
        vm((2, 32, 2048), BF16),
        vm((4, 32, 128), F32),
        vm((8, 8, 128), F32),
        vm((8, 8, 128), F32),
        vm((8, 128), F32),
        vm((8, 128), F32),
        vm((4, 32, 128), F32),
        vm((4, 32, 128), F32),
        vm((4, 4, 4, 8, 128), F32),
        vm((8, 32, 512), F32),
        vm((32, 128), F32),
        vm((32, 128), F32),
        vm((32, 512), F32),
        vm((4, 4, 4, 8, 128), F32),
        vm((4, 32, 128), F32),
        vm((32, 512), F32),
        vm((32, 512), F32),
        vm((8, 384), F32),
        vm((8, 512), F32),
        vm((2, 4, 512), A_x.dtype),
        pltpu.SemaphoreType.DMA((NS,)),
        pltpu.SemaphoreType.DMA((N_HSEM,)),
        pltpu.SemaphoreType.DMA((4,)),
    ]
    out = pl.pallas_call(
        body,
        out_shape=jax.ShapeDtypeStruct((B, 2 * D), A_x.dtype),
        in_specs=[pl.BlockSpec(memory_space=pl.ANY)] * 11,
        out_specs=pl.BlockSpec(memory_space=pl.ANY),
        scratch_shapes=scratch,
        compiler_params=pltpu.CompilerParams(
            vmem_limit_bytes=64 * 1024 * 1024,
            disable_bounds_checks=True,
            disable_semaphore_checks=True,
        ),
    )(
        A_x.reshape(B, D),
        A_k_cache.reshape(B * H, Sk, Dh),
        A_v_cache.reshape(B * H, Sk, Dh),
        A_wq.reshape(4, 128, 4096),
        A_wo.reshape(8, 512, 512),
        B_x.reshape(B, D),
        B_c_kv.reshape(16, 1024, 512),
        B_w_q.reshape(4, 128, 4, 8, 128),
        B_w_uk.reshape(4, 128, 4, 8, 128),
        B_w_uv.reshape(4, 128, 4, 8, 128),
        B_w_o.reshape(4, 2, 512, 512),
    )
    return out.reshape(B, Sq, 2 * D)
```

```python
import jax
import jax.numpy as jnp
from jax import lax
import jax.experimental.pallas as pl
import jax.experimental.pallas.tpu as pltpu

F32 = jnp.float32
BF16 = jnp.bfloat16
_NT = (((1,), (1,)), ((), ()))
_NN = (((1,), (0,)), ((), ()))

LO, HI = 1, 0
NS = 16
N_MAIN = 112

S_WQ = 0
S_WBQ = 4
S_WUK = 5
S_WUV = 6
S_WBO = 7
S_WO = 8
N_HSEM = 11
NSPLIT = 6
NBIG = 3
C_RUNS = ((0, 2, 960), (2, 14, 0))
WLAG = 256
ROT = 14
ROTC = ((32 - ROT) % 32) * 128
_PW = ROT // 4
WO_RUNS = [(a, n) for a, n in ((0, _PW), (_PW, 1), (_PW + 1, 3 - _PW)) if n > 0] if ROT else [(0, 4)]


def _dot(a, b):
    return lax.dot_general(a, b, _NN, preferred_element_type=F32)


def _dot_nt(a, b):
    return lax.dot_general(a, b, _NT, preferred_element_type=F32)


def _mo(x, m):
    return x if isinstance(x, int) else pl.multiple_of(x, m)


def _nop(_=None):
    return None


def _kernel(xa_hbm, k_hbm, v_hbm, wq_hbm, wo_hbm, xb_hbm, c_hbm, wbq_hbm, wuk_hbm,
            wuv_hbm, wbo_hbm, out_hbm,
            kvbuf, cbuf, wq_buf, wo_buf, wbq_buf, wuk_buf, wuv_buf, wbo_buf,
            xa_buf, xb_buf, e0_ref, xa32_ref, xexp_ref,
            qa_ref, sa_ref, pa_ref, psum_ref, oacc_ref, oa_ref,
            qb_ref, qabs_ref, sb_ref, mb_ref, lb_ref, cacc_ref, cc_ref, ctx_ref,
            acca_ref, accb_ref, olast_ref, part_ref, obuf,
            lsem, hsem, xsem, *, win_off, scale):

    def start_c(it, t, sem):
        row = _mo(it * 16 + (t >> 1) * 8, 8)
        col = (t & 1) * 256
        for seg, n, lag in C_RUNS:
            pltpu.make_async_copy(
                c_hbm.at[pl.ds(seg, n), pl.ds(_mo((row + lag) & 1023, 8), 8), pl.ds(col, 256)],
                cbuf.at[pl.ds(seg, n), pl.ds(row, 8), pl.ds(col, 256)],
                lsem.at[sem]).start(priority=LO)

    def wait_c(it, t, sem):
        dst = cbuf.at[:, pl.ds(_mo(it * 16 + (t >> 1) * 8, 8), 8), pl.ds((t & 1) * 256, 256)]
        pltpu.make_async_copy(dst, dst, lsem.at[sem]).wait()

    def batch_of(g):
        return (g >> 1) & 3

    def hg_of(g):
        return (g >> 3) * 2 + (g & 1)

    def nprev_of(g):
        n = ROT - hg_of(g) * 8
        return max(0, min(8, n)) if isinstance(n, int) else jnp.clip(n, 0, 8)

    def low_heads(src, kv, head, slot, n, r, t, sem, lag=0):
        row = _mo(r * 128 + t * 16, 16)
        srow = (row + lag) & 1023 if lag else row
        return pltpu.make_async_copy(
            src.at[pl.ds(head, n), pl.ds(_mo(win_off + srow, 16), 16), :],
            kvbuf.at[kv, pl.ds(slot, n), pl.ds(row, 16), :],
            lsem.at[sem])

    def start16(src, kv, sg, r, t, sem):
        head = (sg & 3) * 32 + (sg >> 2) * 16 - ROT
        low_heads(src, kv, head, 0, 16, r, t, sem).start(priority=LO)

    def start16_first(src, kv, r, t, sem):
        if ROT:
            low_heads(src, kv, 128 - ROT, 0, ROT, r, t, sem).start(priority=LO)
        low_heads(src, kv, 0, ROT, 16 - ROT, r, t, sem, WLAG).start(priority=LO)

    def wait16(kv, r, t, sem):
        dst = kvbuf.at[kv, :, pl.ds(_mo(r * 128 + t * 16, 16), 16), :]
        pltpu.make_async_copy(dst, dst, lsem.at[sem]).wait()

    def low_v8(e, r, t, sem):
        row = _mo(r * 128 + t * 32, 32)
        return pltpu.make_async_copy(
            v_hbm.at[pl.ds(112 - ROT + e * 8, 8), pl.ds(_mo(win_off + row, 32), 32), :],
            kvbuf.at[1, pl.ds(e * 8, 8), pl.ds(row, 32), :],
            lsem.at[sem])

    def wo_copy(p0, np_, row, rows, col, cols, sem):
        flat = (p0 * 512 + row + ROTC) & 4095
        return pltpu.make_async_copy(
            wo_hbm.at[pl.ds(flat >> 9, np_), pl.ds(_mo(flat & 511, 8), rows), pl.ds(col, cols)],
            wo_buf.at[pl.ds(p0, np_), pl.ds(_mo(row, 8), rows), pl.ds(col, cols)], sem)

    def low_wo(n, sem):
        return wo_copy(7, 1, n * 64, 64, 0, 512, lsem.at[sem])

    def start_wq(row, col, cols, sem):
        row = _mo(row, 8)
        src = (col + ROTC) % 4096
        first = min(cols, 4096 - src)
        for c0, s0, n in ((col, src, first), (col + first, 0, cols - first)):
            if n:
                pltpu.make_async_copy(
                    wq_hbm.at[:, pl.ds(row, 8), pl.ds(s0, n)],
                    wq_buf.at[:, pl.ds(row, 8), pl.ds(c0, n)], hsem.at[sem]).start(priority=HI)

    def high_3d(src, dst, row, hg, nhg, sem):
        return pltpu.make_async_copy(
            src.at[:, row, pl.ds(hg, nhg)], dst.at[:, row, pl.ds(hg, nhg)], hsem.at[sem])

    def high_wbo(half, row, col):
        row = _mo(row, 8)
        return pltpu.make_async_copy(
            wbo_hbm.at[:, half, pl.ds(row, 8), pl.ds(col, 256)],
            wbo_buf.at[:, half, pl.ds(row, 8), pl.ds(col, 256)], hsem.at[S_WBO])

    def high_wo(p0, np_, row, rows, col, cols, sem):
        return wo_copy(p0, np_, row, rows, col, cols, hsem.at[sem])

    def out_copy(h):
        return pltpu.make_async_copy(
            obuf.at[h], out_hbm.at[:, pl.ds(h * 512, 512)], xsem.at[2 + h])

    def wait_all(buf, sem):
        pltpu.make_async_copy(buf, buf, hsem.at[sem]).wait()

    for r in range(2):
        for t in range(8):
            start16_first(k_hbm, 0, r, t, r * 8 + t)
    cp_xa = pltpu.make_async_copy(xa_hbm, xa_buf, xsem.at[0])
    cp_xb = pltpu.make_async_copy(xb_hbm, xb_buf, xsem.at[1])
    cp_xa.start(priority=HI)
    cp_xb.start(priority=HI)

    row8 = lax.broadcasted_iota(jnp.int32, (8, 128), 0)
    row32 = lax.broadcasted_iota(jnp.int32, (32, 128), 0) & 7
    lane32 = lax.broadcasted_iota(jnp.int32, (32, 128), 1) & 7

    def e0_body(i, c):
        r0 = pl.multiple_of(i * 16, 16)
        rr = lax.broadcasted_iota(jnp.int32, (16, 1024), 0) + r0
        cc = lax.broadcasted_iota(jnp.int32, (16, 1024), 1) >> 3
        e0_ref[pl.ds(r0, 16), :] = jnp.where(rr == cc, 1.0, 0.0).astype(BF16)
        return c
    lax.fori_loop(0, 8, e0_body, 0)

    qa_ref[...] = jnp.zeros(qa_ref.shape, F32)
    qb_ref[...] = jnp.zeros(qb_ref.shape, F32)
    ctx_ref[...] = jnp.zeros(ctx_ref.shape, F32)
    acca_ref[...] = jnp.zeros(acca_ref.shape, F32)
    accb_ref[...] = jnp.zeros(accb_ref.shape, F32)
    mb_ref[...] = jnp.zeros(mb_ref.shape, F32)
    lb_ref[...] = jnp.zeros(lb_ref.shape, F32)
    cacc_ref[...] = jnp.zeros(cacc_ref.shape, F32)
    olast_ref[...] = jnp.zeros(olast_ref.shape, F32)
    part_ref[...] = jnp.zeros(part_ref.shape, F32)
    oa_ref[...] = jnp.zeros(oa_ref.shape, F32)

    def expand(c32, fl=_nop):
        ce = _dot(c32.astype(BF16), e0_ref[...])
        fl()
        return jnp.concatenate(
            [jnp.where(row32 == lane32, ce[:, 128 * k:128 * k + 128], 0.0).astype(BF16)
             for k in range(8)], axis=1)

    def x_prep():
        cp_xa.wait()
        cp_xb.wait()
        xa = xa_buf[...].astype(F32)
        xb = xb_buf[...].astype(F32)
        xa32_ref[...] = jnp.concatenate(
            [jnp.broadcast_to(xa[b:b + 1, :], (8, 512)) for b in range(4)], axis=0).astype(BF16)
        xb32 = jnp.concatenate(
            [jnp.broadcast_to(xb[b:b + 1, :], (8, 512)) for b in range(4)], axis=0)
        for u in range(4):
            xexp_ref[u >> 1, :, (u & 1) * 1024:(u & 1) * 1024 + 1024] = expand(
                xb32[:, 128 * u:128 * u + 128])

    def qa_item(hg, half):
        col = pl.multiple_of(hg * 1024 + half * 512, 512)
        w = wq_buf[:, :, pl.ds(col, 512)].reshape(512, 512)
        r = _dot(xa32_ref[...], w)
        new = qa_ref[hg]
        for j in range(4):
            new = jnp.where(row32 == half * 4 + j, r[:, 128 * j:128 * j + 128], new)
        qa_ref[hg] = new

    def qb_item(n):
        hg = n >> 1
        half = n & 1
        w = wbq_buf[pl.ds(half * 2, 2), :, hg].reshape(2048, 128)
        qb_ref[hg] = qb_ref[hg] + _dot(xexp_ref[half], w)

    def qabs_item(n, fl):
        hg = n & 3
        u = n >> 2
        q = qb_ref[hg].astype(BF16)
        w = wuk_buf[u, :, hg].reshape(1024, 128)
        r = _dot_nt(q, w)
        fl()
        r = jnp.concatenate(
            [jnp.where(row32 == lane32, r[:, 128 * k:128 * k + 128], 0.0).astype(BF16)
             for k in range(8)], axis=1)
        qa = _dot_nt(r, e0_ref[...])
        for b in range(4):
            qabs_ref[u, b, hg] = qa[8 * b:8 * b + 8, :]

    def score_item(b, n, fl):
        qa = jnp.concatenate(
            [qabs_ref[u, b].reshape(32, 128).astype(BF16) for u in range(4)], axis=1)
        seg = b * 4 + (n >> 1)
        m = jnp.where(n == 0, -jnp.inf, mb_ref[...])
        for k in range(4):
            row = pl.multiple_of((n & 1) * 512 + k * 128, 128)
            s = _dot_nt(qa, cbuf[seg, pl.ds(row, 128), :])
            if k == 0:
                fl()
            sb_ref[n, :, 128 * k:128 * k + 128] = s
            m = jnp.maximum(m, s)
        mb_ref[...] = m

    def max_b():
        mb_ref[...] = jnp.broadcast_to(jnp.max(mb_ref[...], axis=1, keepdims=True), (32, 128))

    def pv_item(b, n, fl):
        m = mb_ref[...]
        ps = [jnp.exp((sb_ref[n, :, 128 * k:128 * k + 128] - m) * scale) for k in range(4)]
        first = n == 0
        lb_ref[...] = jnp.where(first, 0.0, lb_ref[...]) + ((ps[0] + ps[1]) + (ps[2] + ps[3]))
        seg = b * 4 + (n >> 1)
        acc = jnp.where(first, 0.0, cacc_ref[...])
        for k in range(4):
            row = pl.multiple_of((n & 1) * 512 + k * 128, 128)
            d = _dot(ps[k].astype(BF16), cbuf[seg, pl.ds(row, 128), :])
            if k == 0:
                fl()
            acc = acc + d
        cacc_ref[...] = acc

    def norm_b(b):
        inv = 1.0 / jnp.sum(lb_ref[...], axis=1, keepdims=True)
        res = cacc_ref[...] * inv
        for u in range(4):
            cc_ref[u, b] = res[:, 128 * u:128 * u + 128].reshape(4, 8, 128)

    def ctx_item(n, fl):
        hg = n >> 2
        u = n & 3
        c32 = jnp.concatenate([cc_ref[u, bb, hg] for bb in range(4)], axis=0)
        w = wuv_buf[u, :, hg].reshape(1024, 128)
        ctx_ref[hg] = ctx_ref[hg] + _dot(expand(c32, fl), w)

    def out_part(o32, w_half, j0, jj, nj, fl=_nop):
        acc = None
        for j in range(jj, jj + nj):
            d = _dot(jnp.where(row32 == j0 + j, o32, 0.0).astype(BF16),
                     w_half[j * 128:j * 128 + 128, :])
            if j == jj:
                fl()
            acc = d if acc is None else acc + d
        return acc

    def out_a_item(n, fl=_nop):
        acca_ref[...] = acca_ref[...] + out_part(
            oa_ref[n >> 1], wo_buf.at[n], (n & 1) * 4, 0, 4, fl)

    def out_b_item(n, fl=_nop):
        accb_ref[...] = accb_ref[...] + out_part(
            ctx_ref[n >> 1], wbo_buf.at[n >> 1, n & 1], (n & 1) * 4, 0, 4, fl)

    def rowsum(acc):
        return jnp.sum(acc.reshape(4, 8, 512), axis=1)

    def k_work(g, r):
        hg, b = hg_of(g), batch_of(g)
        q = jnp.where(row8 < nprev_of(g),
                      qa_ref[hg, pl.ds(_mo(((b + 3) & 3) * 8, 8), 8), :],
                      qa_ref[hg, pl.ds(_mo(b * 8, 8), 8), :]).astype(BF16)
        row = pl.multiple_of(r * 128, 128)
        h0 = (g & 1) * 8
        s = jnp.zeros((8, 128), F32)
        for j in range(8):
            sj = _dot_nt(q, kvbuf[0, h0 + j, pl.ds(row, 128), :])
            s = jnp.where(row8 == j, sj, s)
        sa_ref[r] = s

    def v_part(g, r):
        p = pa_ref[r].astype(BF16)
        row = _mo(r * 128, 128)
        h0 = (g & 1) * 8
        o = jnp.zeros((8, 128), F32)
        for j in range(8):
            oj = _dot(p, kvbuf[1, h0 + j, pl.ds(row, 128), :])
            o = jnp.where(row8 == j, oj, o)
        return oacc_ref[...] + o

    def finalize_o(g):
        l = jnp.sum(psum_ref[...], axis=1, keepdims=True)
        o = oacc_ref[...] * (1.0 / l)
        hg, b = hg_of(g), batch_of(g)
        prev = row8 < nprev_of(g)
        rp = pl.ds(_mo(((b + 3) & 3) * 8, 8), 8)
        rc = pl.ds(_mo(b * 8, 8), 8)
        oa_ref[hg, rp, :] = jnp.where(prev, o, oa_ref[hg, rp, :])
        oa_ref[hg, rc, :] = jnp.where(prev, oa_ref[hg, rc, :], o)

    def softmax_a():
        s = sa_ref[...]
        m = jnp.max(jnp.max(s, axis=0), axis=1, keepdims=True)
        p = jnp.exp((s - m[None]) * scale)
        pa_ref[...] = p
        psum_ref[...] = jnp.sum(p, axis=0)
        oacc_ref[...] = jnp.zeros((8, 128), F32)

    def k0_tick(r, t, s0):
        wait16(0, r, t, s0 + t)
        start_wq(r * 16 + (t >> 2) * 8, (t & 3) * 512, 512, S_WQ)

    def k0a_body(r, carry):
        s0 = (r & 1) * 8
        for t in range(8):
            k0_tick(r, t, s0)
            start16_first(k_hbm, 0, r + 2, t, s0 + t)
        return carry
    lax.fori_loop(0, 6, k0a_body, 0)

    x_prep()

    def k0b_body(r, carry):
        s0 = r * 8
        for t in range(8):
            k0_tick(r + 6, t, s0)
            start_c(r * 2 + (t >> 2), t & 3, s0 + t)
        return carry
    lax.fori_loop(0, 2, k0b_body, 0)

    def c0_body(it, carry):
        s0 = (it & 3) * 4
        for t in range(4):
            wait_c(it, t, s0 + t)
            high_3d(wbq_hbm, wbq_buf, it * 4 + t, 0, 4, S_WBQ).start(priority=HI)
            start_c(it + 4, t, s0 + t)

        @pl.when(it == 1)
        def _():
            wait_all(wq_buf.at[:, :, pl.ds(0, 2048)], S_WQ)

        @pl.when(jnp.logical_and(it >= 1, it < 5))
        def _():
            qa_item((it - 1) >> 1, (it - 1) & 1)

        @pl.when(jnp.logical_and(it >= 5, it < 13))
        def _():
            k_work(0, it - 5)

        @pl.when(it == 13)
        def _():
            softmax_a()
        return carry
    lax.fori_loop(0, 32, c0_body, 0)

    def c1_tick(it, t, s0):
        wait_c(32 + it, t, s0 + t)
        high_3d(wuk_hbm, wuk_buf, it * 4 + t, 0, 4, S_WUK).start(priority=HI)

    def c1_body(it, carry):
        s0 = (it & 3) * 4
        for t in range(4):
            c1_tick(it, t, s0)
            start_c(36 + it, t, s0 + t)

        @pl.when(it == 1)
        def _():
            wait_all(wbq_buf, S_WBQ)

        @pl.when(jnp.logical_and(it >= 1, it < 9))
        def _():
            qb_item(it - 1)
        return carry
    lax.fori_loop(0, 28, c1_body, 0)

    def c1b_body(r, carry):
        for t in range(8):
            c1_tick(28 + r * 2 + (t >> 2), t & 3, r * 8 + (t >> 2) * 4)
            start16_first(v_hbm, 1, r, t, r * 8 + t)
        return carry
    lax.fori_loop(0, 2, c1b_body, 0)

    def make_main(high, hook, extra, first, last):
        def body(i, carry):
            g = i >> 3
            r = i & 7
            i2 = i + 2
            g2 = i2 >> 3
            r2 = i2 & 7
            sg2 = (g2 + 1) >> 1
            odd2 = (g2 & 1) == 1
            s0 = (i & 1) * 8
            kv = 1 - (g & 1)

            def tick(t, with_high=True):
                wait16(kv, r, t, s0 + t)
                if with_high:
                    high(i, t)

                @pl.when(odd2)
                def _():
                    start16(k_hbm, 0, sg2, r2, t, s0 + t)

                if first:
                    @pl.when(i2 < 8)
                    def _():
                        start16_first(v_hbm, 1, r2, t, s0 + t)

                    @pl.when(i2 >= 16)
                    def _():
                        start16(v_hbm, 1, sg2, r2, t, s0 + t)
                elif not last:
                    @pl.when(jnp.logical_not(odd2))
                    def _():
                        start16(v_hbm, 1, sg2, r2, t, s0 + t)
                else:
                    @pl.when(jnp.logical_and(jnp.logical_not(odd2), i2 < N_MAIN))
                    def _():
                        start16(v_hbm, 1, sg2, r2, t, s0 + t)

                    @pl.when(i2 >= N_MAIN)
                    def _():
                        low_v8(0, 2 * r2 + (t >> 2), t & 3, s0 + t).start(priority=LO)

            tick(0)
            tick(1)

            @pl.when(jnp.logical_and(r == 0, i > 0))
            def _():
                finalize_o(g - 1)
                softmax_a()

            extra(i)
            tick(2)
            tick(3)
            hook(i, lambda: high(i, 5))
            tick(4)
            tick(5, False)
            tick(6)
            tick(7)
            oacc_ref[...] = v_part(g, r)
            k_work(g + 1, r)
            return carry
        return body

    def high0(i, t):
        start_wq(i * 8, 2048 + t * 256, 256, S_WQ + 1)

    def hook0(i, fl):
        @pl.when(i == 0)
        def _():
            wait_all(wuk_buf, S_WUK)

        qabs_item(i, fl)

    def high1(i, t):
        @pl.when(i < 48)
        def _():
            high_3d(wuv_hbm, wuv_buf, (i - 16) * 4 + (t >> 1), (t & 1) * 2, 2,
                    S_WUV).start(priority=HI)

        @pl.when(i >= 48)
        def _():
            high_wbo((i >> 4) - 3, (i & 15) * 32 + (t >> 1) * 8, (t & 1) * 256).start(priority=HI)

    def extra1(i):
        n = i - 16

        @pl.when(i == 25)
        def _():
            wait_all(wq_buf.at[:, :, pl.ds(2048, 2048)], S_WQ + 1)

        @pl.when(jnp.logical_and(i >= 25, i < 29))
        def _():
            qa_item(2 + ((i - 25) >> 1), (i - 25) & 1)

        @pl.when((n & 15) == 8)
        def _():
            max_b()

        @pl.when(jnp.logical_and((n & 15) == 1, n > 16))
        def _():
            norm_b((n >> 4) - 1)

    def hook1(i, fl):
        n = i - 16

        @pl.when((n & 8) == 0)
        def _():
            score_item(n >> 4, n & 7, fl)

        @pl.when((n & 8) != 0)
        def _():
            pv_item(n >> 4, n & 7, fl)

    def high2(i, t):
        row = (i & 15) * 32 + (t >> 1) * 8

        @pl.when(i < 96)
        def _():
            for p0, np_ in WO_RUNS:
                high_wo(p0, np_, row, 8, (t & 1) * 256, 256, S_WO).start(priority=HI)

        @pl.when(i >= 96)
        def _():
            high_wo(4, 2, row, 8, (t & 1) * 256, 256, S_WO + 1).start(priority=HI)

    def extra2(i):
        @pl.when(i == 80)
        def _():
            wait_all(wuv_buf, S_WUV)
            norm_b(3)

        @pl.when(i == 96)
        def _():
            wait_all(wbo_buf, S_WBO)

        @pl.when(i == 105)
        def _():
            wait_all(wo_buf.at[pl.ds(0, 4)], S_WO)
            obuf[1] = rowsum(accb_ref[...]).astype(obuf.dtype)
            out_copy(1).start(priority=HI)

    def hook2(i, fl):
        @pl.when(i < 96)
        def _():
            ctx_item(i - 80, fl)

        @pl.when(jnp.logical_and(i >= 96, i < 104))
        def _():
            out_b_item(i - 96, fl)

        @pl.when(jnp.logical_and(i >= 105, i < 109))
        def _():
            out_a_item(i - 105, fl)

        @pl.when(jnp.logical_or(i == 104, i >= 109))
        def _():
            fl()

    lax.fori_loop(0, 16, make_main(high0, hook0, _nop, True, False), 0)
    lax.fori_loop(16, 80, make_main(high1, hook1, extra1, False, False), 0)
    lax.fori_loop(80, N_MAIN, make_main(high2, hook2, extra2, False, True), 0)

    finalize_o(13)
    softmax_a()

    def g14_body(r, carry):
        s0 = (r & 3) * 4
        nx = r + 4
        for t in range(4):
            low_v8(0, r, t, s0 + t).wait()
            high_wo(6, 1, r * 32 + t * 8, 8, 0, 512, S_WO + 2).start(priority=HI)
            low_v8(nx >> 3, nx & 7, t, s0 + t).start(priority=LO)
        oacc_ref[...] = v_part(14, r)
        k_work(15, r)
        return carry
    lax.fori_loop(0, 8, g14_body, 0)

    finalize_o(14)
    softmax_a()

    def v15_body(r, carry):
        s0 = (r & 3) * 4
        for t in range(4):
            low_v8(1, r, t, s0 + t).wait()

            @pl.when(r < NBIG)
            def _():
                high_wo(6, 1, 256 + r * 64 + t * 16, 16, 0, 512, S_WO + 2).start(priority=HI)

            @pl.when(jnp.logical_and(r >= NBIG, r < 8 - NBIG))
            def _():
                high_wo(6, 1, 256 + NBIG * 32 + r * 32 + t * 8, 8, 0, 512,
                        S_WO + 2).start(priority=HI)

            @pl.when(r < 4)
            def _():
                low_v8(1, r + 4, t, s0 + t).start(priority=LO)

            @pl.when(jnp.logical_and(r >= 4, r < 6))
            def _():
                low_wo(s0 + t, s0 + t).start(priority=LO)

            if t == 1:
                @pl.when(r == 1)
                def _():
                    wait_all(wo_buf.at[pl.ds(4, 2)], S_WO + 1)

                @pl.when(jnp.logical_and(r >= 1, r < 3))
                def _():
                    out_a_item(r + 3)

                @pl.when(r == 4)
                def _():
                    l = jnp.sum(psum_ref[...], axis=1, keepdims=True)
                    psum_ref[...] = jnp.broadcast_to(1.0 / l, (8, 128))
        oacc_ref[...] = v_part(15, r)
        return carry
    lax.fori_loop(0, 7, v15_body, 0)

    for t in range(4):
        low_v8(1, 7, t, 12 + t).wait()
    oa_ref[3, 24:32, :] = v_part(15, 7) * psum_ref[...]
    wait_all(wo_buf.at[pl.ds(6, 1)], S_WO + 2)
    for n in range(2):
        low_wo(n, n).wait()
    o32 = oa_ref[3]
    part_ref[0:4, :] = rowsum(acca_ref[...] + out_part(o32, wo_buf.at[6], 0, 0, 4)
                              + out_part(o32, wo_buf.at[7], 4, 0, 1))
    for j in range(5, 8):
        olast_ref[0:4, (j - 5) * 128:(j - 4) * 128] = o32.reshape(4, 8, 128)[:, j, :]
    for n in range(2, NSPLIT):
        low_wo(n, n).wait()
    k1 = NSPLIT * 64
    part_ref[...] = part_ref[...] + _dot(
        olast_ref[:, 0:k1 - 128].astype(BF16), wo_buf[7, 128:k1, :])
    lhs = olast_ref[:, k1 - 128:384].astype(BF16)
    for n in range(NSPLIT, 8):
        low_wo(n, n).wait()
    res = part_ref[...] + _dot(lhs, wo_buf[7, k1:512, :])
    obuf[0] = res[0:4, :].astype(obuf.dtype)
    out_copy(0).start(priority=HI)
    out_copy(1).wait()
    out_copy(0).wait()


@jax.jit
def pallas_concat_heads__sliding_block_cached__compressed_kv_cla__decode_kernel(
    A_x: jax.Array,
    A_k_cache: jax.Array,
    A_v_cache: jax.Array,
    A_wq: jax.Array,
    A_wo: jax.Array,
    B_x: jax.Array,
    B_c_kv: jax.Array,
    B_w_q: jax.Array,
    B_w_uk: jax.Array,
    B_w_uv: jax.Array,
    B_w_o: jax.Array,
):
    B, Sq, D = A_x.shape
    _, H, Sk, Dh = A_k_cache.shape
    W = min(4096, max(256, Sk // 4))
    assert (B, Sq, D, H, Sk, Dh, W) == (4, 1, 512, 32, 4096, 128, 1024)
    assert B_c_kv.shape == (4, 4096, 512) and B_w_q.shape == (512, 32, 128)

    def body(*refs):
        _kernel(*refs, win_off=Sk - W, scale=float(Dh) ** -0.5)

    vm = pltpu.VMEM
    scratch = [
        vm((2, 16, 1024, 128), BF16),
        vm((16, 1024, 512), BF16),
        vm((4, 128, 4096), BF16),
        vm((8, 512, 512), BF16),
        vm((4, 128, 4, 8, 128), BF16),
        vm((4, 128, 4, 8, 128), BF16),
        vm((4, 128, 4, 8, 128), BF16),
        vm((4, 2, 512, 512), BF16),
        vm((4, 512), BF16),
        vm((4, 512), BF16),
        vm((128, 1024), BF16),
        vm((32, 512), BF16),
        vm((2, 32, 2048), BF16),
        vm((4, 32, 128), F32),
        vm((8, 8, 128), F32),
        vm((8, 8, 128), F32),
        vm((8, 128), F32),
        vm((8, 128), F32),
        vm((4, 32, 128), F32),
        vm((4, 32, 128), F32),
        vm((4, 4, 4, 8, 128), F32),
        vm((8, 32, 512), F32),
        vm((32, 128), F32),
        vm((32, 128), F32),
        vm((32, 512), F32),
        vm((4, 4, 4, 8, 128), F32),
        vm((4, 32, 128), F32),
        vm((32, 512), F32),
        vm((32, 512), F32),
        vm((8, 384), F32),
        vm((8, 512), F32),
        vm((2, 4, 512), A_x.dtype),
        pltpu.SemaphoreType.DMA((NS,)),
        pltpu.SemaphoreType.DMA((N_HSEM,)),
        pltpu.SemaphoreType.DMA((4,)),
    ]
    out = pl.pallas_call(
        body,
        out_shape=jax.ShapeDtypeStruct((B, 2 * D), A_x.dtype),
        in_specs=[pl.BlockSpec(memory_space=pl.ANY)] * 11,
        out_specs=pl.BlockSpec(memory_space=pl.ANY),
        scratch_shapes=scratch,
        compiler_params=pltpu.CompilerParams(
            vmem_limit_bytes=64 * 1024 * 1024,
            disable_bounds_checks=True,
            disable_semaphore_checks=True,
        ),
    )(
        A_x.reshape(B, D),
        A_k_cache.reshape(B * H, Sk, Dh),
        A_v_cache.reshape(B * H, Sk, Dh),
        A_wq.reshape(4, 128, 4096),
        A_wo.reshape(8, 512, 512),
        B_x.reshape(B, D),
        B_c_kv.reshape(16, 1024, 512),
        B_w_q.reshape(4, 128, 4, 8, 128),
        B_w_uk.reshape(4, 128, 4, 8, 128),
        B_w_uv.reshape(4, 128, 4, 8, 128),
        B_w_o.reshape(4, 2, 512, 512),
    )
    return out.reshape(B, Sq, 2 * D)
```

```python
import jax
import jax.numpy as jnp
from jax import lax
import jax.experimental.pallas as pl
import jax.experimental.pallas.tpu as pltpu

F32 = jnp.float32
BF16 = jnp.bfloat16
_NT = (((1,), (1,)), ((), ()))
_NN = (((1,), (0,)), ((), ()))

LO, HI = 1, 0
NS = 16
N_MAIN = 112

S_WQ = 0
S_WBQ = 4
S_WUK = 5
S_WUV = 6
S_WBO = 7
S_WO = 8
N_HSEM = 11
NSPLIT = 6
NBIG = 3
C_RUNS = (((0, 2, 960), (2, 6, 0)), ((8, 8, 0),))
WLAG = 256
ROT = 14
ROTC = ((32 - ROT) % 32) * 128
_PW = ROT // 4
WO_RUNS = [(a, n) for a, n in ((0, _PW), (_PW, 1), (_PW + 1, 3 - _PW)) if n > 0] if ROT else [(0, 4)]


def _dot(a, b):
    return lax.dot_general(a, b, _NN, preferred_element_type=F32)


def _dot_nt(a, b):
    return lax.dot_general(a, b, _NT, preferred_element_type=F32)


def _mo(x, m):
    return x if isinstance(x, int) else pl.multiple_of(x, m)


def _nop(_=None):
    return None


def _kernel(xa_hbm, k_hbm, v_hbm, wq_hbm, wo_hbm, xb_hbm, c_hbm, wbq_hbm, wuk_hbm,
            wuv_hbm, wbo_hbm, out_hbm,
            kvbuf, cbuf, wq_buf, wo_buf, wbq_buf, wuk_buf, wuv_buf, wbo_buf,
            xa_buf, xb_buf, e0_ref, xa32_ref, xexp_ref,
            qa_ref, sa_ref, pa_ref, psum_ref, oacc_ref, oa_ref,
            qb_ref, qabs_ref, sb_ref, mb_ref, lb_ref, cacc_ref, cc_ref, ctx_ref,
            acca_ref, accb_ref, olast_ref, part_ref, obuf,
            lsem, hsem, xsem, *, win_off, scale):

    def start_c(it, t, sem, h):
        row = _mo(it * 16 + (t >> 1) * 8, 8)
        col = (t & 1) * 256
        for seg, n, lag in C_RUNS[h]:
            pltpu.make_async_copy(
                c_hbm.at[pl.ds(seg, n), pl.ds(_mo((row + lag) & 1023, 8), 8), pl.ds(col, 256)],
                cbuf.at[pl.ds(seg, n), pl.ds(row, 8), pl.ds(col, 256)],
                lsem.at[sem + h * NS]).start(priority=LO)

    def wait_c(it, t, sem, h):
        dst = cbuf.at[pl.ds(h * 8, 8), pl.ds(_mo(it * 16 + (t >> 1) * 8, 8), 8),
                      pl.ds((t & 1) * 256, 256)]
        pltpu.make_async_copy(dst, dst, lsem.at[sem + h * NS]).wait()

    def batch_of(g):
        return (g >> 1) & 3

    def hg_of(g):
        return (g >> 3) * 2 + (g & 1)

    def nprev_of(g):
        n = ROT - hg_of(g) * 8
        return max(0, min(8, n)) if isinstance(n, int) else jnp.clip(n, 0, 8)

    def low_heads(src, kv, head, slot, n, r, t, sem, lag=0):
        row = _mo(r * 128 + t * 16, 16)
        srow = (row + lag) & 1023 if lag else row
        return pltpu.make_async_copy(
            src.at[pl.ds(head, n), pl.ds(_mo(win_off + srow, 16), 16), :],
            kvbuf.at[kv, pl.ds(slot, n), pl.ds(row, 16), :],
            lsem.at[sem])

    def start16(src, kv, sg, r, t, sem):
        head = (sg & 3) * 32 + (sg >> 2) * 16 - ROT
        low_heads(src, kv, head, 0, 16, r, t, sem).start(priority=LO)

    def start16_first(src, kv, r, t, sem):
        if ROT:
            low_heads(src, kv, 128 - ROT, 0, ROT, r, t, sem).start(priority=LO)
        low_heads(src, kv, 0, ROT, 16 - ROT, r, t, sem, WLAG).start(priority=LO)

    def start_k0(r, t, sem, h):
        n = max(0, min(8, ROT - h * 8))
        if n:
            low_heads(k_hbm, 0, 128 - ROT + h * 8, h * 8, n, r, t, sem + h * NS).start(priority=LO)
        if n < 8:
            low_heads(k_hbm, 0, h * 8 + n - ROT, h * 8 + n, 8 - n, r, t, sem + h * NS,
                      WLAG).start(priority=LO)

    def wait_k0(r, t, sem, h):
        dst = kvbuf.at[0, pl.ds(h * 8, 8), pl.ds(_mo(r * 128 + t * 16, 16), 16), :]
        pltpu.make_async_copy(dst, dst, lsem.at[sem + h * NS]).wait()

    def wait16(kv, r, t, sem):
        dst = kvbuf.at[kv, :, pl.ds(_mo(r * 128 + t * 16, 16), 16), :]
        pltpu.make_async_copy(dst, dst, lsem.at[sem]).wait()

    def low_v8(e, r, t, sem):
        row = _mo(r * 128 + t * 32, 32)
        return pltpu.make_async_copy(
            v_hbm.at[pl.ds(112 - ROT + e * 8, 8), pl.ds(_mo(win_off + row, 32), 32), :],
            kvbuf.at[1, pl.ds(e * 8, 8), pl.ds(row, 32), :],
            lsem.at[sem])

    def wo_copy(p0, np_, row, rows, col, cols, sem):
        flat = (p0 * 512 + row + ROTC) & 4095
        return pltpu.make_async_copy(
            wo_hbm.at[pl.ds(flat >> 9, np_), pl.ds(_mo(flat & 511, 8), rows), pl.ds(col, cols)],
            wo_buf.at[pl.ds(p0, np_), pl.ds(_mo(row, 8), rows), pl.ds(col, cols)], sem)

    def low_wo(n, sem):
        return wo_copy(7, 1, n * 64, 64, 0, 512, lsem.at[sem])

    def start_wq(row, col, cols, sem):
        row = _mo(row, 8)
        src = (col + ROTC) % 4096
        first = min(cols, 4096 - src)
        for c0, s0, n in ((col, src, first), (col + first, 0, cols - first)):
            if n:
                pltpu.make_async_copy(
                    wq_hbm.at[:, pl.ds(row, 8), pl.ds(s0, n)],
                    wq_buf.at[:, pl.ds(row, 8), pl.ds(c0, n)], hsem.at[sem]).start(priority=HI)

    def high_3d(src, dst, row, hg, nhg, sem):
        return pltpu.make_async_copy(
            src.at[:, row, pl.ds(hg, nhg)], dst.at[:, row, pl.ds(hg, nhg)], hsem.at[sem])

    def high_wbo(half, row, col):
        row = _mo(row, 8)
        return pltpu.make_async_copy(
            wbo_hbm.at[:, half, pl.ds(row, 8), pl.ds(col, 256)],
            wbo_buf.at[:, half, pl.ds(row, 8), pl.ds(col, 256)], hsem.at[S_WBO])

    def high_wo(p0, np_, row, rows, col, cols, sem):
        return wo_copy(p0, np_, row, rows, col, cols, hsem.at[sem])

    def out_copy(h):
        return pltpu.make_async_copy(
            obuf.at[h], out_hbm.at[:, pl.ds(h * 512, 512)], xsem.at[2 + h])

    def wait_all(buf, sem):
        pltpu.make_async_copy(buf, buf, hsem.at[sem]).wait()

    for r in range(2):
        for t in range(8):
            for h in range(2):
                start_k0(r, t, r * 8 + t, h)
    cp_xa = pltpu.make_async_copy(xa_hbm, xa_buf, xsem.at[0])
    cp_xb = pltpu.make_async_copy(xb_hbm, xb_buf, xsem.at[1])
    cp_xa.start(priority=HI)
    cp_xb.start(priority=HI)

    row8 = lax.broadcasted_iota(jnp.int32, (8, 128), 0)
    row32 = lax.broadcasted_iota(jnp.int32, (32, 128), 0) & 7
    lane32 = lax.broadcasted_iota(jnp.int32, (32, 128), 1) & 7

    def e0_body(i, c):
        r0 = pl.multiple_of(i * 16, 16)
        rr = lax.broadcasted_iota(jnp.int32, (16, 1024), 0) + r0
        cc = lax.broadcasted_iota(jnp.int32, (16, 1024), 1) >> 3
        e0_ref[pl.ds(r0, 16), :] = jnp.where(rr == cc, 1.0, 0.0).astype(BF16)
        return c
    lax.fori_loop(0, 8, e0_body, 0)

    qa_ref[...] = jnp.zeros(qa_ref.shape, F32)
    qb_ref[...] = jnp.zeros(qb_ref.shape, F32)
    ctx_ref[...] = jnp.zeros(ctx_ref.shape, F32)
    acca_ref[...] = jnp.zeros(acca_ref.shape, F32)
    accb_ref[...] = jnp.zeros(accb_ref.shape, F32)
    mb_ref[...] = jnp.zeros(mb_ref.shape, F32)
    lb_ref[...] = jnp.zeros(lb_ref.shape, F32)
    cacc_ref[...] = jnp.zeros(cacc_ref.shape, F32)
    olast_ref[...] = jnp.zeros(olast_ref.shape, F32)
    part_ref[...] = jnp.zeros(part_ref.shape, F32)
    oa_ref[...] = jnp.zeros(oa_ref.shape, F32)

    def expand(c32, fl=_nop):
        ce = _dot(c32.astype(BF16), e0_ref[...])
        fl()
        return jnp.concatenate(
            [jnp.where(row32 == lane32, ce[:, 128 * k:128 * k + 128], 0.0).astype(BF16)
             for k in range(8)], axis=1)

    def x_prep():
        cp_xa.wait()
        cp_xb.wait()
        xa = xa_buf[...].astype(F32)
        xb = xb_buf[...].astype(F32)
        xa32_ref[...] = jnp.concatenate(
            [jnp.broadcast_to(xa[b:b + 1, :], (8, 512)) for b in range(4)], axis=0).astype(BF16)
        xb32 = jnp.concatenate(
            [jnp.broadcast_to(xb[b:b + 1, :], (8, 512)) for b in range(4)], axis=0)
        for u in range(4):
            xexp_ref[u >> 1, :, (u & 1) * 1024:(u & 1) * 1024 + 1024] = expand(
                xb32[:, 128 * u:128 * u + 128])

    def qa_item(hg, half):
        col = pl.multiple_of(hg * 1024 + half * 512, 512)
        w = wq_buf[:, :, pl.ds(col, 512)].reshape(512, 512)
        r = _dot(xa32_ref[...], w)
        new = qa_ref[hg]
        for j in range(4):
            new = jnp.where(row32 == half * 4 + j, r[:, 128 * j:128 * j + 128], new)
        qa_ref[hg] = new

    def qb_item(n):
        hg = n >> 1
        half = n & 1
        w = wbq_buf[pl.ds(half * 2, 2), :, hg].reshape(2048, 128)
        qb_ref[hg] = qb_ref[hg] + _dot(xexp_ref[half], w)

    def qabs_item(n, fl):
        hg = n & 3
        u = n >> 2
        q = qb_ref[hg].astype(BF16)
        w = wuk_buf[u, :, hg].reshape(1024, 128)
        r = _dot_nt(q, w)
        fl()
        r = jnp.concatenate(
            [jnp.where(row32 == lane32, r[:, 128 * k:128 * k + 128], 0.0).astype(BF16)
             for k in range(8)], axis=1)
        qa = _dot_nt(r, e0_ref[...])
        for b in range(4):
            qabs_ref[u, b, hg] = qa[8 * b:8 * b + 8, :]

    def score_item(b, n, fl):
        qa = jnp.concatenate(
            [qabs_ref[u, b].reshape(32, 128).astype(BF16) for u in range(4)], axis=1)
        seg = b * 4 + (n >> 1)
        m = jnp.where(n == 0, -jnp.inf, mb_ref[...])
        for k in range(4):
            row = pl.multiple_of((n & 1) * 512 + k * 128, 128)
            s = _dot_nt(qa, cbuf[seg, pl.ds(row, 128), :])
            if k == 0:
                fl()
            sb_ref[n, :, 128 * k:128 * k + 128] = s
            m = jnp.maximum(m, s)
        mb_ref[...] = m

    def max_b():
        mb_ref[...] = jnp.broadcast_to(jnp.max(mb_ref[...], axis=1, keepdims=True), (32, 128))

    def pv_item(b, n, fl):
        m = mb_ref[...]
        ps = [jnp.exp((sb_ref[n, :, 128 * k:128 * k + 128] - m) * scale) for k in range(4)]
        first = n == 0
        lb_ref[...] = jnp.where(first, 0.0, lb_ref[...]) + ((ps[0] + ps[1]) + (ps[2] + ps[3]))
        seg = b * 4 + (n >> 1)
        acc = jnp.where(first, 0.0, cacc_ref[...])
        for k in range(4):
            row = pl.multiple_of((n & 1) * 512 + k * 128, 128)
            d = _dot(ps[k].astype(BF16), cbuf[seg, pl.ds(row, 128), :])
            if k == 0:
                fl()
            acc = acc + d
        cacc_ref[...] = acc

    def norm_b(b):
        inv = 1.0 / jnp.sum(lb_ref[...], axis=1, keepdims=True)
        res = cacc_ref[...] * inv
        for u in range(4):
            cc_ref[u, b] = res[:, 128 * u:128 * u + 128].reshape(4, 8, 128)

    def ctx_item(n, fl):
        hg = n >> 2
        u = n & 3
        c32 = jnp.concatenate([cc_ref[u, bb, hg] for bb in range(4)], axis=0)
        w = wuv_buf[u, :, hg].reshape(1024, 128)
        ctx_ref[hg] = ctx_ref[hg] + _dot(expand(c32, fl), w)

    def out_part(o32, w_half, j0, jj, nj, fl=_nop):
        acc = None
        for j in range(jj, jj + nj):
            d = _dot(jnp.where(row32 == j0 + j, o32, 0.0).astype(BF16),
                     w_half[j * 128:j * 128 + 128, :])
            if j == jj:
                fl()
            acc = d if acc is None else acc + d
        return acc

    def out_a_item(n, fl=_nop):
        acca_ref[...] = acca_ref[...] + out_part(
            oa_ref[n >> 1], wo_buf.at[n], (n & 1) * 4, 0, 4, fl)

    def out_b_item(n, fl=_nop):
        accb_ref[...] = accb_ref[...] + out_part(
            ctx_ref[n >> 1], wbo_buf.at[n >> 1, n & 1], (n & 1) * 4, 0, 4, fl)

    def rowsum(acc):
        return jnp.sum(acc.reshape(4, 8, 512), axis=1)

    def k_work(g, r):
        hg, b = hg_of(g), batch_of(g)
        q = jnp.where(row8 < nprev_of(g),
                      qa_ref[hg, pl.ds(_mo(((b + 3) & 3) * 8, 8), 8), :],
                      qa_ref[hg, pl.ds(_mo(b * 8, 8), 8), :]).astype(BF16)
        row = pl.multiple_of(r * 128, 128)
        h0 = (g & 1) * 8
        s = jnp.zeros((8, 128), F32)
        for j in range(8):
            sj = _dot_nt(q, kvbuf[0, h0 + j, pl.ds(row, 128), :])
            s = jnp.where(row8 == j, sj, s)
        sa_ref[r] = s

    def v_part(g, r):
        p = pa_ref[r].astype(BF16)
        row = _mo(r * 128, 128)
        h0 = (g & 1) * 8
        o = jnp.zeros((8, 128), F32)
        for j in range(8):
            oj = _dot(p, kvbuf[1, h0 + j, pl.ds(row, 128), :])
            o = jnp.where(row8 == j, oj, o)
        return oacc_ref[...] + o

    def finalize_o(g):
        l = jnp.sum(psum_ref[...], axis=1, keepdims=True)
        o = oacc_ref[...] * (1.0 / l)
        hg, b = hg_of(g), batch_of(g)
        prev = row8 < nprev_of(g)
        rp = pl.ds(_mo(((b + 3) & 3) * 8, 8), 8)
        rc = pl.ds(_mo(b * 8, 8), 8)
        oa_ref[hg, rp, :] = jnp.where(prev, o, oa_ref[hg, rp, :])
        oa_ref[hg, rc, :] = jnp.where(prev, oa_ref[hg, rc, :], o)

    def softmax_a():
        s = sa_ref[...]
        m = jnp.max(jnp.max(s, axis=0), axis=1, keepdims=True)
        p = jnp.exp((s - m[None]) * scale)
        pa_ref[...] = p
        psum_ref[...] = jnp.sum(p, axis=0)
        oacc_ref[...] = jnp.zeros((8, 128), F32)

    def k0_tick(r, t, s0, h):
        wait_k0(r, t, s0 + t, h)
        start_wq(r * 16 + (t >> 2) * 8, (t & 3) * 512 + h * 256, 256, S_WQ)

    def k0a_body(r, carry):
        s0 = (r & 1) * 8
        for t in range(8):
            for h in range(2):
                k0_tick(r, t, s0, h)
                start_k0(r + 2, t, s0 + t, h)
        return carry
    lax.fori_loop(0, 6, k0a_body, 0)

    x_prep()

    def k0b_body(r, carry):
        s0 = r * 8
        for t in range(8):
            for h in range(2):
                k0_tick(r + 6, t, s0, h)
                start_c(r * 2 + (t >> 2), t & 3, s0 + t, h)
        return carry
    lax.fori_loop(0, 2, k0b_body, 0)

    def c0_body(it, carry):
        s0 = (it & 3) * 4
        for t in range(4):
            for h in range(2):
                wait_c(it, t, s0 + t, h)
                high_3d(wbq_hbm, wbq_buf, it * 4 + t, h * 2, 2, S_WBQ).start(priority=HI)
                start_c(it + 4, t, s0 + t, h)

        @pl.when(it == 1)
        def _():
            wait_all(wq_buf.at[:, :, pl.ds(0, 2048)], S_WQ)

        @pl.when(jnp.logical_and(it >= 1, it < 5))
        def _():
            qa_item((it - 1) >> 1, (it - 1) & 1)

        @pl.when(jnp.logical_and(it >= 5, it < 13))
        def _():
            k_work(0, it - 5)

        @pl.when(it == 13)
        def _():
            softmax_a()
        return carry
    lax.fori_loop(0, 32, c0_body, 0)

    def c1_tick(it, t, s0, h):
        wait_c(32 + it, t, s0 + t, h)
        high_3d(wuk_hbm, wuk_buf, it * 4 + t, h * 2, 2, S_WUK).start(priority=HI)

    def c1_body(it, carry):
        s0 = (it & 3) * 4
        for t in range(4):
            for h in range(2):
                c1_tick(it, t, s0, h)
                start_c(36 + it, t, s0 + t, h)

        @pl.when(it == 1)
        def _():
            wait_all(wbq_buf, S_WBQ)

        @pl.when(jnp.logical_and(it >= 1, it < 9))
        def _():
            qb_item(it - 1)
        return carry
    lax.fori_loop(0, 28, c1_body, 0)

    def c1b_body(r, carry):
        for t in range(8):
            for h in range(2):
                c1_tick(28 + r * 2 + (t >> 2), t & 3, r * 8 + (t >> 2) * 4, h)
            start16_first(v_hbm, 1, r, t, r * 8 + t)
        return carry
    lax.fori_loop(0, 2, c1b_body, 0)

    def make_main(high, hook, extra, first, last):
        def body(i, carry):
            g = i >> 3
            r = i & 7
            i2 = i + 2
            g2 = i2 >> 3
            r2 = i2 & 7
            sg2 = (g2 + 1) >> 1
            odd2 = (g2 & 1) == 1
            s0 = (i & 1) * 8
            kv = 1 - (g & 1)

            def tick(t, with_high=True):
                wait16(kv, r, t, s0 + t)
                if with_high:
                    high(i, t)

                @pl.when(odd2)
                def _():
                    start16(k_hbm, 0, sg2, r2, t, s0 + t)

                if first:
                    @pl.when(i2 < 8)
                    def _():
                        start16_first(v_hbm, 1, r2, t, s0 + t)

                    @pl.when(i2 >= 16)
                    def _():
                        start16(v_hbm, 1, sg2, r2, t, s0 + t)
                elif not last:
                    @pl.when(jnp.logical_not(odd2))
                    def _():
                        start16(v_hbm, 1, sg2, r2, t, s0 + t)
                else:
                    @pl.when(jnp.logical_and(jnp.logical_not(odd2), i2 < N_MAIN))
                    def _():
                        start16(v_hbm, 1, sg2, r2, t, s0 + t)

                    @pl.when(i2 >= N_MAIN)
                    def _():
                        low_v8(0, 2 * r2 + (t >> 2), t & 3, s0 + t).start(priority=LO)

            tick(0)
            tick(1)

            @pl.when(jnp.logical_and(r == 0, i > 0))
            def _():
                finalize_o(g - 1)
                softmax_a()

            extra(i)
            tick(2)
            tick(3)
            hook(i, lambda: high(i, 5))
            tick(4)
            tick(5, False)
            tick(6)
            tick(7)
            oacc_ref[...] = v_part(g, r)
            k_work(g + 1, r)
            return carry
        return body

    def high0(i, t):
        start_wq(i * 8, 2048 + t * 256, 256, S_WQ + 1)

    def hook0(i, fl):
        @pl.when(i == 0)
        def _():
            wait_all(wuk_buf, S_WUK)

        qabs_item(i, fl)

    def high1(i, t):
        @pl.when(i < 48)
        def _():
            high_3d(wuv_hbm, wuv_buf, (i - 16) * 4 + (t >> 1), (t & 1) * 2, 2,
                    S_WUV).start(priority=HI)

        @pl.when(i >= 48)
        def _():
            high_wbo((i >> 4) - 3, (i & 15) * 32 + (t >> 1) * 8, (t & 1) * 256).start(priority=HI)

    def extra1(i):
        n = i - 16

        @pl.when(i == 25)
        def _():
            wait_all(wq_buf.at[:, :, pl.ds(2048, 2048)], S_WQ + 1)

        @pl.when(jnp.logical_and(i >= 25, i < 29))
        def _():
            qa_item(2 + ((i - 25) >> 1), (i - 25) & 1)

        @pl.when((n & 15) == 8)
        def _():
            max_b()

        @pl.when(jnp.logical_and((n & 15) == 1, n > 16))
        def _():
            norm_b((n >> 4) - 1)

    def hook1(i, fl):
        n = i - 16

        @pl.when((n & 8) == 0)
        def _():
            score_item(n >> 4, n & 7, fl)

        @pl.when((n & 8) != 0)
        def _():
            pv_item(n >> 4, n & 7, fl)

    def high2(i, t):
        row = (i & 15) * 32 + (t >> 1) * 8

        @pl.when(i < 96)
        def _():
            for p0, np_ in WO_RUNS:
                high_wo(p0, np_, row, 8, (t & 1) * 256, 256, S_WO).start(priority=HI)

        @pl.when(i >= 96)
        def _():
            high_wo(4, 2, row, 8, (t & 1) * 256, 256, S_WO + 1).start(priority=HI)

    def extra2(i):
        @pl.when(i == 80)
        def _():
            wait_all(wuv_buf, S_WUV)
            norm_b(3)

        @pl.when(i == 96)
        def _():
            wait_all(wbo_buf, S_WBO)

        @pl.when(i == 105)
        def _():
            wait_all(wo_buf.at[pl.ds(0, 4)], S_WO)
            obuf[1] = rowsum(accb_ref[...]).astype(obuf.dtype)
            out_copy(1).start(priority=HI)

    def hook2(i, fl):
        @pl.when(i < 96)
        def _():
            ctx_item(i - 80, fl)

        @pl.when(jnp.logical_and(i >= 96, i < 104))
        def _():
            out_b_item(i - 96, fl)

        @pl.when(jnp.logical_and(i >= 105, i < 109))
        def _():
            out_a_item(i - 105, fl)

        @pl.when(jnp.logical_or(i == 104, i >= 109))
        def _():
            fl()

    lax.fori_loop(0, 16, make_main(high0, hook0, _nop, True, False), 0)
    lax.fori_loop(16, 80, make_main(high1, hook1, extra1, False, False), 0)
    lax.fori_loop(80, N_MAIN, make_main(high2, hook2, extra2, False, True), 0)

    finalize_o(13)
    softmax_a()

    def g14_body(r, carry):
        s0 = (r & 3) * 4
        nx = r + 4
        for t in range(4):
            low_v8(0, r, t, s0 + t).wait()
            high_wo(6, 1, r * 32 + t * 8, 8, 0, 512, S_WO + 2).start(priority=HI)
            low_v8(nx >> 3, nx & 7, t, s0 + t).start(priority=LO)
        oacc_ref[...] = v_part(14, r)
        k_work(15, r)
        return carry
    lax.fori_loop(0, 8, g14_body, 0)

    finalize_o(14)
    softmax_a()

    def v15_body(r, carry):
        s0 = (r & 3) * 4
        for t in range(4):
            low_v8(1, r, t, s0 + t).wait()

            @pl.when(r < NBIG)
            def _():
                high_wo(6, 1, 256 + r * 64 + t * 16, 16, 0, 512, S_WO + 2).start(priority=HI)

            @pl.when(jnp.logical_and(r >= NBIG, r < 8 - NBIG))
            def _():
                high_wo(6, 1, 256 + NBIG * 32 + r * 32 + t * 8, 8, 0, 512,
                        S_WO + 2).start(priority=HI)

            @pl.when(r < 4)
            def _():
                low_v8(1, r + 4, t, s0 + t).start(priority=LO)

            @pl.when(jnp.logical_and(r >= 4, r < 6))
            def _():
                low_wo(s0 + t, s0 + t).start(priority=LO)

            if t == 1:
                @pl.when(r == 1)
                def _():
                    wait_all(wo_buf.at[pl.ds(4, 2)], S_WO + 1)

                @pl.when(jnp.logical_and(r >= 1, r < 3))
                def _():
                    out_a_item(r + 3)

                @pl.when(r == 4)
                def _():
                    l = jnp.sum(psum_ref[...], axis=1, keepdims=True)
                    psum_ref[...] = jnp.broadcast_to(1.0 / l, (8, 128))
        oacc_ref[...] = v_part(15, r)
        return carry
    lax.fori_loop(0, 7, v15_body, 0)

    for t in range(4):
        low_v8(1, 7, t, 12 + t).wait()
    oa_ref[3, 24:32, :] = v_part(15, 7) * psum_ref[...]
    wait_all(wo_buf.at[pl.ds(6, 1)], S_WO + 2)
    for n in range(2):
        low_wo(n, n).wait()
    o32 = oa_ref[3]
    part_ref[0:4, :] = rowsum(acca_ref[...] + out_part(o32, wo_buf.at[6], 0, 0, 4)
                              + out_part(o32, wo_buf.at[7], 4, 0, 1))
    for j in range(5, 8):
        olast_ref[0:4, (j - 5) * 128:(j - 4) * 128] = o32.reshape(4, 8, 128)[:, j, :]
    for n in range(2, NSPLIT):
        low_wo(n, n).wait()
    k1 = NSPLIT * 64
    part_ref[...] = part_ref[...] + _dot(
        olast_ref[:, 0:k1 - 128].astype(BF16), wo_buf[7, 128:k1, :])
    lhs = olast_ref[:, k1 - 128:384].astype(BF16)
    for n in range(NSPLIT, 8):
        low_wo(n, n).wait()
    res = part_ref[...] + _dot(lhs, wo_buf[7, k1:512, :])
    obuf[0] = res[0:4, :].astype(obuf.dtype)
    out_copy(0).start(priority=HI)
    out_copy(1).wait()
    out_copy(0).wait()


@jax.jit
def pallas_concat_heads__sliding_block_cached__compressed_kv_cla__decode_kernel(
    A_x: jax.Array,
    A_k_cache: jax.Array,
    A_v_cache: jax.Array,
    A_wq: jax.Array,
    A_wo: jax.Array,
    B_x: jax.Array,
    B_c_kv: jax.Array,
    B_w_q: jax.Array,
    B_w_uk: jax.Array,
    B_w_uv: jax.Array,
    B_w_o: jax.Array,
):
    B, Sq, D = A_x.shape
    _, H, Sk, Dh = A_k_cache.shape
    W = min(4096, max(256, Sk // 4))
    assert (B, Sq, D, H, Sk, Dh, W) == (4, 1, 512, 32, 4096, 128, 1024)
    assert B_c_kv.shape == (4, 4096, 512) and B_w_q.shape == (512, 32, 128)

    def body(*refs):
        _kernel(*refs, win_off=Sk - W, scale=float(Dh) ** -0.5)

    vm = pltpu.VMEM
    scratch = [
        vm((2, 16, 1024, 128), BF16),
        vm((16, 1024, 512), BF16),
        vm((4, 128, 4096), BF16),
        vm((8, 512, 512), BF16),
        vm((4, 128, 4, 8, 128), BF16),
        vm((4, 128, 4, 8, 128), BF16),
        vm((4, 128, 4, 8, 128), BF16),
        vm((4, 2, 512, 512), BF16),
        vm((4, 512), BF16),
        vm((4, 512), BF16),
        vm((128, 1024), BF16),
        vm((32, 512), BF16),
        vm((2, 32, 2048), BF16),
        vm((4, 32, 128), F32),
        vm((8, 8, 128), F32),
        vm((8, 8, 128), F32),
        vm((8, 128), F32),
        vm((8, 128), F32),
        vm((4, 32, 128), F32),
        vm((4, 32, 128), F32),
        vm((4, 4, 4, 8, 128), F32),
        vm((8, 32, 512), F32),
        vm((32, 128), F32),
        vm((32, 128), F32),
        vm((32, 512), F32),
        vm((4, 4, 4, 8, 128), F32),
        vm((4, 32, 128), F32),
        vm((32, 512), F32),
        vm((32, 512), F32),
        vm((8, 384), F32),
        vm((8, 512), F32),
        vm((2, 4, 512), A_x.dtype),
        pltpu.SemaphoreType.DMA((2 * NS,)),
        pltpu.SemaphoreType.DMA((N_HSEM,)),
        pltpu.SemaphoreType.DMA((4,)),
    ]
    out = pl.pallas_call(
        body,
        out_shape=jax.ShapeDtypeStruct((B, 2 * D), A_x.dtype),
        in_specs=[pl.BlockSpec(memory_space=pl.ANY)] * 11,
        out_specs=pl.BlockSpec(memory_space=pl.ANY),
        scratch_shapes=scratch,
        compiler_params=pltpu.CompilerParams(
            vmem_limit_bytes=64 * 1024 * 1024,
            disable_bounds_checks=True,
            disable_semaphore_checks=True,
        ),
    )(
        A_x.reshape(B, D),
        A_k_cache.reshape(B * H, Sk, Dh),
        A_v_cache.reshape(B * H, Sk, Dh),
        A_wq.reshape(4, 128, 4096),
        A_wo.reshape(8, 512, 512),
        B_x.reshape(B, D),
        B_c_kv.reshape(16, 1024, 512),
        B_w_q.reshape(4, 128, 4, 8, 128),
        B_w_uk.reshape(4, 128, 4, 8, 128),
        B_w_uv.reshape(4, 128, 4, 8, 128),
        B_w_o.reshape(4, 2, 512, 512),
    )
    return out.reshape(B, Sq, 2 * D)
```

```python
import jax
import jax.numpy as jnp
from jax import lax
import jax.experimental.pallas as pl
import jax.experimental.pallas.tpu as pltpu

F32 = jnp.float32
BF16 = jnp.bfloat16
_NT = (((1,), (1,)), ((), ()))
_NN = (((1,), (0,)), ((), ()))

LO, HI = 1, 0
NS = 16
N_MAIN = 112

S_WQ = 0
S_WBQ = 4
S_WUK = 5
S_WUV = 6
S_WBO = 7
S_WO = 8
N_HSEM = 11
NSPLIT = 6
NBIG = 3
C_RUNS = (((0, 2, 960), (2, 6, 0)), ((8, 8, 0),))
FINE_T = (1, 2, 3, 6, 7)
WLAG = 256
ROT = 14
ROTC = ((32 - ROT) % 32) * 128
_PW = ROT // 4
WO_RUNS = [(a, n) for a, n in ((0, _PW), (_PW, 1), (_PW + 1, 3 - _PW)) if n > 0] if ROT else [(0, 4)]


def _dot(a, b):
    return lax.dot_general(a, b, _NN, preferred_element_type=F32)


def _dot_nt(a, b):
    return lax.dot_general(a, b, _NT, preferred_element_type=F32)


def _mo(x, m):
    return x if isinstance(x, int) else pl.multiple_of(x, m)


def _nop(_=None):
    return None


def _kernel(xa_hbm, k_hbm, v_hbm, wq_hbm, wo_hbm, xb_hbm, c_hbm, wbq_hbm, wuk_hbm,
            wuv_hbm, wbo_hbm, out_hbm,
            kvbuf, cbuf, wq_buf, wo_buf, wbq_buf, wuk_buf, wuv_buf, wbo_buf,
            xa_buf, xb_buf, e0_ref, xa32_ref, xexp_ref,
            qa_ref, sa_ref, pa_ref, psum_ref, oacc_ref, oa_ref,
            qb_ref, qabs_ref, sb_ref, mb_ref, lb_ref, cacc_ref, cc_ref, ctx_ref,
            acca_ref, accb_ref, olast_ref, part_ref, obuf,
            lsem, hsem, xsem, *, win_off, scale):

    def start_c(it, t, sem, h):
        row = _mo(it * 16 + (t >> 1) * 8, 8)
        col = (t & 1) * 256
        for seg, n, lag in C_RUNS[h]:
            pltpu.make_async_copy(
                c_hbm.at[pl.ds(seg, n), pl.ds(_mo((row + lag) & 1023, 8), 8), pl.ds(col, 256)],
                cbuf.at[pl.ds(seg, n), pl.ds(row, 8), pl.ds(col, 256)],
                lsem.at[sem + h * NS]).start(priority=LO)

    def wait_c(it, t, sem, h):
        dst = cbuf.at[pl.ds(h * 8, 8), pl.ds(_mo(it * 16 + (t >> 1) * 8, 8), 8),
                      pl.ds((t & 1) * 256, 256)]
        pltpu.make_async_copy(dst, dst, lsem.at[sem + h * NS]).wait()

    def batch_of(g):
        return (g >> 1) & 3

    def hg_of(g):
        return (g >> 3) * 2 + (g & 1)

    def nprev_of(g):
        n = ROT - hg_of(g) * 8
        return max(0, min(8, n)) if isinstance(n, int) else jnp.clip(n, 0, 8)

    def low_heads(src, kv, head, slot, n, r, t, sem, lag=0):
        row = _mo(r * 128 + t * 16, 16)
        srow = (row + lag) & 1023 if lag else row
        return pltpu.make_async_copy(
            src.at[pl.ds(head, n), pl.ds(_mo(win_off + srow, 16), 16), :],
            kvbuf.at[kv, pl.ds(slot, n), pl.ds(row, 16), :],
            lsem.at[sem])

    def span(h):
        return (0, 16, 0) if h is None else (h * 8, 8, h * NS)

    def start16(src, kv, sg, r, t, sem, h=None):
        s1, n, so = span(h)
        head = (sg & 3) * 32 + (sg >> 2) * 16 - ROT + s1
        low_heads(src, kv, head, s1, n, r, t, sem + so).start(priority=LO)

    def start16_first(src, kv, r, t, sem, h=None):
        s1, n, so = span(h)
        nb = max(0, min(n, ROT - s1))
        if nb:
            low_heads(src, kv, 128 - ROT + s1, s1, nb, r, t, sem + so).start(priority=LO)
        if nb < n:
            low_heads(src, kv, s1 + nb - ROT, s1 + nb, n - nb, r, t, sem + so,
                      WLAG).start(priority=LO)

    def wait16(kv, r, t, sem, h=None):
        s1, n, so = span(h)
        dst = kvbuf.at[kv, pl.ds(s1, n), pl.ds(_mo(r * 128 + t * 16, 16), 16), :]
        pltpu.make_async_copy(dst, dst, lsem.at[sem + so]).wait()

    def halves(t):
        return (0, 1) if t in FINE_T else (None,)

    def low_v8(e, r, t, sem):
        row = _mo(r * 128 + t * 32, 32)
        return pltpu.make_async_copy(
            v_hbm.at[pl.ds(112 - ROT + e * 8, 8), pl.ds(_mo(win_off + row, 32), 32), :],
            kvbuf.at[1, pl.ds(e * 8, 8), pl.ds(row, 32), :],
            lsem.at[sem])

    def wo_copy(p0, np_, row, rows, col, cols, sem):
        flat = (p0 * 512 + row + ROTC) & 4095
        return pltpu.make_async_copy(
            wo_hbm.at[pl.ds(flat >> 9, np_), pl.ds(_mo(flat & 511, 8), rows), pl.ds(col, cols)],
            wo_buf.at[pl.ds(p0, np_), pl.ds(_mo(row, 8), rows), pl.ds(col, cols)], sem)

    def low_wo(n, sem):
        return wo_copy(7, 1, n * 64, 64, 0, 512, lsem.at[sem])

    def start_wq(row, col, cols, sem):
        row = _mo(row, 8)
        src = (col + ROTC) % 4096
        first = min(cols, 4096 - src)
        for c0, s0, n in ((col, src, first), (col + first, 0, cols - first)):
            if n:
                pltpu.make_async_copy(
                    wq_hbm.at[:, pl.ds(row, 8), pl.ds(s0, n)],
                    wq_buf.at[:, pl.ds(row, 8), pl.ds(c0, n)], hsem.at[sem]).start(priority=HI)

    def high_3d(src, dst, row, hg, nhg, sem):
        return pltpu.make_async_copy(
            src.at[:, row, pl.ds(hg, nhg)], dst.at[:, row, pl.ds(hg, nhg)], hsem.at[sem])

    def high_wbo(half, row, col, cols):
        row = _mo(row, 8)
        return pltpu.make_async_copy(
            wbo_hbm.at[:, half, pl.ds(row, 8), pl.ds(col, cols)],
            wbo_buf.at[:, half, pl.ds(row, 8), pl.ds(col, cols)], hsem.at[S_WBO])

    def high_wo(p0, np_, row, rows, col, cols, sem):
        return wo_copy(p0, np_, row, rows, col, cols, hsem.at[sem])

    def out_copy(h):
        return pltpu.make_async_copy(
            obuf.at[h], out_hbm.at[:, pl.ds(h * 512, 512)], xsem.at[2 + h])

    def wait_all(buf, sem):
        pltpu.make_async_copy(buf, buf, hsem.at[sem]).wait()

    for r in range(2):
        for t in range(8):
            for h in range(2):
                start16_first(k_hbm, 0, r, t, r * 8 + t, h)
    cp_xa = pltpu.make_async_copy(xa_hbm, xa_buf, xsem.at[0])
    cp_xb = pltpu.make_async_copy(xb_hbm, xb_buf, xsem.at[1])
    cp_xa.start(priority=HI)
    cp_xb.start(priority=HI)

    row8 = lax.broadcasted_iota(jnp.int32, (8, 128), 0)
    row32 = lax.broadcasted_iota(jnp.int32, (32, 128), 0) & 7
    lane32 = lax.broadcasted_iota(jnp.int32, (32, 128), 1) & 7

    def e0_body(i, c):
        r0 = pl.multiple_of(i * 16, 16)
        rr = lax.broadcasted_iota(jnp.int32, (16, 1024), 0) + r0
        cc = lax.broadcasted_iota(jnp.int32, (16, 1024), 1) >> 3
        e0_ref[pl.ds(r0, 16), :] = jnp.where(rr == cc, 1.0, 0.0).astype(BF16)
        return c
    lax.fori_loop(0, 8, e0_body, 0)

    qa_ref[...] = jnp.zeros(qa_ref.shape, F32)
    qb_ref[...] = jnp.zeros(qb_ref.shape, F32)
    ctx_ref[...] = jnp.zeros(ctx_ref.shape, F32)
    acca_ref[...] = jnp.zeros(acca_ref.shape, F32)
    accb_ref[...] = jnp.zeros(accb_ref.shape, F32)
    mb_ref[...] = jnp.zeros(mb_ref.shape, F32)
    lb_ref[...] = jnp.zeros(lb_ref.shape, F32)
    cacc_ref[...] = jnp.zeros(cacc_ref.shape, F32)
    olast_ref[...] = jnp.zeros(olast_ref.shape, F32)
    part_ref[...] = jnp.zeros(part_ref.shape, F32)
    oa_ref[...] = jnp.zeros(oa_ref.shape, F32)

    def expand(c32, fl=_nop):
        ce = _dot(c32.astype(BF16), e0_ref[...])
        fl()
        return jnp.concatenate(
            [jnp.where(row32 == lane32, ce[:, 128 * k:128 * k + 128], 0.0).astype(BF16)
             for k in range(8)], axis=1)

    def x_prep():
        cp_xa.wait()
        cp_xb.wait()
        xa = xa_buf[...].astype(F32)
        xb = xb_buf[...].astype(F32)
        xa32_ref[...] = jnp.concatenate(
            [jnp.broadcast_to(xa[b:b + 1, :], (8, 512)) for b in range(4)], axis=0).astype(BF16)
        xb32 = jnp.concatenate(
            [jnp.broadcast_to(xb[b:b + 1, :], (8, 512)) for b in range(4)], axis=0)
        for u in range(4):
            xexp_ref[u >> 1, :, (u & 1) * 1024:(u & 1) * 1024 + 1024] = expand(
                xb32[:, 128 * u:128 * u + 128])

    def qa_item(hg, half):
        col = pl.multiple_of(hg * 1024 + half * 512, 512)
        w = wq_buf[:, :, pl.ds(col, 512)].reshape(512, 512)
        r = _dot(xa32_ref[...], w)
        new = qa_ref[hg]
        for j in range(4):
            new = jnp.where(row32 == half * 4 + j, r[:, 128 * j:128 * j + 128], new)
        qa_ref[hg] = new

    def qb_item(n):
        hg = n >> 1
        half = n & 1
        w = wbq_buf[pl.ds(half * 2, 2), :, hg].reshape(2048, 128)
        qb_ref[hg] = qb_ref[hg] + _dot(xexp_ref[half], w)

    def qabs_item(n, fl):
        hg = n & 3
        u = n >> 2
        q = qb_ref[hg].astype(BF16)
        w = wuk_buf[u, :, hg].reshape(1024, 128)
        r = _dot_nt(q, w)
        fl()
        r = jnp.concatenate(
            [jnp.where(row32 == lane32, r[:, 128 * k:128 * k + 128], 0.0).astype(BF16)
             for k in range(8)], axis=1)
        qa = _dot_nt(r, e0_ref[...])
        for b in range(4):
            qabs_ref[u, b, hg] = qa[8 * b:8 * b + 8, :]

    def score_item(b, n, fl):
        qa = jnp.concatenate(
            [qabs_ref[u, b].reshape(32, 128).astype(BF16) for u in range(4)], axis=1)
        seg = b * 4 + (n >> 1)
        m = jnp.where(n == 0, -jnp.inf, mb_ref[...])
        for k in range(4):
            row = pl.multiple_of((n & 1) * 512 + k * 128, 128)
            s = _dot_nt(qa, cbuf[seg, pl.ds(row, 128), :])
            if k == 0:
                fl()
            sb_ref[n, :, 128 * k:128 * k + 128] = s
            m = jnp.maximum(m, s)
        mb_ref[...] = m

    def max_b():
        mb_ref[...] = jnp.broadcast_to(jnp.max(mb_ref[...], axis=1, keepdims=True), (32, 128))

    def pv_item(b, n, fl):
        m = mb_ref[...]
        ps = [jnp.exp((sb_ref[n, :, 128 * k:128 * k + 128] - m) * scale) for k in range(4)]
        first = n == 0
        lb_ref[...] = jnp.where(first, 0.0, lb_ref[...]) + ((ps[0] + ps[1]) + (ps[2] + ps[3]))
        seg = b * 4 + (n >> 1)
        acc = jnp.where(first, 0.0, cacc_ref[...])
        for k in range(4):
            row = pl.multiple_of((n & 1) * 512 + k * 128, 128)
            d = _dot(ps[k].astype(BF16), cbuf[seg, pl.ds(row, 128), :])
            if k == 0:
                fl()
            acc = acc + d
        cacc_ref[...] = acc

    def norm_b(b):
        inv = 1.0 / jnp.sum(lb_ref[...], axis=1, keepdims=True)
        res = cacc_ref[...] * inv
        for u in range(4):
            cc_ref[u, b] = res[:, 128 * u:128 * u + 128].reshape(4, 8, 128)

    def ctx_item(n, fl):
        hg = n >> 2
        u = n & 3
        c32 = jnp.concatenate([cc_ref[u, bb, hg] for bb in range(4)], axis=0)
        w = wuv_buf[u, :, hg].reshape(1024, 128)
        ctx_ref[hg] = ctx_ref[hg] + _dot(expand(c32, fl), w)

    def out_part(o32, w_half, j0, jj, nj, fl=_nop):
        acc = None
        for j in range(jj, jj + nj):
            d = _dot(jnp.where(row32 == j0 + j, o32, 0.0).astype(BF16),
                     w_half[j * 128:j * 128 + 128, :])
            if j == jj:
                fl()
            acc = d if acc is None else acc + d
        return acc

    def out_a_item(n, fl=_nop):
        acca_ref[...] = acca_ref[...] + out_part(
            oa_ref[n >> 1], wo_buf.at[n], (n & 1) * 4, 0, 4, fl)

    def out_b_item(n, fl=_nop):
        accb_ref[...] = accb_ref[...] + out_part(
            ctx_ref[n >> 1], wbo_buf.at[n >> 1, n & 1], (n & 1) * 4, 0, 4, fl)

    def rowsum(acc):
        return jnp.sum(acc.reshape(4, 8, 512), axis=1)

    def k_work(g, r):
        hg, b = hg_of(g), batch_of(g)
        q = jnp.where(row8 < nprev_of(g),
                      qa_ref[hg, pl.ds(_mo(((b + 3) & 3) * 8, 8), 8), :],
                      qa_ref[hg, pl.ds(_mo(b * 8, 8), 8), :]).astype(BF16)
        row = pl.multiple_of(r * 128, 128)
        h0 = (g & 1) * 8
        s = jnp.zeros((8, 128), F32)
        for j in range(8):
            sj = _dot_nt(q, kvbuf[0, h0 + j, pl.ds(row, 128), :])
            s = jnp.where(row8 == j, sj, s)
        sa_ref[r] = s

    def v_part(g, r):
        p = pa_ref[r].astype(BF16)
        row = _mo(r * 128, 128)
        h0 = (g & 1) * 8
        o = jnp.zeros((8, 128), F32)
        for j in range(8):
            oj = _dot(p, kvbuf[1, h0 + j, pl.ds(row, 128), :])
            o = jnp.where(row8 == j, oj, o)
        return oacc_ref[...] + o

    def finalize_o(g):
        l = jnp.sum(psum_ref[...], axis=1, keepdims=True)
        o = oacc_ref[...] * (1.0 / l)
        hg, b = hg_of(g), batch_of(g)
        prev = row8 < nprev_of(g)
        rp = pl.ds(_mo(((b + 3) & 3) * 8, 8), 8)
        rc = pl.ds(_mo(b * 8, 8), 8)
        oa_ref[hg, rp, :] = jnp.where(prev, o, oa_ref[hg, rp, :])
        oa_ref[hg, rc, :] = jnp.where(prev, oa_ref[hg, rc, :], o)

    def softmax_a():
        s = sa_ref[...]
        m = jnp.max(jnp.max(s, axis=0), axis=1, keepdims=True)
        p = jnp.exp((s - m[None]) * scale)
        pa_ref[...] = p
        psum_ref[...] = jnp.sum(p, axis=0)
        oacc_ref[...] = jnp.zeros((8, 128), F32)

    def k0_tick(r, t, s0, h):
        wait16(0, r, t, s0 + t, h)
        start_wq(r * 16 + (t >> 2) * 8, (t & 3) * 512 + h * 256, 256, S_WQ)

    def k0a_body(r, carry):
        s0 = (r & 1) * 8
        for t in range(8):
            for h in range(2):
                k0_tick(r, t, s0, h)
                start16_first(k_hbm, 0, r + 2, t, s0 + t, h)
        return carry
    lax.fori_loop(0, 6, k0a_body, 0)

    x_prep()

    def k0b_body(r, carry):
        s0 = r * 8
        for t in range(8):
            for h in range(2):
                k0_tick(r + 6, t, s0, h)
                start_c(r * 2 + (t >> 2), t & 3, s0 + t, h)
        return carry
    lax.fori_loop(0, 2, k0b_body, 0)

    def c0_body(it, carry):
        s0 = (it & 3) * 4
        for t in range(4):
            for h in range(2):
                wait_c(it, t, s0 + t, h)
                high_3d(wbq_hbm, wbq_buf, it * 4 + t, h * 2, 2, S_WBQ).start(priority=HI)
                start_c(it + 4, t, s0 + t, h)

        @pl.when(it == 1)
        def _():
            wait_all(wq_buf.at[:, :, pl.ds(0, 2048)], S_WQ)

        @pl.when(jnp.logical_and(it >= 1, it < 5))
        def _():
            qa_item((it - 1) >> 1, (it - 1) & 1)

        @pl.when(jnp.logical_and(it >= 5, it < 13))
        def _():
            k_work(0, it - 5)

        @pl.when(it == 13)
        def _():
            softmax_a()
        return carry
    lax.fori_loop(0, 32, c0_body, 0)

    def c1_tick(it, t, s0, h):
        wait_c(32 + it, t, s0 + t, h)
        high_3d(wuk_hbm, wuk_buf, it * 4 + t, h * 2, 2, S_WUK).start(priority=HI)

    def c1_body(it, carry):
        s0 = (it & 3) * 4
        for t in range(4):
            for h in range(2):
                c1_tick(it, t, s0, h)
                start_c(36 + it, t, s0 + t, h)

        @pl.when(it == 1)
        def _():
            wait_all(wbq_buf, S_WBQ)

        @pl.when(jnp.logical_and(it >= 1, it < 9))
        def _():
            qb_item(it - 1)
        return carry
    lax.fori_loop(0, 28, c1_body, 0)

    def c1b_body(r, carry):
        for t in range(8):
            for h in range(2):
                c1_tick(28 + r * 2 + (t >> 2), t & 3, r * 8 + (t >> 2) * 4, h)
            for h in halves(t):
                start16_first(v_hbm, 1, r, t, r * 8 + t, h)
        return carry
    lax.fori_loop(0, 2, c1b_body, 0)

    def make_main(high, hook, extra, first, last):
        def body(i, carry):
            g = i >> 3
            r = i & 7
            i2 = i + 2
            g2 = i2 >> 3
            r2 = i2 & 7
            sg2 = (g2 + 1) >> 1
            odd2 = (g2 & 1) == 1
            s0 = (i & 1) * 8
            kv = 1 - (g & 1)

            def half_tick(t, h, with_high):
                wait16(kv, r, t, s0 + t, h)
                if with_high:
                    high(i, t, h)

                @pl.when(odd2)
                def _():
                    start16(k_hbm, 0, sg2, r2, t, s0 + t, h)

                if first:
                    @pl.when(i2 < 8)
                    def _():
                        start16_first(v_hbm, 1, r2, t, s0 + t, h)

                    @pl.when(i2 >= 16)
                    def _():
                        start16(v_hbm, 1, sg2, r2, t, s0 + t, h)
                elif not last:
                    @pl.when(jnp.logical_not(odd2))
                    def _():
                        start16(v_hbm, 1, sg2, r2, t, s0 + t, h)
                else:
                    @pl.when(jnp.logical_and(jnp.logical_not(odd2), i2 < N_MAIN))
                    def _():
                        start16(v_hbm, 1, sg2, r2, t, s0 + t, h)

                    if h != 1:
                        @pl.when(i2 >= N_MAIN)
                        def _():
                            low_v8(0, 2 * r2 + (t >> 2), t & 3, s0 + t).start(priority=LO)

            def tick(t, with_high=True):
                for h in halves(t):
                    half_tick(t, h, with_high)

            tick(0)
            tick(1)

            @pl.when(jnp.logical_and(r == 0, i > 0))
            def _():
                finalize_o(g - 1)
                softmax_a()

            extra(i)
            tick(2)
            tick(3)
            hook(i, lambda: high(i, 5, None))
            tick(4)
            tick(5, False)
            tick(6)
            tick(7)
            oacc_ref[...] = v_part(g, r)
            k_work(g + 1, r)
            return carry
        return body

    def cut(h, n):
        return (0, n) if h is None else (h * (n // 2), n // 2)

    def high0(i, t, h):
        o, n = cut(h, 256)
        start_wq(i * 8, 2048 + t * 256 + o, n, S_WQ + 1)

    def hook0(i, fl):
        @pl.when(i == 0)
        def _():
            wait_all(wuk_buf, S_WUK)

        qabs_item(i, fl)

    def high1(i, t, h):
        @pl.when(i < 48)
        def _():
            o, n = cut(h, 2)
            high_3d(wuv_hbm, wuv_buf, (i - 16) * 4 + (t >> 1), (t & 1) * 2 + o, n,
                    S_WUV).start(priority=HI)

        @pl.when(i >= 48)
        def _():
            o, n = cut(h, 256)
            high_wbo((i >> 4) - 3, (i & 15) * 32 + (t >> 1) * 8, (t & 1) * 256 + o,
                     n).start(priority=HI)

    def extra1(i):
        n = i - 16

        @pl.when(i == 25)
        def _():
            wait_all(wq_buf.at[:, :, pl.ds(2048, 2048)], S_WQ + 1)

        @pl.when(jnp.logical_and(i >= 25, i < 29))
        def _():
            qa_item(2 + ((i - 25) >> 1), (i - 25) & 1)

        @pl.when((n & 15) == 8)
        def _():
            max_b()

        @pl.when(jnp.logical_and((n & 15) == 1, n > 16))
        def _():
            norm_b((n >> 4) - 1)

    def hook1(i, fl):
        n = i - 16

        @pl.when((n & 8) == 0)
        def _():
            score_item(n >> 4, n & 7, fl)

        @pl.when((n & 8) != 0)
        def _():
            pv_item(n >> 4, n & 7, fl)

    def high2(i, t, h):
        row = (i & 15) * 32 + (t >> 1) * 8
        o, n = cut(h, 256)

        @pl.when(i < 96)
        def _():
            for p0, np_ in WO_RUNS:
                high_wo(p0, np_, row, 8, (t & 1) * 256 + o, n, S_WO).start(priority=HI)

        @pl.when(i >= 96)
        def _():
            high_wo(4, 2, row, 8, (t & 1) * 256 + o, n, S_WO + 1).start(priority=HI)

    def extra2(i):
        @pl.when(i == 80)
        def _():
            wait_all(wuv_buf, S_WUV)
            norm_b(3)

        @pl.when(i == 96)
        def _():
            wait_all(wbo_buf, S_WBO)

        @pl.when(i == 105)
        def _():
            wait_all(wo_buf.at[pl.ds(0, 4)], S_WO)
            obuf[1] = rowsum(accb_ref[...]).astype(obuf.dtype)
            out_copy(1).start(priority=HI)

    def hook2(i, fl):
        @pl.when(i < 96)
        def _():
            ctx_item(i - 80, fl)

        @pl.when(jnp.logical_and(i >= 96, i < 104))
        def _():
            out_b_item(i - 96, fl)

        @pl.when(jnp.logical_and(i >= 105, i < 109))
        def _():
            out_a_item(i - 105, fl)

        @pl.when(jnp.logical_or(i == 104, i >= 109))
        def _():
            fl()

    lax.fori_loop(0, 16, make_main(high0, hook0, _nop, True, False), 0)
    lax.fori_loop(16, 80, make_main(high1, hook1, extra1, False, False), 0)
    lax.fori_loop(80, N_MAIN, make_main(high2, hook2, extra2, False, True), 0)

    finalize_o(13)
    softmax_a()

    def g14_body(r, carry):
        s0 = (r & 3) * 4
        nx = r + 4
        for t in range(4):
            low_v8(0, r, t, s0 + t).wait()
            high_wo(6, 1, r * 32 + t * 8, 8, 0, 512, S_WO + 2).start(priority=HI)
            low_v8(nx >> 3, nx & 7, t, s0 + t).start(priority=LO)
        oacc_ref[...] = v_part(14, r)
        k_work(15, r)
        return carry
    lax.fori_loop(0, 8, g14_body, 0)

    finalize_o(14)
    softmax_a()

    def v15_body(r, carry):
        s0 = (r & 3) * 4
        for t in range(4):
            low_v8(1, r, t, s0 + t).wait()

            @pl.when(r < NBIG)
            def _():
                high_wo(6, 1, 256 + r * 64 + t * 16, 16, 0, 512, S_WO + 2).start(priority=HI)

            @pl.when(jnp.logical_and(r >= NBIG, r < 8 - NBIG))
            def _():
                high_wo(6, 1, 256 + NBIG * 32 + r * 32 + t * 8, 8, 0, 512,
                        S_WO + 2).start(priority=HI)

            @pl.when(r < 4)
            def _():
                low_v8(1, r + 4, t, s0 + t).start(priority=LO)

            @pl.when(jnp.logical_and(r >= 4, r < 6))
            def _():
                low_wo(s0 + t, s0 + t).start(priority=LO)

            if t == 1:
                @pl.when(r == 1)
                def _():
                    wait_all(wo_buf.at[pl.ds(4, 2)], S_WO + 1)

                @pl.when(jnp.logical_and(r >= 1, r < 3))
                def _():
                    out_a_item(r + 3)

                @pl.when(r == 4)
                def _():
                    l = jnp.sum(psum_ref[...], axis=1, keepdims=True)
                    psum_ref[...] = jnp.broadcast_to(1.0 / l, (8, 128))
        oacc_ref[...] = v_part(15, r)
        return carry
    lax.fori_loop(0, 7, v15_body, 0)

    for t in range(4):
        low_v8(1, 7, t, 12 + t).wait()
    oa_ref[3, 24:32, :] = v_part(15, 7) * psum_ref[...]
    wait_all(wo_buf.at[pl.ds(6, 1)], S_WO + 2)
    for n in range(2):
        low_wo(n, n).wait()
    o32 = oa_ref[3]
    part_ref[0:4, :] = rowsum(acca_ref[...] + out_part(o32, wo_buf.at[6], 0, 0, 4)
                              + out_part(o32, wo_buf.at[7], 4, 0, 1))
    for j in range(5, 8):
        olast_ref[0:4, (j - 5) * 128:(j - 4) * 128] = o32.reshape(4, 8, 128)[:, j, :]
    for n in range(2, NSPLIT):
        low_wo(n, n).wait()
    k1 = NSPLIT * 64
    part_ref[...] = part_ref[...] + _dot(
        olast_ref[:, 0:k1 - 128].astype(BF16), wo_buf[7, 128:k1, :])
    lhs = olast_ref[:, k1 - 128:384].astype(BF16)
    for n in range(NSPLIT, 8):
        low_wo(n, n).wait()
    res = part_ref[...] + _dot(lhs, wo_buf[7, k1:512, :])
    obuf[0] = res[0:4, :].astype(obuf.dtype)
    out_copy(0).start(priority=HI)
    out_copy(1).wait()
    out_copy(0).wait()


@jax.jit
def pallas_concat_heads__sliding_block_cached__compressed_kv_cla__decode_kernel(
    A_x: jax.Array,
    A_k_cache: jax.Array,
    A_v_cache: jax.Array,
    A_wq: jax.Array,
    A_wo: jax.Array,
    B_x: jax.Array,
    B_c_kv: jax.Array,
    B_w_q: jax.Array,
    B_w_uk: jax.Array,
    B_w_uv: jax.Array,
    B_w_o: jax.Array,
):
    B, Sq, D = A_x.shape
    _, H, Sk, Dh = A_k_cache.shape
    W = min(4096, max(256, Sk // 4))
    assert (B, Sq, D, H, Sk, Dh, W) == (4, 1, 512, 32, 4096, 128, 1024)
    assert B_c_kv.shape == (4, 4096, 512) and B_w_q.shape == (512, 32, 128)

    def body(*refs):
        _kernel(*refs, win_off=Sk - W, scale=float(Dh) ** -0.5)

    vm = pltpu.VMEM
    scratch = [
        vm((2, 16, 1024, 128), BF16),
        vm((16, 1024, 512), BF16),
        vm((4, 128, 4096), BF16),
        vm((8, 512, 512), BF16),
        vm((4, 128, 4, 8, 128), BF16),
        vm((4, 128, 4, 8, 128), BF16),
        vm((4, 128, 4, 8, 128), BF16),
        vm((4, 2, 512, 512), BF16),
        vm((4, 512), BF16),
        vm((4, 512), BF16),
        vm((128, 1024), BF16),
        vm((32, 512), BF16),
        vm((2, 32, 2048), BF16),
        vm((4, 32, 128), F32),
        vm((8, 8, 128), F32),
        vm((8, 8, 128), F32),
        vm((8, 128), F32),
        vm((8, 128), F32),
        vm((4, 32, 128), F32),
        vm((4, 32, 128), F32),
        vm((4, 4, 4, 8, 128), F32),
        vm((8, 32, 512), F32),
        vm((32, 128), F32),
        vm((32, 128), F32),
        vm((32, 512), F32),
        vm((4, 4, 4, 8, 128), F32),
        vm((4, 32, 128), F32),
        vm((32, 512), F32),
        vm((32, 512), F32),
        vm((8, 384), F32),
        vm((8, 512), F32),
        vm((2, 4, 512), A_x.dtype),
        pltpu.SemaphoreType.DMA((2 * NS,)),
        pltpu.SemaphoreType.DMA((N_HSEM,)),
        pltpu.SemaphoreType.DMA((4,)),
    ]
    out = pl.pallas_call(
        body,
        out_shape=jax.ShapeDtypeStruct((B, 2 * D), A_x.dtype),
        in_specs=[pl.BlockSpec(memory_space=pl.ANY)] * 11,
        out_specs=pl.BlockSpec(memory_space=pl.ANY),
        scratch_shapes=scratch,
        compiler_params=pltpu.CompilerParams(
            vmem_limit_bytes=64 * 1024 * 1024,
            disable_bounds_checks=True,
            disable_semaphore_checks=True,
        ),
    )(
        A_x.reshape(B, D),
        A_k_cache.reshape(B * H, Sk, Dh),
        A_v_cache.reshape(B * H, Sk, Dh),
        A_wq.reshape(4, 128, 4096),
        A_wo.reshape(8, 512, 512),
        B_x.reshape(B, D),
        B_c_kv.reshape(16, 1024, 512),
        B_w_q.reshape(4, 128, 4, 8, 128),
        B_w_uk.reshape(4, 128, 4, 8, 128),
        B_w_uv.reshape(4, 128, 4, 8, 128),
        B_w_o.reshape(4, 2, 512, 512),
    )
    return out.reshape(B, Sq, 2 * D)
```
